```python
import jax
import jax.numpy as jnp

def _softmax(x, axis=-1):
    return jax.nn.softmax(x, axis=axis)

def _gelu(x):
    return jax.nn.gelu(x, approximate=True)

def _silu(x):
    return jax.nn.silu(x)

def _sigmoid(x):
    return jax.nn.sigmoid(x)

def _layernorm(x, axis=-1, eps=1e-05):
    m = jnp.mean(x, axis=axis, keepdims=True)
    v = jnp.var(x, axis=axis, keepdims=True)
    return (x - m) / jnp.sqrt(v + eps)

def _scatter_add(tgt, idx, src, axis=0):
    return tgt.at[idx].add(src)

def _segment_sum(src, seg, n):
    return jax.ops.segment_sum(src, seg, n)

class _Rng:

    def __init__(self, key):
        self._k = key

    def _next(self):
        self._k, sub = jax.random.split(self._k)
        return sub

    def normal(self, shape):
        return jax.random.normal(self._next(), shape, dtype=jnp.bfloat16)

    def randint(self, lo, hi, shape):
        return jax.random.randint(self._next(), shape, lo, hi, dtype=jnp.int32)

    def uniform(self, shape, lo=0.0, hi=1.0):
        return jax.random.uniform(self._next(), shape, jnp.bfloat16, lo, hi)

    def permutation(self, n):
        return jax.random.permutation(self._next(), n)
kernel_name = 'interleave_layers__memory_aug_recurrent_mem_tr__sliding_local_dilated__prompt'

def setup_inputs():
    _rng = _Rng(jax.random.key(int.from_bytes(__import__("os").urandom(4), "little")))
    _w = lambda a: (lambda t: t.astype(jnp.bfloat16) if jnp.issubdtype(t.dtype, jnp.floating) else t)(jnp.asarray(a))

    def _A_setup():
        B, S, Dm = (1, 2048, 640)
        H, Dh = (32, 192)
        M, seg = (8, 32)
        seg = min(seg, S)
        S = S // seg * seg
        return {'x': _w((lambda *s: _rng.normal(s) * 0.05)(B, S, Dm)), 'mem0': _w((lambda *s: _rng.normal(s) * 0.05)(B, M, Dm)), 'Wq': _w((lambda *s: _rng.normal(s) * 0.05)(Dm, H, Dh) * Dm ** (-0.5)), 'Wk': _w((lambda *s: _rng.normal(s) * 0.05)(Dm, H, Dh) * Dm ** (-0.5)), 'Wv': _w((lambda *s: _rng.normal(s) * 0.05)(Dm, H, Dh) * Dm ** (-0.5)), 'Wo': _w((lambda *s: _rng.normal(s) * 0.05)(H, Dh, Dm) * (H * Dh) ** (-0.5)), 'seg_len': seg}
    _A_in = _A_setup()

    def _B_setup():
        B, S, D = (1, 2048, 640)
        return {'x': _w((lambda *s: _rng.normal(s) * 0.05)(B, S, D)), 'wqkv': _w((lambda *s: _rng.normal(s) * 0.05)(D, 3 * D)), 'wo': _w((lambda *s: _rng.normal(s) * 0.05)(D, D))}
    _B_in = _B_setup()
    return {'A_x': _A_in['x'], 'A_mem0': _A_in['mem0'], 'A_Wq': _A_in['Wq'], 'A_Wk': _A_in['Wk'], 'A_Wv': _A_in['Wv'], 'A_Wo': _A_in['Wo'], 'A_seg_len': _A_in['seg_len'], 'B_x': _B_in['x'], 'B_wqkv': _B_in['wqkv'], 'B_wo': _B_in['wo']}

def reference(A_x, A_mem0, A_Wq, A_Wk, A_Wv, A_Wo, A_seg_len, B_x, B_wqkv, B_wo):

    def _A_ref(x, mem0, Wq, Wk, Wv, Wo, seg_len):
        B, S, Dm = x.shape
        H, Dh = (Wq.shape[1], Wq.shape[2])
        M = mem0.shape[1]
        scale = Dh ** (-0.5)
        n_seg = S // seg_len
        L = M + seg_len
        idx = jnp.arange(L)
        mask = (idx[:, None] < M) | (idx[:, None] >= idx[None, :])
        mem = mem0
        outs = []
        for s in range(n_seg):
            xs = x[:, s * seg_len:(s + 1) * seg_len, :].copy()
            h = jnp.concatenate([mem, xs], axis=1)
            q = jnp.einsum('btd,dhe->bhte', h, Wq)
            k = jnp.einsum('btd,dhe->bhte', h, Wk)
            v = jnp.einsum('btd,dhe->bhte', h, Wv)
            scores = jnp.einsum('bhqe,bhke->bhqk', q, k) * scale
            scores = jnp.where(mask[None, None], scores, -1000000000.0)
            p = _softmax(scores, axis=-1)
            o = jnp.einsum('bhqk,bhke->bhqe', p, v)
            o = jnp.einsum('bhte,hed->btd', o, Wo)
            mem = o[:, :M, :].copy()
            outs.append(o[:, M:, :])
        return jnp.concatenate(outs, axis=1)

    def _B_ref(x, wqkv, wo):
        B, S, D = x.shape
        H = 32
        Dh = D // H
        W, dil = (8, 2)
        qkv = (lambda x, *d: x.transpose(*d))((x @ wqkv).reshape(B, S, 3, H, Dh), 2, 0, 3, 1, 4)
        q, k, v = (qkv[0], qkv[1], qkv[2])
        scale = Dh ** (-0.5)
        pos = jnp.arange(S)
        off = jnp.arange(W) * dil
        idx = pos[:, None] - off[None, :]
        mask = idx >= 0
        idx_c = jnp.where(mask, idx, 0).reshape(-1)
        kg = k[:, :, idx_c, :].reshape(B, H, S, W, Dh)
        vg = v[:, :, idx_c, :].reshape(B, H, S, W, Dh)
        logits = jnp.einsum('bhsd,bhswd->bhsw', q, kg) * scale
        logits = jnp.where(mask[None, None, :, :], logits, -1000000000.0)
        attn = _softmax(logits, axis=-1)
        o = jnp.einsum('bhsw,bhswd->bhsd', attn, vg)
        return (lambda x, *d: x.transpose(*d))(o, 0, 2, 1, 3).reshape(B, S, D) @ wo
    x = A_x
    x = x + _A_ref(_layernorm(x, axis=-1), A_mem0, A_Wq, A_Wk, A_Wv, A_Wo, A_seg_len)
    x = x + _B_ref(_layernorm(x, axis=-1), B_wqkv, B_wo)
    x = x + _A_ref(_layernorm(x, axis=-1), A_mem0, A_Wq, A_Wk, A_Wv, A_Wo, A_seg_len)
    x = x + _B_ref(_layernorm(x, axis=-1), B_wqkv, B_wo)
    return x
```

```python
import jax
import jax.numpy as jnp
from jax import lax
import jax.experimental.pallas as pl
import jax.experimental.pallas.tpu as pltpu

S, D = 2048, 640
H, DH = 32, 192
HD = H * DH
M, SEG = 8, 32
NSEG = S // SEG
R = 2 * (M + SEG)
PW = 2 * DH
NPAIR = H // 2
BH, BDH, BW, BDIL = 32, 20, 8, 2
NC = D // 128
F32, BF16 = jnp.float32, jnp.bfloat16
NT = (((1,), (1,)), ((), ()))


def _ln(x):
    m = jnp.mean(x, axis=-1, keepdims=True)
    xc = x - m
    v = jnp.mean(xc * xc, axis=-1, keepdims=True)
    return xc * lax.rsqrt(v + 1e-5)


def _kernel(x_ref, mem0_ref, wq_ref, wk_ref, wv_ref, wo_ref, bwqkv_ref, bwo_ref,
            out_ref,
            h_ref, res_ref, xb_ref, bq_ref, bkv_ref, bo_ref, pwqkv_ref, pwo_ref):
    ri = lax.broadcasted_iota(jnp.int32, (D, D), 0)
    ci = lax.broadcasted_iota(jnp.int32, (D, D), 1)
    pm = (ri == (ci & 31) * BDH + (ci >> 5)).astype(F32).astype(BF16)
    pmt = (ci == (ri & 31) * BDH + (ri >> 5)).astype(F32).astype(BF16)
    for j in range(3):
        pwqkv_ref[:, j * D:(j + 1) * D] = jnp.dot(
            bwqkv_ref[:, j * D:(j + 1) * D], pm, preferred_element_type=F32).astype(BF16)
    pwo_ref[...] = jnp.dot(pmt, bwo_ref[...], preferred_element_type=F32).astype(BF16)

    mem0 = mem0_ref[...].astype(F32)
    x0 = x_ref[0:SEG, :].astype(F32)
    h_ref[...] = jnp.concatenate(
        [mem0, mem0, _ln(x0), jnp.zeros((SEG, D), F32)], axis=0).astype(BF16)
    res_ref[...] = jnp.concatenate([x0, jnp.zeros((SEG, D), F32)], axis=0)
    xb_ref[...] = jnp.zeros((2 * SEG, D), F32)
    bkv_ref[...] = jnp.zeros(bkv_ref.shape, F32)

    def a_phase():
        qi = lax.broadcasted_iota(jnp.int32, (R, R), 0)
        ki = lax.broadcasted_iota(jnp.int32, (R, R), 1)
        lay = lambda i: jnp.where(i < 2 * M, i >> 3, (i - 2 * M) >> 5)
        same = lay(qi) == lay(ki)
        allowed = same & ((qi < 2 * M) | (ki <= qi))
        fill = jnp.where(same, -1e9, -jnp.inf).astype(F32)
        lo = lax.broadcasted_iota(jnp.int32, (R, 128), 1) < 64
        scale = DH ** -0.5

        def softmax(s):
            s = jnp.where(allowed, s * scale, fill)
            m = jnp.max(s, axis=-1, keepdims=True)
            e = jnp.exp(s - m)
            return (e * (1.0 / jnp.sum(e, axis=-1, keepdims=True))).astype(BF16)

        h = h_ref[...]
        acc = jnp.zeros((R, D), F32)
        for p in range(NPAIR):
            rows = pl.ds(p * PW, PW)
            q = lax.dot_general(h, wq_ref[rows, :], NT, preferred_element_type=F32).astype(BF16)
            k = lax.dot_general(h, wk_ref[rows, :], NT, preferred_element_type=F32)
            v = lax.dot_general(h, wv_ref[rows, :], NT, preferred_element_type=F32).astype(BF16)
            km = k[:, 128:256]
            ka = jnp.concatenate([k[:, :128], jnp.where(lo, km, 0.0)], axis=1).astype(BF16)
            kb = jnp.concatenate([jnp.where(lo, 0.0, km), k[:, 256:]], axis=1).astype(BF16)
            sa = lax.dot_general(q[:, :256], ka, NT, preferred_element_type=F32)
            sb = lax.dot_general(q[:, 128:], kb, NT, preferred_element_type=F32)
            oa = jnp.dot(softmax(sa), v[:, :256], preferred_element_type=F32)
            ob = jnp.dot(softmax(sb), v[:, 128:], preferred_element_type=F32)
            o = jnp.concatenate(
                [oa[:, :128], jnp.where(lo, oa[:, 128:], ob[:, :128]), ob[:, 128:]],
                axis=1).astype(BF16)
            acc = acc + jnp.dot(o, wo_ref[rows, :], preferred_element_type=F32)
        return acc

    def b_phase(t):
        xb = xb_ref[...]
        qkv = jnp.dot(_ln(xb).astype(BF16), pwqkv_ref[...], preferred_element_type=F32)
        for l in range(2):
            for c in range(NC):
                bq_ref[c, l * SEG:(l + 1) * SEG, :] = qkv[l * SEG:(l + 1) * SEG, c * 128:(c + 1) * 128]
                for j in range(2):
                    bkv_ref[l, j, c, 0:16, :] = bkv_ref[l, j, c, SEG:SEG + 16, :]
                    bkv_ref[l, j, c, 16:16 + SEG, :] = qkv[
                        l * SEG:(l + 1) * SEG, (j + 1) * D + c * 128:(j + 1) * D + (c + 1) * 128]
        bscale = BDH ** -0.5
        ri8 = lax.broadcasted_iota(jnp.int32, (8, 128), 0)
        for l in range(2):
            seg = t - 1 - 2 * l
            for r in range(SEG // 8):
                pos = seg * SEG + r * 8 + ri8
                q = [bq_ref[c, l * SEG + r * 8:l * SEG + r * 8 + 8, :] for c in range(NC)]
                lg = []
                for w in range(BW):
                    o0 = 16 + r * 8 - BDIL * w
                    s = q[0] * bkv_ref[l, 0, 0, o0:o0 + 8, :]
                    for c in range(1, NC):
                        s = s + q[c] * bkv_ref[l, 0, c, o0:o0 + 8, :]
                    s = s + pltpu.roll(s, 64, 1)
                    s = s + pltpu.roll(s, 32, 1)
                    s = s * bscale
                    if r * 8 - BDIL * w < 0:
                        s = jnp.where(pos - BDIL * w >= 0, s, -1e9)
                    lg.append(s)
                m = lg[0]
                for w in range(1, BW):
                    m = jnp.maximum(m, lg[w])
                e = [jnp.exp(s - m) for s in lg]
                den = e[0]
                for w in range(1, BW):
                    den = den + e[w]
                inv = 1.0 / den
                for c in range(NC):
                    o = e[0] * bkv_ref[l, 1, c, 16 + r * 8:16 + r * 8 + 8, :]
                    for w in range(1, BW):
                        o0 = 16 + r * 8 - BDIL * w
                        o = o + e[w] * bkv_ref[l, 1, c, o0:o0 + 8, :]
                    bo_ref[l * SEG + r * 8:l * SEG + r * 8 + 8, c * 128:(c + 1) * 128] = o * inv
        y = jnp.dot(bo_ref[...].astype(BF16), pwo_ref[...], preferred_element_type=F32)
        return xb + y

    def write_out(t, xo):
        row = pl.multiple_of(jnp.maximum(t - 3, 0) * SEG, SEG)
        out_ref[pl.ds(row, SEG), :] = xo.astype(out_ref.dtype)

    def step(t, carry):
        yb = b_phase(t)
        acc = a_phase()
        write_out(t, yb[SEG:])
        xb_ref[...] = res_ref[...] + acc[2 * M:]
        nrow = pl.multiple_of(jnp.minimum(t + 1, NSEG - 1) * SEG, SEG)
        xn = x_ref[pl.ds(nrow, SEG), :].astype(F32)
        x2 = yb[:SEG]
        mem2 = jnp.where(t < 2, mem0_ref[...].astype(F32), acc[M:2 * M])
        h_ref[...] = jnp.concatenate([acc[:M], mem2, _ln(xn), _ln(x2)], axis=0).astype(BF16)
        res_ref[...] = jnp.concatenate([xn, x2], axis=0)
        return carry

    lax.fori_loop(0, NSEG + 2, step, 0)
    yb = b_phase(NSEG + 2)
    write_out(NSEG + 2, yb[SEG:])


@jax.jit
def pallas_interleave_layers__memory_aug_recurrent_mem_tr__sliding_local_dilated__prompt_kernel(
    A_x, A_mem0, A_Wq, A_Wk, A_Wv, A_Wo, A_seg_len, B_x, B_wqkv, B_wo,
):
    del A_seg_len, B_x
    wt = lambda w: jnp.transpose(w, (1, 2, 0)).reshape(HD, D)
    vm = pl.BlockSpec(memory_space=pltpu.VMEM)
    out = pl.pallas_call(
        _kernel,
        out_shape=jax.ShapeDtypeStruct((S, D), A_x.dtype),
        in_specs=[vm] * 8,
        out_specs=vm,
        scratch_shapes=[
            pltpu.VMEM((R, D), BF16),
            pltpu.VMEM((2 * SEG, D), F32),
            pltpu.VMEM((2 * SEG, D), F32),
            pltpu.VMEM((NC, 2 * SEG, 128), F32),
            pltpu.VMEM((2, 2, NC, 16 + SEG, 128), F32),
            pltpu.VMEM((2 * SEG, D), F32),
            pltpu.VMEM((D, 3 * D), BF16),
            pltpu.VMEM((D, D), BF16),
        ],
        compiler_params=pltpu.CompilerParams(vmem_limit_bytes=100 * 2 ** 20),
    )(A_x.reshape(S, D), A_mem0.reshape(M, D), wt(A_Wq), wt(A_Wk), wt(A_Wv),
      A_Wo.reshape(HD, D), B_wqkv, B_wo)
    return out.reshape(1, S, D)
```

```python
import jax
import jax.numpy as jnp
from jax import lax
import jax.experimental.pallas as pl
import jax.experimental.pallas.tpu as pltpu

S, D = 2048, 640
H, DH = 32, 192
HD = H * DH
M, SEG = 8, 32
L = M + SEG
NSEG = S // SEG
R = 2 * L
R1 = 2 * M + SEG
PW = 2 * DH
NPAIR = H // 2
BDH, BW, BDIL = 20, 8, 2
NC = D // 128
XF = 4 * SEG
F32, BF16, U32 = jnp.float32, jnp.bfloat16, jnp.uint32
WIN = 2
NT = (((1,), (1,)), ((), ()))
BWO_PAIR = 10


def _ln(x):
    m = jnp.mean(x, axis=-1, keepdims=True)
    xc = x - m
    v = jnp.mean(xc * xc, axis=-1, keepdims=True)
    return xc * lax.rsqrt(v + 1e-5)


def _nt(a, b):
    return lax.dot_general(a, b, NT, preferred_element_type=F32)


def _nn(a, b):
    return jnp.dot(a, b, preferred_element_type=F32)


def _cat0(*a):
    return jnp.concatenate(a, axis=0)


def _kernel(x_hbm, mem0_ref, wq_hbm, wk_hbm, wv_hbm, wo_hbm, bwqkv_hbm, bwo_hbm,
            out_hbm,
            x_ref, out_ref, wl_ref, w_ref, bwqkv_ref, bwo_ref, pwqkv_ref, pwo_ref,
            h_ref, res_ref, xb_ref, bq_ref, bkv_ref, bo_ref, wsem, sem):
    def w_copies(p):
        rows = pl.ds(p * PW, PW)
        return [pltpu.make_async_copy(src.at[rows, :], wl_ref.at[m, rows, :], wsem.at[p])
                for m, src in enumerate((wq_hbm, wk_hbm, wv_hbm, wo_hbm))]

    x_first = pltpu.make_async_copy(x_hbm.at[pl.ds(0, XF), :], x_ref.at[pl.ds(0, XF), :], sem.at[0])
    x_rest = pltpu.make_async_copy(x_hbm.at[pl.ds(XF, S - XF), :], x_ref.at[pl.ds(XF, S - XF), :], sem.at[1])
    bw1 = pltpu.make_async_copy(bwqkv_hbm, bwqkv_ref, sem.at[2])
    bw2 = pltpu.make_async_copy(bwo_hbm, bwo_ref, sem.at[3])
    osplit = (NSEG - 2) * SEG
    out_a = pltpu.make_async_copy(out_ref.at[pl.ds(0, osplit), :], out_hbm.at[pl.ds(0, osplit), :], sem.at[4])
    out_b = pltpu.make_async_copy(out_ref.at[pl.ds(osplit, S - osplit), :],
                                  out_hbm.at[pl.ds(osplit, S - osplit), :], sem.at[5])
    def start_w(p):
        for cp in w_copies(p):
            cp.start()

    x_first.start()
    for p in range(WIN):
        start_w(p)

    def wait_w(p):
        for cp in w_copies(p):
            cp.wait()
        if p == 0:
            bw2.start()
            bw1.start()
        if p + WIN < NPAIR:
            start_w(p + WIN)
        if p + WIN == NPAIR:
            x_rest.start()

    def weights(m, p):
        return pltpu.bitcast(w_ref[m, pl.ds(p * PW // 2, PW // 2), :], BF16)

    def weights_first(m, p):
        w = wl_ref[m, pl.ds(p * PW, PW), :]
        w_ref[m, pl.ds(p * PW // 2, PW // 2), :] = pltpu.bitcast(w, U32)
        return w

    def permute_b(p):
        i = p - 3
        if not 0 <= i < 8:
            return
        j, half = i // 2, i % 2
        hr = D // 2
        if j == 0:
            if half == 0:
                bw2.wait()
            ri = lax.broadcasted_iota(jnp.int32, (hr, D), 0) + half * hr
            ci = lax.broadcasted_iota(jnp.int32, (hr, D), 1)
            pmt = (ci == (ri & 31) * BDH + (ri >> 5)).astype(F32).astype(BF16)
            y = _nn(pmt, bwo_ref[...]).astype(BF16)
            pwo_ref[half * hr // 2:(half + 1) * hr // 2, :] = pltpu.bitcast(y, U32)
        else:
            if i == 2:
                bw1.wait()
            ri = lax.broadcasted_iota(jnp.int32, (D, D), 0)
            ci = lax.broadcasted_iota(jnp.int32, (D, D), 1)
            pm = (ri == (ci & 31) * BDH + (ci >> 5)).astype(F32).astype(BF16)
            cols = slice((j - 1) * D, j * D)
            y = _nn(bwqkv_ref[half * hr:(half + 1) * hr, cols], pm).astype(BF16)
            pwqkv_ref[half * hr // 2:(half + 1) * hr // 2, cols] = pltpu.bitcast(y, U32)

    scale = DH ** -0.5
    ninf = -jnp.inf

    def softmax2(s, first, allowed):
        s = jnp.where(allowed, s * scale, -1e9)
        m0 = jnp.max(jnp.where(first, s, ninf), axis=-1, keepdims=True)
        m1 = jnp.max(jnp.where(first, ninf, s), axis=-1, keepdims=True)
        e = jnp.exp(s - jnp.where(first, m0, m1))
        d0 = jnp.sum(jnp.where(first, e, 0.0), axis=-1, keepdims=True)
        d1 = jnp.sum(jnp.where(first, 0.0, e), axis=-1, keepdims=True)
        return e, pl.reciprocal(d0, approx=True), pl.reciprocal(d1, approx=True)

    def masks(rows):
        qi = lax.broadcasted_iota(jnp.int32, (rows, R), 0)
        ki = lax.broadcasted_iota(jnp.int32, (rows, R), 1)
        first = ki < L
        kk = jnp.where(first, ki, ki - L)
        qq = M + ((qi - 2 * M) & (SEG - 1))
        allowed = (qi < 2 * M) | (kk <= qq)
        return qi, first, allowed

    def attn_two_layers():
        qi, first, allowed = masks(R)
        row_l1 = (qi < M) | ((qi >= 2 * M) & (qi < R1))
        is_a = first == row_l1
        lo = lax.broadcasted_iota(jnp.int32, (L, 128), 1) < 64

        def arrange(a):
            a1 = _cat0(a[0:M], a[2 * M:R1])
            a2 = _cat0(a[M:2 * M], a[R1:])
            cat = lambda u, w: _cat0(u, w).astype(BF16)
            m1, m2 = a1[:, 128:256], a2[:, 128:256]
            return (cat(a1[:, :128], a2[:, :128]), cat(a2[:, 256:], a1[:, 256:]),
                    cat(jnp.where(lo, m1, 0.0), jnp.where(lo, 0.0, m1)),
                    cat(jnp.where(lo, 0.0, m2), jnp.where(lo, m2, 0.0)))

        g1 = lambda a: a[0:R1]
        g2 = lambda a: _cat0(a[0:2 * M], a[R1:])
        merge = lambda u1, u2: _cat0(u1[0:M], u2[M:2 * M], u1[2 * M:], u2[2 * M:])

        def scores(q, kt):
            qm = q[:, 128:256]
            return _nt(q[:, :128], kt[0]), _nt(q[:, 256:], kt[1]), _nt(g1(qm), kt[2]), _nt(g2(qm), kt[3])

        lo_r = lax.broadcasted_iota(jnp.int32, (R, 128), 1) < 64
        pick = lambda u1, u2: _cat0(u1[0:M], u2[M:2 * M], u1[2 * M:R1], u2[R1:])

        def pv(s4, vt):
            sa, sb, s1, s2 = s4
            p, r0, r1 = softmax2(jnp.where(is_a, sa, sb) + merge(s1, s2), first, allowed)
            pb = p.astype(BF16)
            oa = _nn(jnp.where(is_a, p, 0.0).astype(BF16), vt[0])
            ob = _nn(jnp.where(is_a, 0.0, p).astype(BF16), vt[1])
            om = merge(_nn(g1(pb), vt[2]), _nn(g2(pb), vt[3]))
            ra, rb = pick(r0, r1), pick(r1, r0)
            return jnp.concatenate(
                [oa * ra, om * jnp.where(lo_r, ra, rb), ob * rb], axis=1).astype(BF16)

        return arrange, scores, pv

    def attn_one_layer(layer):
        _, first, allowed = masks(R1)
        head_a = lax.broadcasted_iota(jnp.int32, (L, PW), 1) < DH

        def arrange(a):
            a1 = _cat0(a[layer * M:(layer + 1) * M], a[2 * M:])
            return _cat0(jnp.where(head_a, a1, 0.0), jnp.where(head_a, 0.0, a1)).astype(BF16)

        head_a1 = lax.broadcasted_iota(jnp.int32, (R1, PW), 1) < DH

        def pv(s, vt):
            p, r0, r1 = softmax2(s, first, allowed)
            return (_nn(p.astype(BF16), vt) * jnp.where(head_a1, r0, r1)).astype(BF16)

        return arrange, _nt, pv

    def a_phase(h, attn, hooks, wait=lambda p: None, weights=weights):
        arrange, scores, pv = attn
        proj = lambda m, p: _nt(h, weights(m, p))
        proj_o = lambda o, p: _nn(o, weights(3, p))
        wait(0)
        q, kt = proj(0, 0).astype(BF16), arrange(proj(1, 0))
        hooks(-1)
        vt = arrange(proj(2, 0))
        acc = None
        held = {}
        for p in range(NPAIR):
            last = p == NPAIR - 1
            s = scores(q, kt)
            if not last:
                wait(p + 1)
                q, kt = proj(0, p + 1).astype(BF16), arrange(proj(1, p + 1))
            else:
                acc = acc + proj_o(held[p - 2], p - 2)
            hooks(p)
            o = pv(s, vt)
            if not last:
                vt = arrange(proj(2, p + 1))
            else:
                acc = acc + proj_o(held[p - 1], p - 1)
            if p in (NPAIR - 3, NPAIR - 2):
                held[p] = o
            else:
                y = proj_o(o, p)
                acc = y if acc is None else acc + y
        return acc

    def b_phase1(t):
        w = pltpu.bitcast(pwqkv_ref[...], BF16)
        qkv = _nn(_ln(xb_ref[...]).astype(BF16), w)
        for l in range(2):
            for c in range(NC):
                bq_ref[c, l * SEG:(l + 1) * SEG, :] = qkv[l * SEG:(l + 1) * SEG, c * 128:(c + 1) * 128]
                for j in range(2):
                    bkv_ref[l, j, c, 0:16, :] = bkv_ref[l, j, c, SEG:SEG + 16, :]
                    bkv_ref[l, j, c, 16:16 + SEG, :] = qkv[
                        l * SEG:(l + 1) * SEG, (j + 1) * D + c * 128:(j + 1) * D + (c + 1) * 128]
        bscale = BDH ** -0.5
        ri8 = lax.broadcasted_iota(jnp.int32, (8, 128), 0)
        for l in range(2):
            seg = t - 1 - 2 * l
            for r in range(SEG // 8):
                pos = seg * SEG + r * 8 + ri8
                q = [bq_ref[c, l * SEG + r * 8:l * SEG + r * 8 + 8, :] for c in range(NC)]
                lg = []
                for w in range(BW):
                    o0 = 16 + r * 8 - BDIL * w
                    s = q[0] * bkv_ref[l, 0, 0, o0:o0 + 8, :]
                    for c in range(1, NC):
                        s = s + q[c] * bkv_ref[l, 0, c, o0:o0 + 8, :]
                    s = s + pltpu.roll(s, 64, 1)
                    s = s + pltpu.roll(s, 32, 1)
                    s = s * bscale
                    if r * 8 - BDIL * w < 0:
                        s = jnp.where(pos - BDIL * w >= 0, s, -1e9)
                    lg.append(s)
                m = lg[0]
                for w in range(1, BW):
                    m = jnp.maximum(m, lg[w])
                e = [jnp.exp(s - m) for s in lg]
                den = e[0]
                for w in range(1, BW):
                    den = den + e[w]
                inv = pl.reciprocal(den, approx=True)
                for c in range(NC):
                    o = e[0] * bkv_ref[l, 1, c, 16 + r * 8:16 + r * 8 + 8, :]
                    for w in range(1, BW):
                        o0 = 16 + r * 8 - BDIL * w
                        o = o + e[w] * bkv_ref[l, 1, c, o0:o0 + 8, :]
                    bo_ref[l * SEG + r * 8:l * SEG + r * 8 + 8, c * 128:(c + 1) * 128] = o * inv

    def b_phase2(t):
        w = pltpu.bitcast(pwo_ref[...], BF16)
        yb = xb_ref[...] + _nn(bo_ref[...].astype(BF16), w)
        if isinstance(t, int):
            row = max(t - 3, 0) * SEG
        else:
            row = pl.multiple_of(jnp.maximum(t - 3, 0) * SEG, SEG)
        out_ref[pl.ds(row, SEG), :] = yb[SEG:].astype(out_ref.dtype)
        return yb[:SEG]

    def x_seg(s):
        row = s * SEG if isinstance(s, int) else pl.multiple_of(s * SEG, SEG)
        return x_ref[pl.ds(row, SEG), :].astype(F32)

    def with_b(t):
        box = {}

        def hooks(p):
            if p == -1:
                b_phase1(t)
            elif p == BWO_PAIR:
                box['x2'] = b_phase2(t)
        return hooks, box

    zeros = jnp.zeros((SEG, D), F32)
    mem0 = mem0_ref[...].astype(F32)
    bkv_ref[...] = jnp.zeros(bkv_ref.shape, F32)

    x_first.wait()
    x0 = x_seg(0)
    h = _cat0(mem0, mem0, _ln(x0)).astype(BF16)
    acc = a_phase(h, attn_one_layer(0), permute_b, wait_w, weights_first)
    xb_ref[...] = _cat0(x0 + acc[2 * M:], zeros)
    x0 = x_seg(1)
    h = _cat0(acc[:M], mem0, _ln(x0)).astype(BF16)
    hooks, box = with_b(1)
    acc = a_phase(h, attn_one_layer(0), hooks)
    xb_ref[...] = _cat0(x0 + acc[2 * M:], zeros)
    xn = x_seg(2)
    h_ref[...] = _cat0(acc[:M], mem0, _ln(xn), _ln(box['x2'])).astype(BF16)
    res_ref[...] = _cat0(xn, box['x2'])
    x_rest.wait()

    def step(t, carry):
        hooks, box = with_b(t)
        acc = a_phase(h_ref[...], attn_two_layers(), hooks)
        xb_ref[...] = res_ref[...] + acc[2 * M:]
        xn = x_seg(jnp.minimum(t + 1, NSEG - 1))
        h_ref[...] = _cat0(acc[:2 * M], _ln(xn), _ln(box['x2'])).astype(BF16)
        res_ref[...] = _cat0(xn, box['x2'])
        return carry

    lax.fori_loop(2, NSEG, step, 0)

    def tail(t, carry):
        hooks, box = with_b(t)
        h = _cat0(h_ref[0:2 * M, :], h_ref[R1:, :])
        acc = a_phase(h, attn_one_layer(1), hooks)
        xb_ref[SEG:, :] = res_ref[SEG:, :] + acc[2 * M:]
        h_ref[0:2 * M, :] = acc[:2 * M].astype(BF16)
        h_ref[R1:, :] = _ln(box['x2']).astype(BF16)
        res_ref[SEG:, :] = box['x2']
        return carry

    tail(NSEG, 0)
    out_a.start()
    tail(NSEG + 1, 0)
    b_phase1(NSEG + 2)
    b_phase2(NSEG + 2)
    out_b.start()
    out_a.wait()
    out_b.wait()


@jax.jit
def pallas_interleave_layers__memory_aug_recurrent_mem_tr__sliding_local_dilated__prompt_kernel(
    A_x, A_mem0, A_Wq, A_Wk, A_Wv, A_Wo, A_seg_len, B_x, B_wqkv, B_wo,
):
    del A_seg_len, B_x
    wt = lambda w: jnp.transpose(w, (1, 2, 0)).reshape(HD, D)
    vm = pl.BlockSpec(memory_space=pltpu.VMEM)
    hbm = pl.BlockSpec(memory_space=pl.ANY)
    out = pl.pallas_call(
        _kernel,
        out_shape=jax.ShapeDtypeStruct((S, D), A_x.dtype),
        in_specs=[hbm, vm, hbm, hbm, hbm, hbm, hbm, hbm],
        out_specs=hbm,
        scratch_shapes=[
            pltpu.VMEM((S, D), BF16),
            pltpu.VMEM((S, D), BF16),
            pltpu.VMEM((4, HD, D), BF16),
            pltpu.VMEM((4, HD // 2, D), U32),
            pltpu.VMEM((D, 3 * D), BF16),
            pltpu.VMEM((D, D), BF16),
            pltpu.VMEM((D // 2, 3 * D), U32),
            pltpu.VMEM((D // 2, D), U32),
            pltpu.VMEM((R, D), BF16),
            pltpu.VMEM((2 * SEG, D), F32),
            pltpu.VMEM((2 * SEG, D), F32),
            pltpu.VMEM((NC, 2 * SEG, 128), F32),
            pltpu.VMEM((2, 2, NC, 16 + SEG, 128), F32),
            pltpu.VMEM((2 * SEG, D), F32),
            pltpu.SemaphoreType.DMA((NPAIR,)),
            pltpu.SemaphoreType.DMA((6,)),
        ],
        compiler_params=pltpu.CompilerParams(vmem_limit_bytes=110 * 2 ** 20),
    )(A_x.reshape(S, D), A_mem0.reshape(M, D), wt(A_Wq), wt(A_Wk), wt(A_Wv),
      A_Wo.reshape(HD, D), B_wqkv, B_wo)
    return out.reshape(1, S, D)
```

```python
import jax
import jax.numpy as jnp
from jax import lax
import jax.experimental.pallas as pl
import jax.experimental.pallas.tpu as pltpu

S, D = 2048, 640
H, DH = 32, 192
HD = H * DH
M, SEG = 8, 32
L = M + SEG
NSEG = S // SEG
R = 2 * L
R1 = 2 * M + SEG
PW = 2 * DH
NPAIR = H // 2
BDH, BW, BDIL = 20, 8, 2
NC = D // 128
XF = 4 * SEG
F32, BF16, U32 = jnp.float32, jnp.bfloat16, jnp.uint32
WIN = 2
NT = (((1,), (1,)), ((), ()))
PERM0, PSZ = 3, 64
HELD = 2
BWO_PAIR = 10


def _ln(x):
    m = jnp.mean(x, axis=-1, keepdims=True)
    xc = x - m
    v = jnp.mean(xc * xc, axis=-1, keepdims=True)
    return xc * lax.rsqrt(v + 1e-5)


def _nt(a, b):
    return lax.dot_general(a, b, NT, preferred_element_type=F32)


def _nn(a, b):
    return jnp.dot(a, b, preferred_element_type=F32)


def _cat0(*a):
    return jnp.concatenate(a, axis=0)


def _kernel(x_hbm, mem0_ref, wq_hbm, wk_hbm, wv_hbm, wo_hbm, bwqkv_hbm, bwo_hbm,
            out_hbm,
            x_ref, out_ref, wl_ref, w_ref, bwqkv_ref, bwo_ref, pwqkv_ref, pwo_ref,
            pm_ref, acc_ref, mem_ref, hx_ref, res_ref, xb_ref, bq_ref, bkv_ref, bo_ref, wsem, sem):
    def al(v, n):
        return v if isinstance(v, int) else pl.multiple_of(v, n)

    def w_copies(p):
        rows = pl.ds(al(p * PW, 128), PW)
        return [pltpu.make_async_copy(src.at[rows, :], wl_ref.at[m, rows, :], wsem.at[p])
                for m, src in enumerate((wq_hbm, wk_hbm, wv_hbm, wo_hbm))]

    x_first = pltpu.make_async_copy(x_hbm.at[pl.ds(0, XF), :], x_ref.at[pl.ds(0, XF), :], sem.at[0])
    x_rest = pltpu.make_async_copy(x_hbm.at[pl.ds(XF, S - XF), :], x_ref.at[pl.ds(XF, S - XF), :], sem.at[1])
    bw1 = pltpu.make_async_copy(bwqkv_hbm, bwqkv_ref, sem.at[2])
    bw2 = pltpu.make_async_copy(bwo_hbm, bwo_ref, sem.at[3])
    osplit = (NSEG - 2) * SEG
    out_a = pltpu.make_async_copy(out_ref.at[pl.ds(0, osplit), :], out_hbm.at[pl.ds(0, osplit), :], sem.at[4])
    out_b = pltpu.make_async_copy(out_ref.at[pl.ds(osplit, S - osplit), :],
                                  out_hbm.at[pl.ds(osplit, S - osplit), :], sem.at[5])
    def start_w(p):
        for cp in w_copies(p):
            cp.start()

    x_first.start()
    for p in range(WIN):
        start_w(p)

    def weights(m, p):
        return pltpu.bitcast(w_ref[m, pl.ds(p * PW // 2, PW // 2), :], BF16)

    scale = DH ** -0.5
    ninf = -jnp.inf

    def softmax2(s, first, allowed):
        s = jnp.where(allowed, s * scale, -1e9)
        m0 = jnp.max(jnp.where(first, s, ninf), axis=-1, keepdims=True)
        m1 = jnp.max(jnp.where(first, ninf, s), axis=-1, keepdims=True)
        e = jnp.exp(s - jnp.where(first, m0, m1))
        d0 = jnp.sum(jnp.where(first, e, 0.0), axis=-1, keepdims=True)
        d1 = jnp.sum(jnp.where(first, 0.0, e), axis=-1, keepdims=True)
        return e, pl.reciprocal(d0, approx=True), pl.reciprocal(d1, approx=True)

    def masks(rows):
        qi = lax.broadcasted_iota(jnp.int32, (rows, R), 0)
        ki = lax.broadcasted_iota(jnp.int32, (rows, R), 1)
        first = ki < L
        kk = jnp.where(first, ki, ki - L)
        qq = M + ((qi - 2 * M) & (SEG - 1))
        allowed = (qi < 2 * M) | (kk <= qq)
        return qi, first, allowed

    def attn_two_layers():
        qi, first, allowed = masks(R)
        row_l1 = (qi < M) | ((qi >= 2 * M) & (qi < R1))
        is_a = first == row_l1
        lo = lax.broadcasted_iota(jnp.int32, (L, 128), 1) < 64

        def arrange(a):
            a1 = _cat0(a[0:M], a[2 * M:R1])
            a2 = _cat0(a[M:2 * M], a[R1:])
            cat = lambda u, w: _cat0(u, w).astype(BF16)
            m1, m2 = a1[:, 128:256], a2[:, 128:256]
            return (cat(a1[:, :128], a2[:, :128]), cat(a2[:, 256:], a1[:, 256:]),
                    cat(jnp.where(lo, m1, 0.0), jnp.where(lo, 0.0, m1)),
                    cat(jnp.where(lo, 0.0, m2), jnp.where(lo, m2, 0.0)))

        g1 = lambda a: a[0:R1]
        g2 = lambda a: _cat0(a[0:2 * M], a[R1:])
        merge = lambda u1, u2: _cat0(u1[0:M], u2[M:2 * M], u1[2 * M:], u2[2 * M:])

        def scores(q, kt):
            qm = q[:, 128:256]
            return _nt(q[:, :128], kt[0]), _nt(q[:, 256:], kt[1]), _nt(g1(qm), kt[2]), _nt(g2(qm), kt[3])

        lo_r = lax.broadcasted_iota(jnp.int32, (R, 128), 1) < 64
        pick = lambda u1, u2: _cat0(u1[0:M], u2[M:2 * M], u1[2 * M:R1], u2[R1:])

        def pv(s4, vt):
            sa, sb, s1, s2 = s4
            p, r0, r1 = softmax2(jnp.where(is_a, sa, sb) + merge(s1, s2), first, allowed)
            pb = p.astype(BF16)
            oa = _nn(jnp.where(is_a, p, 0.0).astype(BF16), vt[0])
            ob = _nn(jnp.where(is_a, 0.0, p).astype(BF16), vt[1])
            om = merge(_nn(g1(pb), vt[2]), _nn(g2(pb), vt[3]))
            ra, rb = pick(r0, r1), pick(r1, r0)
            return jnp.concatenate(
                [oa * ra, om * jnp.where(lo_r, ra, rb), ob * rb], axis=1).astype(BF16)

        return arrange, scores, pv

    def attn_one_layer():
        _, first, allowed = masks(R1)
        head_a = lax.broadcasted_iota(jnp.int32, (L, PW), 1) < DH

        def arrange(a):
            a1 = _cat0(a[0:M], a[2 * M:])
            return _cat0(jnp.where(head_a, a1, 0.0), jnp.where(head_a, 0.0, a1)).astype(BF16)

        head_a1 = lax.broadcasted_iota(jnp.int32, (R1, PW), 1) < DH

        def pv(s, vt):
            p, r0, r1 = softmax2(s, first, allowed)
            return (_nn(p.astype(BF16), vt) * jnp.where(head_a1, r0, r1)).astype(BF16)

        return arrange, _nt, pv

    def a_phase(h, attn, hooks):
        arrange, scores, pv = attn
        proj = lambda m, p: _nt(h, weights(m, p))
        proj_o = lambda o, p: _nn(o, weights(3, p))
        q, kt = proj(0, 0).astype(BF16), arrange(proj(1, 0))
        hooks(-1)
        vt = arrange(proj(2, 0))
        acc = None
        held = {}
        for p in range(NPAIR):
            last = p == NPAIR - 1
            s = scores(q, kt)
            if not last:
                q, kt = proj(0, p + 1).astype(BF16), arrange(proj(1, p + 1))
            else:
                for pp in range(p - HELD, p - 1):
                    acc = acc + proj_o(held[pp], pp)
            hooks(p)
            o = pv(s, vt)
            if not last:
                vt = arrange(proj(2, p + 1))
            else:
                acc = acc + proj_o(held[p - 1], p - 1)
            if NPAIR - 1 - HELD <= p < NPAIR - 1:
                held[p] = o
            else:
                y = proj_o(o, p)
                acc = y if acc is None else acc + y
        return acc

    def b_phase1(t):
        w = pltpu.bitcast(pwqkv_ref[...], BF16)
        qkv = _nn(_ln(xb_ref[...]).astype(BF16), w)
        for l in range(2):
            for c in range(NC):
                bq_ref[c, l * SEG:(l + 1) * SEG, :] = qkv[l * SEG:(l + 1) * SEG, c * 128:(c + 1) * 128]
                for j in range(2):
                    bkv_ref[l, j, c, 0:16, :] = bkv_ref[l, j, c, SEG:SEG + 16, :]
                    bkv_ref[l, j, c, 16:16 + SEG, :] = qkv[
                        l * SEG:(l + 1) * SEG, (j + 1) * D + c * 128:(j + 1) * D + (c + 1) * 128]
        bscale = BDH ** -0.5
        ri8 = lax.broadcasted_iota(jnp.int32, (8, 128), 0)
        for l in range(2):
            seg = t - 1 - 2 * l
            for r in range(SEG // 8):
                pos = seg * SEG + r * 8 + ri8
                q = [bq_ref[c, l * SEG + r * 8:l * SEG + r * 8 + 8, :] for c in range(NC)]
                lg = []
                for w in range(BW):
                    o0 = 16 + r * 8 - BDIL * w
                    s = q[0] * bkv_ref[l, 0, 0, o0:o0 + 8, :]
                    for c in range(1, NC):
                        s = s + q[c] * bkv_ref[l, 0, c, o0:o0 + 8, :]
                    s = s + pltpu.roll(s, 64, 1)
                    s = s + pltpu.roll(s, 32, 1)
                    s = s * bscale
                    if r * 8 - BDIL * w < 0:
                        s = jnp.where(pos - BDIL * w >= 0, s, -1e9)
                    lg.append(s)
                m = lg[0]
                for w in range(1, BW):
                    m = jnp.maximum(m, lg[w])
                e = [jnp.exp(s - m) for s in lg]
                den = e[0]
                for w in range(1, BW):
                    den = den + e[w]
                inv = pl.reciprocal(den, approx=True)
                for c in range(NC):
                    o = e[0] * bkv_ref[l, 1, c, 16 + r * 8:16 + r * 8 + 8, :]
                    for w in range(1, BW):
                        o0 = 16 + r * 8 - BDIL * w
                        o = o + e[w] * bkv_ref[l, 1, c, o0:o0 + 8, :]
                    bo_ref[l * SEG + r * 8:l * SEG + r * 8 + 8, c * 128:(c + 1) * 128] = o * inv

    def b_phase2(t):
        w = pltpu.bitcast(pwo_ref[...], BF16)
        yb = xb_ref[...] + _nn(bo_ref[...].astype(BF16), w)
        if isinstance(t, int):
            row = max(t - 3, 0) * SEG
        else:
            row = pl.multiple_of(jnp.maximum(t - 3, 0) * SEG, SEG)
        out_ref[pl.ds(row, SEG), :] = yb[SEG:].astype(out_ref.dtype)
        return yb[:SEG]

    def x_seg(s):
        row = s * SEG if isinstance(s, int) else pl.multiple_of(s * SEG, SEG)
        return x_ref[pl.ds(row, SEG), :].astype(F32)

    def with_b(t):
        box = {}

        def hooks(p):
            if p == -1:
                b_phase1(t)
            elif p == BWO_PAIR:
                box['x2'] = b_phase2(t)
        return hooks, box

    def prepare_next(t, x2):
        xn = x_seg(jnp.minimum(t + 1, NSEG - 1))
        hx_ref[...] = _cat0(_ln(xn), _ln(x2)).astype(BF16)
        res_ref[...] = _cat0(xn, x2)

    ri = lax.broadcasted_iota(jnp.int32, (D, D), 0)
    ci = lax.broadcasted_iota(jnp.int32, (D, D), 1)
    pm_ref[...] = (ri == (ci & 31) * BDH + (ci >> 5)).astype(F32).astype(BF16)
    mem0 = mem0_ref[...].astype(F32)
    mem_ref[...] = _cat0(mem0, mem0)
    bkv_ref[...] = jnp.zeros(bkv_ref.shape, F32)
    acc_ref[...] = jnp.zeros(acc_ref.shape, F32)
    x_first.wait()
    hx_ref[0:SEG, :] = _ln(x_seg(0)).astype(BF16)

    def step0(p, carry):
        for cp in w_copies(p):
            cp.wait()

        @pl.when(p == 0)
        def _():
            bw2.start()
            bw1.start()

        @pl.when(p + WIN < NPAIR)
        def _():
            start_w(p + WIN)

        @pl.when(p == NPAIR - 1)
        def _():
            x_rest.start()

        def wfirst(m):
            w = wl_ref[m, pl.ds(al(p * PW, 128), PW), :]
            w_ref[m, pl.ds(al(p * (PW // 2), 64), PW // 2), :] = pltpu.bitcast(w, U32)
            return w

        arrange, scores, pv = attn_one_layer()
        h = _cat0(mem_ref[...].astype(BF16), hx_ref[0:SEG, :])
        q, kt, vt = _nt(h, wfirst(0)).astype(BF16), arrange(_nt(h, wfirst(1))), arrange(_nt(h, wfirst(2)))
        acc_ref[...] += _nn(pv(scores(q, kt), vt), wfirst(3))

        @pl.when(p == PERM0)
        def _():
            bw2.wait()
            bw1.wait()

        @pl.when((p >= PERM0) & (p < PERM0 + D // PSZ))
        def _():
            r0 = (p - PERM0) * PSZ
            rows = pl.ds(al(r0, PSZ), PSZ)
            prow = pl.ds(al((p - PERM0) * (PSZ // 2), PSZ // 2), PSZ // 2)
            w3 = _cat0(*[bwqkv_ref[rows, j * D:(j + 1) * D] for j in range(3)])
            y = _nn(w3, pm_ref[...]).astype(BF16)
            for j in range(3):
                pwqkv_ref[prow, j * D:(j + 1) * D] = pltpu.bitcast(y[j * PSZ:(j + 1) * PSZ], U32)
            rn = lax.broadcasted_iota(jnp.int32, (PSZ, D), 0) + r0
            co = lax.broadcasted_iota(jnp.int32, (PSZ, D), 1)
            pmt = (co == (rn & 31) * BDH + (rn >> 5)).astype(F32).astype(BF16)
            pwo_ref[prow, :] = pltpu.bitcast(_nn(pmt, bwo_ref[...]).astype(BF16), U32)

        return carry

    lax.fori_loop(0, NPAIR, step0, 0)
    zeros = jnp.zeros((SEG, D), F32)
    mem_ref[0:M, :] = acc_ref[0:M, :]
    xb_ref[...] = _cat0(x_seg(0) + acc_ref[2 * M:, :], zeros)
    prepare_next(0, zeros)

    def single(t, carry):
        @pl.when(t == NSEG + 1)
        def _():
            out_a.start()

        l = (t >= NSEG).astype(jnp.int32)
        mrows = pl.ds(al(l * M, M), M)
        xrows = pl.ds(al(l * SEG, SEG), SEG)
        hooks, box = with_b(t)
        mem = mem_ref[mrows, :]
        h = _cat0(_cat0(mem, mem).astype(BF16), hx_ref[xrows, :])
        acc = a_phase(h, attn_one_layer(), hooks)
        mem_ref[mrows, :] = acc[:M]
        xb_ref[xrows, :] = res_ref[xrows, :] + acc[2 * M:]
        prepare_next(t, box['x2'])
        return carry

    def step(t, carry):
        hooks, box = with_b(t)
        h = _cat0(mem_ref[...].astype(BF16), hx_ref[...])
        acc = a_phase(h, attn_two_layers(), hooks)
        mem_ref[...] = acc[:2 * M]
        xb_ref[...] = res_ref[...] + acc[2 * M:]
        prepare_next(t, box['x2'])
        return carry

    def outer(i, carry):
        lax.fori_loop(1 + (NSEG - 1) * i, 2 + NSEG * i, single, 0)

        @pl.when(i == 0)
        def _():
            x_rest.wait()

        lax.fori_loop(2, NSEG - (NSEG - 2) * i, step, 0)
        return carry

    lax.fori_loop(0, 2, outer, 0)
    b_phase1(NSEG + 2)
    b_phase2(NSEG + 2)
    out_b.start()
    out_a.wait()
    out_b.wait()


@jax.jit
def pallas_interleave_layers__memory_aug_recurrent_mem_tr__sliding_local_dilated__prompt_kernel(
    A_x, A_mem0, A_Wq, A_Wk, A_Wv, A_Wo, A_seg_len, B_x, B_wqkv, B_wo,
):
    del A_seg_len, B_x
    wt = lambda w: jnp.transpose(w, (1, 2, 0)).reshape(HD, D)
    vm = pl.BlockSpec(memory_space=pltpu.VMEM)
    hbm = pl.BlockSpec(memory_space=pl.ANY)
    out = pl.pallas_call(
        _kernel,
        out_shape=jax.ShapeDtypeStruct((S, D), A_x.dtype),
        in_specs=[hbm, vm, hbm, hbm, hbm, hbm, hbm, hbm],
        out_specs=hbm,
        scratch_shapes=[
            pltpu.VMEM((S, D), BF16),
            pltpu.VMEM((S, D), BF16),
            pltpu.VMEM((4, HD, D), BF16),
            pltpu.VMEM((4, HD // 2, D), U32),
            pltpu.VMEM((D, 3 * D), BF16),
            pltpu.VMEM((D, D), BF16),
            pltpu.VMEM((D // 2, 3 * D), U32),
            pltpu.VMEM((D // 2, D), U32),
            pltpu.VMEM((D, D), BF16),
            pltpu.VMEM((R1, D), F32),
            pltpu.VMEM((2 * M, D), F32),
            pltpu.VMEM((2 * SEG, D), BF16),
            pltpu.VMEM((2 * SEG, D), F32),
            pltpu.VMEM((2 * SEG, D), F32),
            pltpu.VMEM((NC, 2 * SEG, 128), F32),
            pltpu.VMEM((2, 2, NC, 16 + SEG, 128), F32),
            pltpu.VMEM((2 * SEG, D), F32),
            pltpu.SemaphoreType.DMA((NPAIR,)),
            pltpu.SemaphoreType.DMA((6,)),
        ],
        compiler_params=pltpu.CompilerParams(vmem_limit_bytes=110 * 2 ** 20),
    )(A_x.reshape(S, D), A_mem0.reshape(M, D), wt(A_Wq), wt(A_Wk), wt(A_Wv),
      A_Wo.reshape(HD, D), B_wqkv, B_wo)
    return out.reshape(1, S, D)
```

```python
import jax
import jax.numpy as jnp
from jax import lax
import jax.experimental.pallas as pl
import jax.experimental.pallas.tpu as pltpu

S, D = 2048, 640
H, DH = 32, 192
HD = H * DH
M, SEG = 8, 32
L = M + SEG
NSEG = S // SEG
R = 2 * L
R1 = 2 * M + SEG
PW = 2 * DH
NPAIR = H // 2
BDH, BW, BDIL = 20, 8, 2
NC = D // 128
XF = 4 * SEG
F32, BF16, U32 = jnp.float32, jnp.bfloat16, jnp.uint32
WIN = 2
NT = (((1,), (1,)), ((), ()))
PERM0, PSZ = 3, 64
SERIAL = 0
HELD = 2
BWO_PAIR = 10


def _ln(x):
    m = jnp.mean(x, axis=-1, keepdims=True)
    xc = x - m
    v = jnp.mean(xc * xc, axis=-1, keepdims=True)
    return xc * lax.rsqrt(v + 1e-5)


def _nt(a, b):
    return lax.dot_general(a, b, NT, preferred_element_type=F32)


def _nn(a, b):
    return jnp.dot(a, b, preferred_element_type=F32)


def _cat0(*a):
    return jnp.concatenate(a, axis=0)


def _kernel(x_hbm, mem0_ref, wq_hbm, wk_hbm, wv_hbm, wo_hbm, bwqkv_hbm, bwo_hbm,
            out_hbm,
            x_ref, out_ref, wl_ref, w_ref, bwqkv_ref, bwo_ref, pwqkv_ref, pwo_ref,
            pm_ref, acc_ref, mem_ref, hx_ref, res_ref, xb_ref, bq_ref, bkv_ref, zero_ref, wsem, sem):
    def al(v, n):
        return v if isinstance(v, int) else pl.multiple_of(v, n)

    def w_copies(p):
        rows = pl.ds(al(p * PW, 128), PW)
        return [pltpu.make_async_copy(src.at[rows, :], wl_ref.at[m, rows, :], wsem.at[p])
                for m, src in enumerate((wq_hbm, wk_hbm, wv_hbm, wo_hbm))]

    x_first = pltpu.make_async_copy(x_hbm.at[pl.ds(0, XF), :], x_ref.at[pl.ds(0, XF), :], sem.at[0])
    x_rest = pltpu.make_async_copy(x_hbm.at[pl.ds(XF, S - XF), :], x_ref.at[pl.ds(XF, S - XF), :], sem.at[1])
    bw1 = pltpu.make_async_copy(bwqkv_hbm, bwqkv_ref, sem.at[2])
    bw2 = pltpu.make_async_copy(bwo_hbm, bwo_ref, sem.at[3])
    osplit = (NSEG - 2) * SEG
    out_a = pltpu.make_async_copy(out_ref.at[pl.ds(0, osplit), :], out_hbm.at[pl.ds(0, osplit), :], sem.at[4])
    out_b = pltpu.make_async_copy(out_ref.at[pl.ds(osplit, S - osplit), :],
                                  out_hbm.at[pl.ds(osplit, S - osplit), :], sem.at[5])
    def start_w(p):
        for cp in w_copies(p):
            cp.start()

    x_first.start()
    for p in range(WIN):
        start_w(p)

    def weights(m, p):
        return pltpu.bitcast(w_ref[m, pl.ds(p * PW // 2, PW // 2), :], BF16)

    scale = DH ** -0.5
    ninf = -jnp.inf

    def softmax2(s, first, allowed):
        s = jnp.where(allowed, s * scale, -1e9)
        m0 = jnp.max(jnp.where(first, s, ninf), axis=-1, keepdims=True)
        m1 = jnp.max(jnp.where(first, ninf, s), axis=-1, keepdims=True)
        e = jnp.exp(s - jnp.where(first, m0, m1))
        d0 = jnp.sum(jnp.where(first, e, 0.0), axis=-1, keepdims=True)
        d1 = jnp.sum(jnp.where(first, 0.0, e), axis=-1, keepdims=True)
        return e, pl.reciprocal(d0, approx=True), pl.reciprocal(d1, approx=True)

    def masks(rows):
        qi = lax.broadcasted_iota(jnp.int32, (rows, R), 0)
        ki = lax.broadcasted_iota(jnp.int32, (rows, R), 1)
        first = ki < L
        kk = jnp.where(first, ki, ki - L)
        qq = M + ((qi - 2 * M) & (SEG - 1))
        allowed = (qi < 2 * M) | (kk <= qq)
        return qi, first, allowed

    def attn_two_layers():
        qi, first, allowed = masks(R)
        row_l1 = (qi < M) | ((qi >= 2 * M) & (qi < R1))
        is_a = first == row_l1
        lo = lax.broadcasted_iota(jnp.int32, (L, 128), 1) < 64

        def arrange(a):
            a1 = _cat0(a[0:M], a[2 * M:R1])
            a2 = _cat0(a[M:2 * M], a[R1:])
            cat = lambda u, w: _cat0(u, w).astype(BF16)
            m1, m2 = a1[:, 128:256], a2[:, 128:256]
            return (cat(a1[:, :128], a2[:, :128]), cat(a2[:, 256:], a1[:, 256:]),
                    cat(jnp.where(lo, m1, 0.0), jnp.where(lo, 0.0, m1)),
                    cat(jnp.where(lo, 0.0, m2), jnp.where(lo, m2, 0.0)))

        g1 = lambda a: a[0:R1]
        g2 = lambda a: _cat0(a[0:2 * M], a[R1:])
        merge = lambda u1, u2: _cat0(u1[0:M], u2[M:2 * M], u1[2 * M:], u2[2 * M:])

        def scores(q, kt):
            qm = q[:, 128:256]
            return _nt(q[:, :128], kt[0]), _nt(q[:, 256:], kt[1]), _nt(g1(qm), kt[2]), _nt(g2(qm), kt[3])

        lo_r = lax.broadcasted_iota(jnp.int32, (R, 128), 1) < 64
        pick = lambda u1, u2: _cat0(u1[0:M], u2[M:2 * M], u1[2 * M:R1], u2[R1:])

        def pv(s4, vt):
            sa, sb, s1, s2 = s4
            p, r0, r1 = softmax2(jnp.where(is_a, sa, sb) + merge(s1, s2), first, allowed)
            pb = p.astype(BF16)
            oa = _nn(jnp.where(is_a, p, 0.0).astype(BF16), vt[0])
            ob = _nn(jnp.where(is_a, 0.0, p).astype(BF16), vt[1])
            om = merge(_nn(g1(pb), vt[2]), _nn(g2(pb), vt[3]))
            r0, r1 = jnp.broadcast_to(r0, (R, 128)), jnp.broadcast_to(r1, (R, 128))
            ra, rb = pick(r0, r1), pick(r1, r0)
            return jnp.concatenate(
                [oa * ra, om * jnp.where(lo_r, ra, rb), ob * rb], axis=1).astype(BF16)

        return arrange, scores, pv

    def attn_one_layer():
        _, first, allowed = masks(R1)
        head_a = lax.broadcasted_iota(jnp.int32, (L, PW), 1) < DH

        def arrange(a):
            a1 = _cat0(a[0:M], a[2 * M:])
            return _cat0(jnp.where(head_a, a1, 0.0), jnp.where(head_a, 0.0, a1)).astype(BF16)

        head_a1 = lax.broadcasted_iota(jnp.int32, (R1, PW), 1) < DH

        def pv(s, vt):
            p, r0, r1 = softmax2(s, first, allowed)
            return (_nn(p.astype(BF16), vt) * jnp.where(head_a1, r0, r1)).astype(BF16)

        return arrange, _nt, pv

    def a_phase(h, attn, hooks):
        arrange, scores, pv = attn
        proj = lambda m, p: _nt(h, weights(m, p))
        proj_o = lambda o, p: _nn(o, weights(3, p))
        q, kt = proj(0, 0).astype(BF16), arrange(proj(1, 0))
        hooks(-1)
        vt = arrange(proj(2, 0))
        acc = None
        held = {}
        for p in range(NPAIR):
            last = p == NPAIR - 1
            s = scores(q, kt)
            if not last:
                q, kt = proj(0, p + 1).astype(BF16), arrange(proj(1, p + 1))
            else:
                for pp in range(p - HELD, p - 1):
                    acc = acc + proj_o(held[pp], pp)
            hooks(p)
            o = pv(s, vt)
            if not last:
                vt = arrange(proj(2, p + 1))
            else:
                acc = acc + proj_o(held[p - 1], p - 1)
            if NPAIR - 1 - HELD <= p < NPAIR - 1:
                held[p] = o
            else:
                y = proj_o(o, p)
                acc = y if acc is None else acc + y
        return acc

    def b_phase1(t):
        w = pltpu.bitcast(pwqkv_ref[...], BF16)
        qkv = _nn(_ln(xb_ref[...]).astype(BF16), w)
        for l in range(2):
            for c in range(NC):
                bq_ref[c, l * SEG:(l + 1) * SEG, :] = qkv[l * SEG:(l + 1) * SEG, c * 128:(c + 1) * 128]
                for j in range(2):
                    bkv_ref[l, j, c, 0:16, :] = bkv_ref[l, j, c, SEG:SEG + 16, :]
                    bkv_ref[l, j, c, 16:16 + SEG, :] = qkv[
                        l * SEG:(l + 1) * SEG, (j + 1) * D + c * 128:(j + 1) * D + (c + 1) * 128]
        bscale = BDH ** -0.5
        ri8 = lax.broadcasted_iota(jnp.int32, (8, 128), 0)
        for l in range(2):
            seg = t - 1 - 2 * l
            for r in range(SEG // 8):
                pos = seg * SEG + r * 8 + ri8
                q = [bq_ref[c, l * SEG + r * 8:l * SEG + r * 8 + 8, :] for c in range(NC)]
                lg = []
                for w in range(BW):
                    o0 = 16 + r * 8 - BDIL * w
                    s = q[0] * bkv_ref[l, 0, 0, o0:o0 + 8, :]
                    for c in range(1, NC):
                        s = s + q[c] * bkv_ref[l, 0, c, o0:o0 + 8, :]
                    s = s + pltpu.roll(s, 64, 1)
                    s = s + pltpu.roll(s, 32, 1)
                    s = s * bscale
                    if r * 8 - BDIL * w < 0:
                        s = jnp.where(pos - BDIL * w >= 0, s, -1e9)
                    lg.append(s)
                m = lg[0]
                for w in range(1, BW):
                    m = jnp.maximum(m, lg[w])
                e = [jnp.exp(s - m) for s in lg]
                den = e[0]
                for w in range(1, BW):
                    den = den + e[w]
                inv = pl.reciprocal(den, approx=True)
                for c in range(NC):
                    o = e[0] * bkv_ref[l, 1, c, 16 + r * 8:16 + r * 8 + 8, :]
                    for w in range(1, BW):
                        o0 = 16 + r * 8 - BDIL * w
                        o = o + e[w] * bkv_ref[l, 1, c, o0:o0 + 8, :]
                    orow = pl.multiple_of(zero_ref[0] + (l * SEG + r * 8), 8) if SERIAL else l * SEG + r * 8
                    bq_ref[c, pl.ds(orow, 8), :] = o * inv

    def b_phase2(t):
        w = pltpu.bitcast(pwo_ref[...], BF16)
        yb = xb_ref[...] + _nn(jnp.concatenate([bq_ref[c] for c in range(NC)], axis=1).astype(BF16), w)
        if isinstance(t, int):
            row = max(t - 3, 0) * SEG
        else:
            row = pl.multiple_of(jnp.maximum(t - 3, 0) * SEG, SEG)
        out_ref[pl.ds(row, SEG), :] = yb[SEG:].astype(out_ref.dtype)
        return yb[:SEG]

    def x_seg(s):
        row = s * SEG if isinstance(s, int) else pl.multiple_of(s * SEG, SEG)
        return x_ref[pl.ds(row, SEG), :].astype(F32)

    def with_b(t):
        box = {}

        def hooks(p):
            if p == -1:
                b_phase1(t)
            elif p == BWO_PAIR:
                box['x2'] = b_phase2(t)
        return hooks, box

    def prepare_next(t, x2):
        xn = x_seg(jnp.minimum(t + 1, NSEG - 1))
        hx_ref[...] = _cat0(_ln(xn), _ln(x2)).astype(BF16)
        res_ref[...] = _cat0(xn, x2)

    ri = lax.broadcasted_iota(jnp.int32, (D, D), 0)
    ci = lax.broadcasted_iota(jnp.int32, (D, D), 1)
    pm_ref[...] = (ri == (ci & 31) * BDH + (ci >> 5)).astype(F32).astype(BF16)
    mem0 = mem0_ref[...].astype(F32)
    mem_ref[...] = _cat0(mem0, mem0)
    bkv_ref[...] = jnp.zeros(bkv_ref.shape, F32)
    acc_ref[...] = jnp.zeros(acc_ref.shape, F32)
    zero_ref[0] = 0
    x_first.wait()
    hx_ref[0:SEG, :] = _ln(x_seg(0)).astype(BF16)

    def step0(p, carry):
        for cp in w_copies(p):
            cp.wait()

        @pl.when(p == 0)
        def _():
            bw2.start()
            bw1.start()

        @pl.when(p + WIN < NPAIR)
        def _():
            start_w(p + WIN)

        @pl.when(p == NPAIR - 1)
        def _():
            x_rest.start()

        def wfirst(m):
            w = wl_ref[m, pl.ds(al(p * PW, 128), PW), :]
            w_ref[m, pl.ds(al(p * (PW // 2), 64), PW // 2), :] = pltpu.bitcast(w, U32)
            return w

        arrange, scores, pv = attn_one_layer()
        h = _cat0(mem_ref[...].astype(BF16), hx_ref[0:SEG, :])
        q, kt, vt = _nt(h, wfirst(0)).astype(BF16), arrange(_nt(h, wfirst(1))), arrange(_nt(h, wfirst(2)))
        acc_ref[...] += _nn(pv(scores(q, kt), vt), wfirst(3))

        @pl.when(p == PERM0)
        def _():
            bw2.wait()
            bw1.wait()

        @pl.when((p >= PERM0) & (p < PERM0 + D // PSZ))
        def _():
            r0 = (p - PERM0) * PSZ
            rows = pl.ds(al(r0, PSZ), PSZ)
            prow = pl.ds(al((p - PERM0) * (PSZ // 2), PSZ // 2), PSZ // 2)
            w3 = _cat0(*[bwqkv_ref[rows, j * D:(j + 1) * D] for j in range(3)])
            y = _nn(w3, pm_ref[...]).astype(BF16)
            for j in range(3):
                pwqkv_ref[prow, j * D:(j + 1) * D] = pltpu.bitcast(y[j * PSZ:(j + 1) * PSZ], U32)
            rn = lax.broadcasted_iota(jnp.int32, (PSZ, D), 0) + r0
            co = lax.broadcasted_iota(jnp.int32, (PSZ, D), 1)
            pmt = (co == (rn & 31) * BDH + (rn >> 5)).astype(F32).astype(BF16)
            pwo_ref[prow, :] = pltpu.bitcast(_nn(pmt, bwo_ref[...]).astype(BF16), U32)

        return carry

    lax.fori_loop(0, NPAIR, step0, 0)
    zeros = jnp.zeros((SEG, D), F32)
    mem_ref[0:M, :] = acc_ref[0:M, :]
    xb_ref[...] = _cat0(x_seg(0) + acc_ref[2 * M:, :], zeros)
    prepare_next(0, zeros)

    def single(t, carry):
        @pl.when(t == NSEG + 1)
        def _():
            out_a.start()

        l = (t >= NSEG).astype(jnp.int32)
        mrows = pl.ds(al(l * M, M), M)
        xrows = pl.ds(al(l * SEG, SEG), SEG)
        hooks, box = with_b(t)
        mem = mem_ref[mrows, :]
        h = _cat0(_cat0(mem, mem).astype(BF16), hx_ref[xrows, :])
        acc = a_phase(h, attn_one_layer(), hooks)
        mem_ref[mrows, :] = acc[:M]
        xb_ref[xrows, :] = res_ref[xrows, :] + acc[2 * M:]
        prepare_next(t, box['x2'])
        return carry

    def step(t, carry):
        hooks, box = with_b(t)
        h = _cat0(mem_ref[...].astype(BF16), hx_ref[...])
        acc = a_phase(h, attn_two_layers(), hooks)
        mem_ref[...] = acc[:2 * M]
        xb_ref[...] = res_ref[...] + acc[2 * M:]
        prepare_next(t, box['x2'])
        return carry

    def outer(i, carry):
        lax.fori_loop(1 + (NSEG - 1) * i, 2 + NSEG * i, single, 0)

        @pl.when(i == 0)
        def _():
            x_rest.wait()

        lax.fori_loop(2, NSEG - (NSEG - 2) * i, step, 0)
        return carry

    lax.fori_loop(0, 2, outer, 0)
    b_phase1(NSEG + 2)
    b_phase2(NSEG + 2)
    out_b.start()
    out_a.wait()
    out_b.wait()


@jax.jit
def pallas_interleave_layers__memory_aug_recurrent_mem_tr__sliding_local_dilated__prompt_kernel(
    A_x, A_mem0, A_Wq, A_Wk, A_Wv, A_Wo, A_seg_len, B_x, B_wqkv, B_wo,
):
    del A_seg_len, B_x
    wt = lambda w: jnp.transpose(w, (1, 2, 0)).reshape(HD, D)
    vm = pl.BlockSpec(memory_space=pltpu.VMEM)
    hbm = pl.BlockSpec(memory_space=pl.ANY)
    out = pl.pallas_call(
        _kernel,
        out_shape=jax.ShapeDtypeStruct((S, D), A_x.dtype),
        in_specs=[hbm, vm, hbm, hbm, hbm, hbm, hbm, hbm],
        out_specs=hbm,
        scratch_shapes=[
            pltpu.VMEM((S, D), BF16),
            pltpu.VMEM((S, D), BF16),
            pltpu.VMEM((4, HD, D), BF16),
            pltpu.VMEM((4, HD // 2, D), U32),
            pltpu.VMEM((D, 3 * D), BF16),
            pltpu.VMEM((D, D), BF16),
            pltpu.VMEM((D // 2, 3 * D), U32),
            pltpu.VMEM((D // 2, D), U32),
            pltpu.VMEM((D, D), BF16),
            pltpu.VMEM((R1, D), F32),
            pltpu.VMEM((2 * M, D), F32),
            pltpu.VMEM((2 * SEG, D), BF16),
            pltpu.VMEM((2 * SEG, D), F32),
            pltpu.VMEM((2 * SEG, D), F32),
            pltpu.VMEM((NC, 2 * SEG, 128), F32),
            pltpu.VMEM((2, 2, NC, 16 + SEG, 128), F32),
            pltpu.SMEM((1,), jnp.int32),
            pltpu.SemaphoreType.DMA((NPAIR,)),
            pltpu.SemaphoreType.DMA((6,)),
        ],
        compiler_params=pltpu.CompilerParams(vmem_limit_bytes=110 * 2 ** 20),
    )(A_x.reshape(S, D), A_mem0.reshape(M, D), wt(A_Wq), wt(A_Wk), wt(A_Wv),
      A_Wo.reshape(HD, D), B_wqkv, B_wo)
    return out.reshape(1, S, D)
```

```python
import jax
import jax.numpy as jnp
from jax import lax
import jax.experimental.pallas as pl
import jax.experimental.pallas.tpu as pltpu

S, D = 2048, 640
H, DH = 32, 192
HD = H * DH
M, SEG = 8, 32
L = M + SEG
NSEG = S // SEG
R = 2 * L
R1 = 2 * M + SEG
PW = 2 * DH
NPAIR = H // 2
BDH, BW, BDIL = 20, 8, 2
NC = D // 128
XB = S // NPAIR
NPRE = 2
BQKV_AT = 0
F32, BF16, U32 = jnp.float32, jnp.bfloat16, jnp.uint32
WIN = 3
NT = (((1,), (1,)), ((), ()))
PERM0, PSZ = 3, 64
HELD = 2
BWO_PAIR = 10


def _ln(x):
    m = jnp.mean(x, axis=-1, keepdims=True)
    xc = x - m
    v = jnp.mean(xc * xc, axis=-1, keepdims=True)
    return xc * lax.rsqrt(v + 1e-5)


def _nt(a, b):
    return lax.dot_general(a, b, NT, preferred_element_type=F32)


def _nn(a, b):
    return jnp.dot(a, b, preferred_element_type=F32)


def _cat0(*a):
    return jnp.concatenate(a, axis=0)


def _kernel(x_hbm, mem0_ref, wq_hbm, wk_hbm, wv_hbm, wo_hbm, bwqkv_hbm, bwo_hbm,
            out_hbm,
            x_ref, out_ref, wl_ref, w_ref, bwqkv_ref, bwo_ref, pwqkv_ref, pwo_ref,
            pm_ref, acc_ref, mem_ref, hx_ref, res_ref, xb_ref, bq_ref, bkv_ref, wn_ref, hxa_ref, pre_ref, wsem, sem):
    def al(v, n):
        return v if isinstance(v, int) else pl.multiple_of(v, n)

    def w_copies(p):
        rows = pl.ds(al(p * PW, 128), PW)
        xrows = pl.ds(al(p * XB, XB), XB)
        return [pltpu.make_async_copy(x_hbm.at[xrows, :], x_ref.at[xrows, :], wsem.at[p])] + [
            pltpu.make_async_copy(src.at[rows, :], wl_ref.at[m, rows, :], wsem.at[p])
            for m, src in enumerate((wq_hbm, wk_hbm, wv_hbm, wo_hbm))]

    bw1 = pltpu.make_async_copy(bwqkv_hbm, bwqkv_ref, sem.at[2])
    bw2 = pltpu.make_async_copy(bwo_hbm, bwo_ref, sem.at[3])
    osplit = (NSEG - 2) * SEG
    out_a = pltpu.make_async_copy(out_ref.at[pl.ds(0, osplit), :], out_hbm.at[pl.ds(0, osplit), :], sem.at[4])
    out_b = pltpu.make_async_copy(out_ref.at[pl.ds(osplit, S - osplit), :],
                                  out_hbm.at[pl.ds(osplit, S - osplit), :], sem.at[5])
    def start_w(p):
        for cp in w_copies(p):
            cp.start()

    def wait_w(p):
        for cp in w_copies(p):
            cp.wait()

    for p in range(WIN):
        start_w(p)

    def weights(m, p):
        return pltpu.bitcast(w_ref[m, pl.ds(p * PW // 2, PW // 2), :], BF16)

    def weights_nn(c0, c1):
        return pltpu.bitcast(wn_ref[:, c0 * PW:c1 * PW], BF16)

    scale = DH ** -0.5
    ninf = -jnp.inf

    def softmax2(s, first, allowed):
        s = jnp.where(allowed, s * scale, -1e9)
        m0 = jnp.max(jnp.where(first, s, ninf), axis=-1, keepdims=True)
        m1 = jnp.max(jnp.where(first, ninf, s), axis=-1, keepdims=True)
        e = jnp.exp(s - jnp.where(first, m0, m1))
        d0 = jnp.sum(jnp.where(first, e, 0.0), axis=-1, keepdims=True)
        d1 = jnp.sum(jnp.where(first, 0.0, e), axis=-1, keepdims=True)
        return e, pl.reciprocal(d0, approx=True), pl.reciprocal(d1, approx=True)

    def masks(rows):
        qi = lax.broadcasted_iota(jnp.int32, (rows, R), 0)
        ki = lax.broadcasted_iota(jnp.int32, (rows, R), 1)
        first = ki < L
        kk = jnp.where(first, ki, ki - L)
        qq = M + ((qi - 2 * M) & (SEG - 1))
        allowed = (qi < 2 * M) | (kk <= qq)
        return qi, first, allowed

    def attn_two_layers():
        qi, first, allowed = masks(R)
        row_l1 = (qi < M) | ((qi >= 2 * M) & (qi < R1))
        is_a = first == row_l1
        lo = lax.broadcasted_iota(jnp.int32, (L, 128), 1) < 64

        def arrange(a):
            a1 = _cat0(a[0:M], a[2 * M:R1])
            a2 = _cat0(a[M:2 * M], a[R1:])
            cat = lambda u, w: _cat0(u, w).astype(BF16)
            m1, m2 = a1[:, 128:256], a2[:, 128:256]
            return (cat(a1[:, :128], a2[:, :128]), cat(a2[:, 256:], a1[:, 256:]),
                    cat(jnp.where(lo, m1, 0.0), jnp.where(lo, 0.0, m1)),
                    cat(jnp.where(lo, 0.0, m2), jnp.where(lo, m2, 0.0)))

        g1 = lambda a: a[0:R1]
        g2 = lambda a: _cat0(a[0:2 * M], a[R1:])
        merge = lambda u1, u2: _cat0(u1[0:M], u2[M:2 * M], u1[2 * M:], u2[2 * M:])

        def scores(q, kt):
            qm = q[:, 128:256]
            return _nt(q[:, :128], kt[0]), _nt(q[:, 256:], kt[1]), _nt(g1(qm), kt[2]), _nt(g2(qm), kt[3])

        lo_r = lax.broadcasted_iota(jnp.int32, (R, 128), 1) < 64
        pick = lambda u1, u2: _cat0(u1[0:M], u2[M:2 * M], u1[2 * M:R1], u2[R1:])

        def pv(s4, vt):
            sa, sb, s1, s2 = s4
            p, r0, r1 = softmax2(jnp.where(is_a, sa, sb) + merge(s1, s2), first, allowed)
            pb = p.astype(BF16)
            oa = _nn(jnp.where(is_a, p, 0.0).astype(BF16), vt[0])
            ob = _nn(jnp.where(is_a, 0.0, p).astype(BF16), vt[1])
            om = merge(_nn(g1(pb), vt[2]), _nn(g2(pb), vt[3]))
            r0, r1 = jnp.broadcast_to(r0, (R, 128)), jnp.broadcast_to(r1, (R, 128))
            ra, rb = pick(r0, r1), pick(r1, r0)
            return jnp.concatenate(
                [oa * ra, om * jnp.where(lo_r, ra, rb), ob * rb], axis=1).astype(BF16)

        return arrange, scores, pv

    def attn_one_layer():
        _, first, allowed = masks(R1)
        head_a = lax.broadcasted_iota(jnp.int32, (L, PW), 1) < DH

        def arrange(a):
            a1 = _cat0(a[0:M], a[2 * M:])
            return _cat0(jnp.where(head_a, a1, 0.0), jnp.where(head_a, 0.0, a1)).astype(BF16)

        head_a1 = lax.broadcasted_iota(jnp.int32, (R1, PW), 1) < DH

        def pv(s, vt):
            p, r0, r1 = softmax2(s, first, allowed)
            return (_nn(p.astype(BF16), vt) * jnp.where(head_a1, r0, r1)).astype(BF16)

        return arrange, _nt, pv

    def a_phase(h, attn, hooks, t=None):
        arrange, scores, pv = attn

        def proj(m, p):
            dt = BF16 if m == 0 else F32
            if p >= NPRE:
                return _nt(h, weights(m, p)).astype(dt)
            c = p * 3 + m
            if t is None:
                return _nn(h, weights_nn(c, c + 1)).astype(dt)
            y = _nn(_cat0(h[0:2 * M], h[R1:]), weights_nn(c, c + 1)).astype(dt)
            pre = pre_ref[pl.ds(al(t * SEG, SEG), SEG), c * PW:(c + 1) * PW].astype(dt)
            return _cat0(y[0:2 * M], pre, y[2 * M:])

        proj_o = lambda o, p: _nn(o, weights(3, p))
        q, kt = proj(0, 0), arrange(proj(1, 0))
        hooks(-1)
        vt = arrange(proj(2, 0))
        acc = None
        held = {}
        for p in range(NPAIR):
            last = p == NPAIR - 1
            s = scores(q, kt)
            hooks(p - 0.5)
            if not last:
                q, kt = proj(0, p + 1), arrange(proj(1, p + 1))
            else:
                for pp in range(p - HELD, p - 1):
                    acc = acc + proj_o(held[pp], pp)
            hooks(p)
            o = pv(s, vt)
            if not last:
                vt = arrange(proj(2, p + 1))
            else:
                acc = acc + proj_o(held[p - 1], p - 1)
            if NPAIR - 1 - HELD <= p < NPAIR - 1:
                held[p] = o
            else:
                y = proj_o(o, p)
                acc = y if acc is None else acc + y
        return acc

    def b_phase1(t):
        w = pltpu.bitcast(pwqkv_ref[...], BF16)
        qkv = _nn(_ln(xb_ref[...]).astype(BF16), w)
        for l in range(2):
            for c in range(NC):
                bq_ref[c, l * SEG:(l + 1) * SEG, :] = qkv[l * SEG:(l + 1) * SEG, c * 128:(c + 1) * 128]
                for j in range(2):
                    bkv_ref[l, j, c, 0:16, :] = bkv_ref[l, j, c, SEG:SEG + 16, :]
                    bkv_ref[l, j, c, 16:16 + SEG, :] = qkv[
                        l * SEG:(l + 1) * SEG, (j + 1) * D + c * 128:(j + 1) * D + (c + 1) * 128]
        bscale = BDH ** -0.5
        ri8 = lax.broadcasted_iota(jnp.int32, (8, 128), 0)
        for l in range(2):
            seg = t - 1 - 2 * l
            for r in range(SEG // 8):
                pos = seg * SEG + r * 8 + ri8
                q = [bq_ref[c, l * SEG + r * 8:l * SEG + r * 8 + 8, :] for c in range(NC)]
                lg = []
                for w in range(BW):
                    o0 = 16 + r * 8 - BDIL * w
                    s = q[0] * bkv_ref[l, 0, 0, o0:o0 + 8, :]
                    for c in range(1, NC):
                        s = s + q[c] * bkv_ref[l, 0, c, o0:o0 + 8, :]
                    s = s + pltpu.roll(s, 64, 1)
                    s = s + pltpu.roll(s, 32, 1)
                    s = s * bscale
                    if r * 8 - BDIL * w < 0:
                        s = jnp.where(pos - BDIL * w >= 0, s, -1e9)
                    lg.append(s)
                m = lg[0]
                for w in range(1, BW):
                    m = jnp.maximum(m, lg[w])
                e = [jnp.exp(s - m) for s in lg]
                den = e[0]
                for w in range(1, BW):
                    den = den + e[w]
                inv = pl.reciprocal(den, approx=True)
                for c in range(NC):
                    o = e[0] * bkv_ref[l, 1, c, 16 + r * 8:16 + r * 8 + 8, :]
                    for w in range(1, BW):
                        o0 = 16 + r * 8 - BDIL * w
                        o = o + e[w] * bkv_ref[l, 1, c, o0:o0 + 8, :]
                    bq_ref[c, l * SEG + r * 8:l * SEG + r * 8 + 8, :] = o * inv

    def b_phase2(t):
        w = pltpu.bitcast(pwo_ref[...], BF16)
        yb = xb_ref[...] + _nn(jnp.concatenate([bq_ref[c] for c in range(NC)], axis=1).astype(BF16), w)
        if isinstance(t, int):
            row = max(t - 3, 0) * SEG
        else:
            row = pl.multiple_of(jnp.maximum(t - 3, 0) * SEG, SEG)
        out_ref[pl.ds(row, SEG), :] = yb[SEG:].astype(out_ref.dtype)
        return yb[:SEG]

    def x_seg(s):
        row = s * SEG if isinstance(s, int) else pl.multiple_of(s * SEG, SEG)
        return x_ref[pl.ds(row, SEG), :].astype(F32)

    def with_b(t):
        box = {}

        def hooks(p):
            if p == BQKV_AT - 0.5:
                b_phase1(t)
            elif p == BWO_PAIR:
                box['x2'] = b_phase2(t)
        return hooks, box

    def prepare_next(t, x2):
        sn = jnp.minimum(t + 1, NSEG - 1)
        hx_ref[0:SEG, :] = hxa_ref[pl.ds(al(sn * SEG, SEG), SEG), :]
        hx_ref[SEG:, :] = _ln(x2).astype(BF16)
        res_ref[...] = _cat0(x_seg(sn), x2)

    ri = lax.broadcasted_iota(jnp.int32, (D, D), 0)
    ci = lax.broadcasted_iota(jnp.int32, (D, D), 1)
    pm_ref[...] = (ri == (ci & 31) * BDH + (ci >> 5)).astype(F32).astype(BF16)
    mem0 = mem0_ref[...].astype(F32)
    mem_ref[...] = _cat0(mem0, mem0)
    bkv_ref[...] = jnp.zeros(bkv_ref.shape, F32)
    acc_ref[...] = jnp.zeros(acc_ref.shape, F32)
    eye = (lax.broadcasted_iota(jnp.int32, (128, 128), 0)
           == lax.broadcasted_iota(jnp.int32, (128, 128), 1)).astype(F32).astype(BF16)
    for p in range(NPRE):
        wait_w(p)
        start_w(p + WIN)
        if p == 0:
            bw2.start()
            bw1.start()
            hx_ref[0:SEG, :] = _ln(x_seg(0)).astype(BF16)
        for m in range(3):
            for c in range(NC):
                y = _nt(eye, wl_ref[m, p * PW:(p + 1) * PW, c * 128:(c + 1) * 128]).astype(BF16)
                wn_ref[c * 64:(c + 1) * 64, (p * 3 + m) * PW:(p * 3 + m + 1) * PW] = pltpu.bitcast(y, U32)

    def step0(p, carry):
        @pl.when(p >= NPRE)
        def _():
            wait_w(p)

        @pl.when((p >= NPRE) & (p + WIN < NPAIR))
        def _():
            start_w(p + WIN)

        def wfirst(m):
            w = wl_ref[m, pl.ds(al(p * PW, 128), PW), :]
            w_ref[m, pl.ds(al(p * (PW // 2), 64), PW // 2), :] = pltpu.bitcast(w, U32)
            return w

        arrange, scores, pv = attn_one_layer()
        h = _cat0(mem_ref[...].astype(BF16), hx_ref[0:SEG, :])
        xrows = pl.ds(al(p * XB, XB), XB)
        xl = _ln(x_ref[xrows, :].astype(F32)).astype(BF16)
        hxa_ref[xrows, :] = xl

        def pre(c0, c1):
            pre_ref[xrows, c0 * PW:c1 * PW] = _nn(xl, weights_nn(c0, c1)).astype(BF16)

        q, kt, vt = _nt(h, wfirst(0)).astype(BF16), arrange(_nt(h, wfirst(1))), arrange(_nt(h, wfirst(2)))
        pre(0, 1)
        s = scores(q, kt)
        pre(1, 2 * NPRE)
        o = pv(s, vt)
        pre(2 * NPRE, 3 * NPRE)
        acc_ref[...] += _nn(o, wfirst(3))

        @pl.when(p == PERM0)
        def _():
            bw2.wait()
            bw1.wait()

        @pl.when((p >= PERM0) & (p < PERM0 + D // PSZ))
        def _():
            r0 = (p - PERM0) * PSZ
            rows = pl.ds(al(r0, PSZ), PSZ)
            prow = pl.ds(al((p - PERM0) * (PSZ // 2), PSZ // 2), PSZ // 2)
            w3 = _cat0(*[bwqkv_ref[rows, j * D:(j + 1) * D] for j in range(3)])
            y = _nn(w3, pm_ref[...]).astype(BF16)
            for j in range(3):
                pwqkv_ref[prow, j * D:(j + 1) * D] = pltpu.bitcast(y[j * PSZ:(j + 1) * PSZ], U32)
            rn = lax.broadcasted_iota(jnp.int32, (PSZ, D), 0) + r0
            co = lax.broadcasted_iota(jnp.int32, (PSZ, D), 1)
            pmt = (co == (rn & 31) * BDH + (rn >> 5)).astype(F32).astype(BF16)
            pwo_ref[prow, :] = pltpu.bitcast(_nn(pmt, bwo_ref[...]).astype(BF16), U32)

        return carry

    lax.fori_loop(0, NPAIR, step0, 0)
    zeros = jnp.zeros((SEG, D), F32)
    mem_ref[0:M, :] = acc_ref[0:M, :]
    xb_ref[...] = _cat0(x_seg(0) + acc_ref[2 * M:, :], zeros)
    prepare_next(0, zeros)

    def single(t, carry):
        @pl.when(t == NSEG + 1)
        def _():
            out_a.start()

        l = (t >= NSEG).astype(jnp.int32)
        mrows = pl.ds(al(l * M, M), M)
        xrows = pl.ds(al(l * SEG, SEG), SEG)
        hooks, box = with_b(t)
        mem = mem_ref[mrows, :]
        h = _cat0(_cat0(mem, mem).astype(BF16), hx_ref[xrows, :])
        acc = a_phase(h, attn_one_layer(), hooks)
        mem_ref[mrows, :] = acc[:M]
        xb_ref[xrows, :] = res_ref[xrows, :] + acc[2 * M:]
        prepare_next(t, box['x2'])
        return carry

    def step(t, carry):
        hooks, box = with_b(t)
        h = _cat0(mem_ref[...].astype(BF16), hx_ref[...])
        acc = a_phase(h, attn_two_layers(), hooks, t)
        mem_ref[...] = acc[:2 * M]
        xb_ref[...] = res_ref[...] + acc[2 * M:]
        prepare_next(t, box['x2'])
        return carry

    def outer(i, carry):
        lax.fori_loop(1 + (NSEG - 1) * i, 2 + NSEG * i, single, 0)
        lax.fori_loop(2, NSEG - (NSEG - 2) * i, step, 0)
        return carry

    lax.fori_loop(0, 2, outer, 0)
    b_phase1(NSEG + 2)
    b_phase2(NSEG + 2)
    out_b.start()
    out_a.wait()
    out_b.wait()


@jax.jit
def pallas_interleave_layers__memory_aug_recurrent_mem_tr__sliding_local_dilated__prompt_kernel(
    A_x, A_mem0, A_Wq, A_Wk, A_Wv, A_Wo, A_seg_len, B_x, B_wqkv, B_wo,
):
    del A_seg_len, B_x
    wt = lambda w: jnp.transpose(w, (1, 2, 0)).reshape(HD, D)
    vm = pl.BlockSpec(memory_space=pltpu.VMEM)
    hbm = pl.BlockSpec(memory_space=pl.ANY)
    out = pl.pallas_call(
        _kernel,
        out_shape=jax.ShapeDtypeStruct((S, D), A_x.dtype),
        in_specs=[hbm, vm, hbm, hbm, hbm, hbm, hbm, hbm],
        out_specs=hbm,
        scratch_shapes=[
            pltpu.VMEM((S, D), BF16),
            pltpu.VMEM((S, D), BF16),
            pltpu.VMEM((4, HD, D), BF16),
            pltpu.VMEM((4, HD // 2, D), U32),
            pltpu.VMEM((D, 3 * D), BF16),
            pltpu.VMEM((D, D), BF16),
            pltpu.VMEM((D // 2, 3 * D), U32),
            pltpu.VMEM((D // 2, D), U32),
            pltpu.VMEM((D, D), BF16),
            pltpu.VMEM((R1, D), F32),
            pltpu.VMEM((2 * M, D), F32),
            pltpu.VMEM((2 * SEG, D), BF16),
            pltpu.VMEM((2 * SEG, D), F32),
            pltpu.VMEM((2 * SEG, D), F32),
            pltpu.VMEM((NC, 2 * SEG, 128), F32),
            pltpu.VMEM((2, 2, NC, 16 + SEG, 128), F32),
            pltpu.VMEM((D // 2, NPRE * 3 * PW), U32),
            pltpu.VMEM((S, D), BF16),
            pltpu.VMEM((S, NPRE * 3 * PW), BF16),
            pltpu.SemaphoreType.DMA((NPAIR,)),
            pltpu.SemaphoreType.DMA((6,)),
        ],
        compiler_params=pltpu.CompilerParams(vmem_limit_bytes=120 * 2 ** 20),
    )(A_x.reshape(S, D), A_mem0.reshape(M, D), wt(A_Wq), wt(A_Wk), wt(A_Wv),
      A_Wo.reshape(HD, D), B_wqkv, B_wo)
    return out.reshape(1, S, D)
```

```python
import jax
import jax.numpy as jnp
from jax import lax
import jax.experimental.pallas as pl
import jax.experimental.pallas.tpu as pltpu

S, D = 2048, 640
H, DH = 32, 192
HD = H * DH
M, SEG = 8, 32
L = M + SEG
NSEG = S // SEG
R = 2 * L
R1 = 2 * M + SEG
PW = 2 * DH
NPAIR = H // 2
BDH, BW, BDIL = 20, 8, 2
NC = D // 128
XB = S // NPAIR
NPRE = 2
BQKV_AT = 0
F32, BF16, U32 = jnp.float32, jnp.bfloat16, jnp.uint32
NT = (((1,), (1,)), ((), ()))
NU = 3 * NC
WIN = 4
HELD = 2
BWO_PAIR = 10


def _ln(x):
    m = jnp.mean(x, axis=-1, keepdims=True)
    xc = x - m
    v = jnp.mean(xc * xc, axis=-1, keepdims=True)
    return xc * lax.rsqrt(v + 1e-5)


def _nt(a, b):
    return lax.dot_general(a, b, NT, preferred_element_type=F32)


def _nn(a, b):
    return jnp.dot(a, b, preferred_element_type=F32)


def _cat0(*a):
    return jnp.concatenate(a, axis=0)


def _kernel(x_hbm, mem0_ref, wq_hbm, wk_hbm, wv_hbm, wo_hbm, bwqkv_hbm, bwo_hbm,
            out_hbm,
            x_ref, out_ref, wl_ref, w_ref, bwqkv_ref, bwo_ref, pwqkv_ref, pwo_ref,
            st_ref, acc_ref, mem_ref, hx_ref, res_ref, xb_ref, bq_ref, bkv_ref, wn_ref, hxa_ref, pre_ref, qsem, wsem, sem):
    def al(v, n):
        return v if isinstance(v, int) else pl.multiple_of(v, n)

    def qkv_copies(p):
        rows = pl.ds(al(p * PW, 128), PW)
        xrows = pl.ds(al(p * XB, XB), XB)
        return [pltpu.make_async_copy(x_hbm.at[xrows, :], x_ref.at[xrows, :], qsem.at[p])] + [
            pltpu.make_async_copy(src.at[rows, :], wl_ref.at[m, rows, :], qsem.at[p])
            for m, src in enumerate((wq_hbm, wk_hbm, wv_hbm))]

    def wo_copy(p):
        rows = pl.ds(al(p * PW, 128), PW)
        return pltpu.make_async_copy(wo_hbm.at[rows, :], wl_ref.at[3, rows, :], wsem.at[p])

    def unit_copy(u):
        src = bwqkv_hbm.at[pl.ds(al((u % NC) * 128, 128), 128), pl.ds(al((u // NC) * D, 128), D)]
        return pltpu.make_async_copy(src, bwqkv_ref.at[u], wsem.at[u])

    bw2 = pltpu.make_async_copy(bwo_hbm, bwo_ref, sem.at[0])
    osplit = (NSEG - 2) * SEG
    out_a = pltpu.make_async_copy(out_ref.at[pl.ds(0, osplit), :], out_hbm.at[pl.ds(0, osplit), :], sem.at[1])
    out_b = pltpu.make_async_copy(out_ref.at[pl.ds(osplit, S - osplit), :],
                                  out_hbm.at[pl.ds(osplit, S - osplit), :], sem.at[2])

    def issue_first(p, carry):
        for cp in qkv_copies(p):
            cp.start()
        return carry

    def issue_rest(p, carry):
        @pl.when((p >= NPRE) & (p < NPAIR))
        def _():
            for cp in qkv_copies(p):
                cp.start()

        @pl.when(p < NU)
        def _():
            unit_copy(p).start()

        @pl.when(p < NPAIR)
        def _():
            wo_copy(p).start()

        @pl.when(p == NPAIR)
        def _():
            bw2.start()

        return carry

    lax.fori_loop(0, NPRE, issue_first, 0)
    lax.fori_loop(0, WIN, issue_rest, 0)

    def weights(m, p):
        return pltpu.bitcast(w_ref[m, pl.ds(p * PW // 2, PW // 2), :], BF16)

    def weights_nn(c0, c1):
        return pltpu.bitcast(wn_ref[:, c0 * PW:c1 * PW], BF16)

    scale = DH ** -0.5
    ninf = -jnp.inf

    def softmax2(s, first, allowed):
        s = jnp.where(allowed, s * scale, -1e9)
        m0 = jnp.max(jnp.where(first, s, ninf), axis=-1, keepdims=True)
        m1 = jnp.max(jnp.where(first, ninf, s), axis=-1, keepdims=True)
        e = jnp.exp(s - jnp.where(first, m0, m1))
        d0 = jnp.sum(jnp.where(first, e, 0.0), axis=-1, keepdims=True)
        d1 = jnp.sum(jnp.where(first, 0.0, e), axis=-1, keepdims=True)
        return e, pl.reciprocal(d0, approx=True), pl.reciprocal(d1, approx=True)

    def masks(rows):
        qi = lax.broadcasted_iota(jnp.int32, (rows, R), 0)
        ki = lax.broadcasted_iota(jnp.int32, (rows, R), 1)
        first = ki < L
        kk = jnp.where(first, ki, ki - L)
        qq = M + ((qi - 2 * M) & (SEG - 1))
        allowed = (qi < 2 * M) | (kk <= qq)
        return qi, first, allowed

    def attn_two_layers():
        qi, first, allowed = masks(R)
        row_l1 = (qi < M) | ((qi >= 2 * M) & (qi < R1))
        is_a = first == row_l1
        lo = lax.broadcasted_iota(jnp.int32, (L, 128), 1) < 64

        def arrange(a):
            a1 = _cat0(a[0:M], a[2 * M:R1])
            a2 = _cat0(a[M:2 * M], a[R1:])
            cat = lambda u, w: _cat0(u, w).astype(BF16)
            m1, m2 = a1[:, 128:256], a2[:, 128:256]
            return (cat(a1[:, :128], a2[:, :128]), cat(a2[:, 256:], a1[:, 256:]),
                    cat(jnp.where(lo, m1, 0.0), jnp.where(lo, 0.0, m1)),
                    cat(jnp.where(lo, 0.0, m2), jnp.where(lo, m2, 0.0)))

        g1 = lambda a: a[0:R1]
        g2 = lambda a: _cat0(a[0:2 * M], a[R1:])
        merge = lambda u1, u2: _cat0(u1[0:M], u2[M:2 * M], u1[2 * M:], u2[2 * M:])

        def scores(q, kt):
            qm = q[:, 128:256]
            return _nt(q[:, :128], kt[0]), _nt(q[:, 256:], kt[1]), _nt(g1(qm), kt[2]), _nt(g2(qm), kt[3])

        lo_r = lax.broadcasted_iota(jnp.int32, (R, 128), 1) < 64
        pick = lambda u1, u2: _cat0(u1[0:M], u2[M:2 * M], u1[2 * M:R1], u2[R1:])

        def pv(s4, vt):
            sa, sb, s1, s2 = s4
            p, r0, r1 = softmax2(jnp.where(is_a, sa, sb) + merge(s1, s2), first, allowed)
            pb = p.astype(BF16)
            oa = _nn(jnp.where(is_a, p, 0.0).astype(BF16), vt[0])
            ob = _nn(jnp.where(is_a, 0.0, p).astype(BF16), vt[1])
            om = merge(_nn(g1(pb), vt[2]), _nn(g2(pb), vt[3]))
            r0, r1 = jnp.broadcast_to(r0, (R, 128)), jnp.broadcast_to(r1, (R, 128))
            ra, rb = pick(r0, r1), pick(r1, r0)
            return jnp.concatenate(
                [oa * ra, om * jnp.where(lo_r, ra, rb), ob * rb], axis=1).astype(BF16)

        return arrange, scores, pv

    def attn_one_layer():
        _, first, allowed = masks(R1)
        head_a = lax.broadcasted_iota(jnp.int32, (L, PW), 1) < DH

        def arrange(a):
            a1 = _cat0(a[0:M], a[2 * M:])
            return _cat0(jnp.where(head_a, a1, 0.0), jnp.where(head_a, 0.0, a1)).astype(BF16)

        head_a1 = lax.broadcasted_iota(jnp.int32, (R1, PW), 1) < DH

        def pv(s, vt):
            p, r0, r1 = softmax2(s, first, allowed)
            return (_nn(p.astype(BF16), vt) * jnp.where(head_a1, r0, r1)).astype(BF16)

        return arrange, _nt, pv

    def a_phase(h, attn, hooks, t=None):
        arrange, scores, pv = attn

        def proj(m, p):
            dt = BF16 if m == 0 else F32
            if p >= NPRE:
                return _nt(h, weights(m, p)).astype(dt)
            c = p * 3 + m
            if t is None:
                return _nn(h, weights_nn(c, c + 1)).astype(dt)
            y = _nn(_cat0(h[0:2 * M], h[R1:]), weights_nn(c, c + 1)).astype(dt)
            pre = pre_ref[pl.ds(al(t * SEG, SEG), SEG), c * PW:(c + 1) * PW].astype(dt)
            return _cat0(y[0:2 * M], pre, y[2 * M:])

        proj_o = lambda o, p: _nn(o, weights(3, p))
        q, kt = proj(0, 0), arrange(proj(1, 0))
        hooks(-1)
        vt = arrange(proj(2, 0))
        acc = None
        held = {}
        for p in range(NPAIR):
            last = p == NPAIR - 1
            s = scores(q, kt)
            hooks(p - 0.5)
            if not last:
                q, kt = proj(0, p + 1), arrange(proj(1, p + 1))
            else:
                for pp in range(p - HELD, p - 1):
                    acc = acc + proj_o(held[pp], pp)
            hooks(p)
            o = pv(s, vt)
            if not last:
                vt = arrange(proj(2, p + 1))
            else:
                acc = acc + proj_o(held[p - 1], p - 1)
            if NPAIR - 1 - HELD <= p < NPAIR - 1:
                held[p] = o
            else:
                y = proj_o(o, p)
                acc = y if acc is None else acc + y
        return acc

    def b_phase1(t):
        w = jnp.concatenate([_cat0(*[pltpu.bitcast(pwqkv_ref[j * NC + c], BF16) for c in range(NC)])
                             for j in range(3)], axis=1)
        qkv = _nn(_ln(xb_ref[...]).astype(BF16), w)
        for l in range(2):
            for c in range(NC):
                bq_ref[c, l * SEG:(l + 1) * SEG, :] = qkv[l * SEG:(l + 1) * SEG, c * 128:(c + 1) * 128]
                for j in range(2):
                    bkv_ref[l, j, c, 0:16, :] = bkv_ref[l, j, c, SEG:SEG + 16, :]
                    bkv_ref[l, j, c, 16:16 + SEG, :] = qkv[
                        l * SEG:(l + 1) * SEG, (j + 1) * D + c * 128:(j + 1) * D + (c + 1) * 128]
        bscale = BDH ** -0.5
        ri8 = lax.broadcasted_iota(jnp.int32, (8, 128), 0)
        for l in range(2):
            seg = t - 1 - 2 * l
            for r in range(SEG // 8):
                pos = seg * SEG + r * 8 + ri8
                q = [bq_ref[c, l * SEG + r * 8:l * SEG + r * 8 + 8, :] for c in range(NC)]
                lg = []
                for w in range(BW):
                    o0 = 16 + r * 8 - BDIL * w
                    s = q[0] * bkv_ref[l, 0, 0, o0:o0 + 8, :]
                    for c in range(1, NC):
                        s = s + q[c] * bkv_ref[l, 0, c, o0:o0 + 8, :]
                    s = s + pltpu.roll(s, 64, 1)
                    s = s + pltpu.roll(s, 32, 1)
                    s = s * bscale
                    if r * 8 - BDIL * w < 0:
                        s = jnp.where(pos - BDIL * w >= 0, s, -1e9)
                    lg.append(s)
                m = lg[0]
                for w in range(1, BW):
                    m = jnp.maximum(m, lg[w])
                e = [jnp.exp(s - m) for s in lg]
                den = e[0]
                for w in range(1, BW):
                    den = den + e[w]
                inv = pl.reciprocal(den, approx=True)
                for c in range(NC):
                    o = e[0] * bkv_ref[l, 1, c, 16 + r * 8:16 + r * 8 + 8, :]
                    for w in range(1, BW):
                        o0 = 16 + r * 8 - BDIL * w
                        o = o + e[w] * bkv_ref[l, 1, c, o0:o0 + 8, :]
                    bq_ref[c, l * SEG + r * 8:l * SEG + r * 8 + 8, :] = o * inv

    def b_phase2(t):
        w = jnp.concatenate([pltpu.bitcast(pwo_ref[c], BF16) for c in range(NC)], axis=1)
        yb = xb_ref[...] + _nn(jnp.concatenate([bq_ref[c] for c in range(NC)], axis=1).astype(BF16), w)
        if isinstance(t, int):
            row = max(t - 3, 0) * SEG
        else:
            row = pl.multiple_of(jnp.maximum(t - 3, 0) * SEG, SEG)
        out_ref[pl.ds(row, SEG), :] = yb[SEG:].astype(out_ref.dtype)
        return yb[:SEG]

    def x_seg(s):
        row = s * SEG if isinstance(s, int) else pl.multiple_of(s * SEG, SEG)
        return x_ref[pl.ds(row, SEG), :].astype(F32)

    def with_b(t):
        box = {}

        def hooks(p):
            if p == BQKV_AT - 0.5:
                b_phase1(t)
            elif p == BWO_PAIR:
                box['x2'] = b_phase2(t)
        return hooks, box

    def prepare_next(t, x2):
        sn = jnp.minimum(t + 1, NSEG - 1)
        hx_ref[0:SEG, :] = hxa_ref[pl.ds(al(sn * SEG, SEG), SEG), :]
        hx_ref[SEG:, :] = _ln(x2).astype(BF16)
        res_ref[...] = _cat0(x_seg(sn), x2)

    def permuted_rows(c):
        rows = [st_ref[c, pl.ds(d, H, stride=BDH), :] for d in range(BDH)]
        return _cat0(*rows).astype(BF16)

    mem0 = mem0_ref[...].astype(F32)
    mem_ref[...] = _cat0(mem0, mem0)
    bkv_ref[...] = jnp.zeros(bkv_ref.shape, F32)
    acc_ref[...] = jnp.zeros(acc_ref.shape, F32)
    eye = (lax.broadcasted_iota(jnp.int32, (128, 128), 0)
           == lax.broadcasted_iota(jnp.int32, (128, 128), 1)).astype(F32).astype(BF16)
    for p in range(NPRE):
        for cp in qkv_copies(p):
            cp.wait()
        if p == 0:
            hx_ref[0:SEG, :] = _ln(x_seg(0)).astype(BF16)
        for m in range(3):
            for c in range(NC):
                y = _nt(eye, wl_ref[m, p * PW:(p + 1) * PW, c * 128:(c + 1) * 128]).astype(BF16)
                wn_ref[c * 64:(c + 1) * 64, (p * 3 + m) * PW:(p * 3 + m + 1) * PW] = pltpu.bitcast(y, U32)

    def step0(p, carry):
        @pl.when(p >= NPRE)
        def _():
            for cp in qkv_copies(p):
                cp.wait()

        @pl.when(p < NU)
        def _():
            unit_copy(p).wait()

        wo_copy(p).wait()
        u = jnp.minimum(p, NU - 1)

        def wfirst(m):
            w = wl_ref[m, pl.ds(al(p * PW, 128), PW), :]
            w_ref[m, pl.ds(al(p * (PW // 2), 64), PW // 2), :] = pltpu.bitcast(w, U32)
            return w

        arrange, scores, pv = attn_one_layer()
        h = _cat0(mem_ref[...].astype(BF16), hx_ref[0:SEG, :])
        xrows = pl.ds(al(p * XB, XB), XB)
        xl = _ln(x_ref[xrows, :].astype(F32)).astype(BF16)
        hxa_ref[xrows, :] = xl

        def pre(c0, c1):
            pre_ref[xrows, c0 * PW:c1 * PW] = _nn(xl, weights_nn(c0, c1)).astype(BF16)

        q, kt, vt = _nt(h, wfirst(0)).astype(BF16), arrange(_nt(h, wfirst(1))), arrange(_nt(h, wfirst(2)))
        for c in range(NC):
            st_ref[0, c * 128:(c + 1) * 128, :] = _nt(eye, bwqkv_ref[u, :, c * 128:(c + 1) * 128])
        pre(0, 1)
        s = scores(q, kt)
        pre(1, 2 * NPRE)
        o = pv(s, vt)
        pwqkv_ref[u] = pltpu.bitcast(_nt(eye, permuted_rows(0)).astype(BF16), U32)
        pre(2 * NPRE, 3 * NPRE)
        acc_ref[...] += _nn(o, wfirst(3))
        issue_rest(p + WIN, 0)

        return carry

    lax.fori_loop(0, NPAIR, step0, 0)
    bw2.wait()
    for c in range(NC):
        st_ref[c] = bwo_ref[:, c * 128:(c + 1) * 128].astype(F32)
        pwo_ref[c] = pltpu.bitcast(permuted_rows(c), U32)
    zeros = jnp.zeros((SEG, D), F32)
    mem_ref[0:M, :] = acc_ref[0:M, :]
    xb_ref[...] = _cat0(x_seg(0) + acc_ref[2 * M:, :], zeros)
    prepare_next(0, zeros)

    def single(t, carry):
        @pl.when(t == NSEG + 1)
        def _():
            out_a.start()

        l = (t >= NSEG).astype(jnp.int32)
        mrows = pl.ds(al(l * M, M), M)
        xrows = pl.ds(al(l * SEG, SEG), SEG)
        hooks, box = with_b(t)
        mem = mem_ref[mrows, :]
        h = _cat0(_cat0(mem, mem).astype(BF16), hx_ref[xrows, :])
        acc = a_phase(h, attn_one_layer(), hooks)
        mem_ref[mrows, :] = acc[:M]
        xb_ref[xrows, :] = res_ref[xrows, :] + acc[2 * M:]
        prepare_next(t, box['x2'])
        return carry

    def step(t, carry):
        hooks, box = with_b(t)
        h = _cat0(mem_ref[...].astype(BF16), hx_ref[...])
        acc = a_phase(h, attn_two_layers(), hooks, t)
        mem_ref[...] = acc[:2 * M]
        xb_ref[...] = res_ref[...] + acc[2 * M:]
        prepare_next(t, box['x2'])
        return carry

    def outer(i, carry):
        lax.fori_loop(1 + (NSEG - 1) * i, 2 + NSEG * i, single, 0)
        lax.fori_loop(2, NSEG - (NSEG - 2) * i, step, 0)
        return carry

    lax.fori_loop(0, 2, outer, 0)
    b_phase1(NSEG + 2)
    b_phase2(NSEG + 2)
    out_b.start()
    out_a.wait()
    out_b.wait()


@jax.jit
def pallas_interleave_layers__memory_aug_recurrent_mem_tr__sliding_local_dilated__prompt_kernel(
    A_x, A_mem0, A_Wq, A_Wk, A_Wv, A_Wo, A_seg_len, B_x, B_wqkv, B_wo,
):
    del A_seg_len, B_x
    wt = lambda w: jnp.transpose(w, (1, 2, 0)).reshape(HD, D)
    vm = pl.BlockSpec(memory_space=pltpu.VMEM)
    hbm = pl.BlockSpec(memory_space=pl.ANY)
    out = pl.pallas_call(
        _kernel,
        out_shape=jax.ShapeDtypeStruct((S, D), A_x.dtype),
        in_specs=[hbm, vm, hbm, hbm, hbm, hbm, hbm, hbm],
        out_specs=hbm,
        scratch_shapes=[
            pltpu.VMEM((S, D), BF16),
            pltpu.VMEM((S, D), BF16),
            pltpu.VMEM((4, HD, D), BF16),
            pltpu.VMEM((4, HD // 2, D), U32),
            pltpu.VMEM((NU, 128, D), BF16),
            pltpu.VMEM((D, D), BF16),
            pltpu.VMEM((NU, 64, D), U32),
            pltpu.VMEM((NC, D // 2, 128), U32),
            pltpu.VMEM((NC, D, 128), F32),
            pltpu.VMEM((R1, D), F32),
            pltpu.VMEM((2 * M, D), F32),
            pltpu.VMEM((2 * SEG, D), BF16),
            pltpu.VMEM((2 * SEG, D), F32),
            pltpu.VMEM((2 * SEG, D), F32),
            pltpu.VMEM((NC, 2 * SEG, 128), F32),
            pltpu.VMEM((2, 2, NC, 16 + SEG, 128), F32),
            pltpu.VMEM((D // 2, NPRE * 3 * PW), U32),
            pltpu.VMEM((S, D), BF16),
            pltpu.VMEM((S, NPRE * 3 * PW), BF16),
            pltpu.SemaphoreType.DMA((NPAIR,)),
            pltpu.SemaphoreType.DMA((NPAIR,)),
            pltpu.SemaphoreType.DMA((3,)),
        ],
        compiler_params=pltpu.CompilerParams(vmem_limit_bytes=120 * 2 ** 20),
    )(A_x.reshape(S, D), A_mem0.reshape(M, D), wt(A_Wq), wt(A_Wk), wt(A_Wv),
      A_Wo.reshape(HD, D), B_wqkv, B_wo)
    return out.reshape(1, S, D)
```

```python
import jax
import jax.numpy as jnp
from jax import lax
import jax.experimental.pallas as pl
import jax.experimental.pallas.tpu as pltpu

S, D = 2048, 640
H, DH = 32, 192
HD = H * DH
M, SEG = 8, 32
L = M + SEG
NSEG = S // SEG
R = 2 * L
R1 = 2 * M + SEG
PW = 2 * DH
NPAIR = H // 2
BDH, BW, BDIL = 20, 8, 2
NC = D // 128
XB = S // NPAIR
NPRE = 2
BQKV_AT = 0
F32, BF16, U32 = jnp.float32, jnp.bfloat16, jnp.uint32
NT = (((1,), (1,)), ((), ()))
LOG2E = 1.4426950408889634
NU = 3 * NC
WIN = 4
ORDER = 'SQKPVW'
ORDER_LAST = 'SxPwW'
MIDFIRST = 3
HELD = 2
BWO2_PAIR = 10
BWO_PAIR = 10


def _ln(x):
    m = jnp.mean(x, axis=-1, keepdims=True)
    xc = x - m
    v = jnp.mean(xc * xc, axis=-1, keepdims=True)
    return xc * lax.rsqrt(v + 1e-5)


def _nt(a, b):
    return lax.dot_general(a, b, NT, preferred_element_type=F32)


def _nn(a, b):
    return jnp.dot(a, b, preferred_element_type=F32)


def _cat0(*a):
    return jnp.concatenate(a, axis=0)


def _kernel(x_hbm, mem0_ref, wq_hbm, wk_hbm, wv_hbm, wo_hbm, bwqkv_hbm, bwo_hbm,
            out_hbm,
            x_ref, out_ref, wl_ref, w_ref, bwqkv_ref, bwo_ref, pwqkv_ref, pwo_ref,
            st_ref, acc_ref, mem_ref, hx_ref, res_ref, xb_ref, bq_ref, bkv_ref, wn_ref, hxa_ref, pre_ref, qsem, wsem, sem):
    def al(v, n):
        return v if isinstance(v, int) else pl.multiple_of(v, n)

    def qkv_copies(p):
        rows = pl.ds(al(p * PW, 128), PW)
        xrows = pl.ds(al(p * XB, XB), XB)
        return [pltpu.make_async_copy(x_hbm.at[xrows, :], x_ref.at[xrows, :], qsem.at[p])] + [
            pltpu.make_async_copy(src.at[rows, :], wl_ref.at[m, rows, :], qsem.at[p])
            for m, src in enumerate((wq_hbm, wk_hbm, wv_hbm))]

    def wo_copy(p):
        rows = pl.ds(al(p * PW, 128), PW)
        return pltpu.make_async_copy(wo_hbm.at[rows, :], wl_ref.at[3, rows, :], wsem.at[p])

    def unit_copy(u):
        src = bwqkv_hbm.at[pl.ds(al((u % NC) * 128, 128), 128), pl.ds(al((u // NC) * D, 128), D)]
        return pltpu.make_async_copy(src, bwqkv_ref.at[u], wsem.at[u])

    bw2 = pltpu.make_async_copy(bwo_hbm, bwo_ref, sem.at[0])
    osplit = (NSEG - 2) * SEG
    out_a = pltpu.make_async_copy(out_ref.at[pl.ds(0, osplit), :], out_hbm.at[pl.ds(0, osplit), :], sem.at[1])
    out_b = pltpu.make_async_copy(out_ref.at[pl.ds(osplit, S - osplit), :],
                                  out_hbm.at[pl.ds(osplit, S - osplit), :], sem.at[2])

    def issue_first(p, carry):
        for cp in qkv_copies(p):
            cp.start()
        return carry

    def issue_rest(p, carry):
        @pl.when((p >= NPRE) & (p < NPAIR))
        def _():
            for cp in qkv_copies(p):
                cp.start()

        @pl.when(p < NU)
        def _():
            unit_copy(p).start()

        @pl.when(p < NPAIR)
        def _():
            wo_copy(p).start()

        @pl.when(p == NPAIR)
        def _():
            bw2.start()

        return carry

    lax.fori_loop(0, NPRE, issue_first, 0)
    lax.fori_loop(0, WIN, issue_rest, 0)

    def weights(m, p):
        return pltpu.bitcast(w_ref[m, pl.ds(p * PW // 2, PW // 2), :], BF16)

    def weights_nn(c0, c1):
        return pltpu.bitcast(wn_ref[:, c0 * PW:c1 * PW], BF16)

    scale = DH ** -0.5
    ninf = -jnp.inf

    def softmax2(s, sel, allowed):
        s = jnp.where(allowed, s, -1e9 / scale)
        m0 = jnp.max(jnp.where(sel, s, ninf), axis=-1, keepdims=True)
        m1 = jnp.max(jnp.where(sel, ninf, s), axis=-1, keepdims=True)
        e = jnp.exp2((s - jnp.where(sel, m0, m1)) * (scale * LOG2E))
        e0, e1 = jnp.where(sel, e, 0.0), jnp.where(sel, 0.0, e)
        d0 = jnp.sum(e0, axis=-1, keepdims=True)
        d1 = jnp.sum(e1, axis=-1, keepdims=True)
        return e, e0, e1, pl.reciprocal(d0, approx=True), pl.reciprocal(d1, approx=True)

    def masks(rows):
        qi = lax.broadcasted_iota(jnp.int32, (rows, R), 0)
        ki = lax.broadcasted_iota(jnp.int32, (rows, R), 1)
        first = ki < L
        kk = jnp.where(first, ki, ki - L)
        qq = M + ((qi - 2 * M) & (SEG - 1))
        allowed = (qi < 2 * M) | (kk <= qq)
        return qi, first, allowed

    def attn_two_layers():
        qi, first, allowed = masks(R)
        row_l1 = (qi < M) | ((qi >= 2 * M) & (qi < R1))
        is_a = first == row_l1
        lo = lax.broadcasted_iota(jnp.int32, (L, 128), 1) < 64

        def arrange(a):
            a1 = _cat0(a[0:M], a[2 * M:R1])
            a2 = _cat0(a[M:2 * M], a[R1:])
            cat = lambda u, w: _cat0(u, w).astype(BF16)
            m1, m2 = a1[:, 128:256], a2[:, 128:256]
            return (cat(a1[:, :128], a2[:, :128]), cat(a2[:, 256:], a1[:, 256:]),
                    cat(jnp.where(lo, m1, 0.0), jnp.where(lo, 0.0, m1)),
                    cat(jnp.where(lo, 0.0, m2), jnp.where(lo, m2, 0.0)))

        g1 = lambda a: a[0:R1]
        g2 = lambda a: _cat0(a[0:2 * M], a[R1:])
        merge = lambda u1, u2: _cat0(u1[0:M], u2[M:2 * M], u1[2 * M:], u2[2 * M:])

        def arrange_q(q):
            qm = q[:, 128:256]
            return [u.astype(BF16) for u in (q[:, :128], q[:, 256:], g1(qm), g2(qm))]

        def scores(q, kt):
            order = (2, 3, 0, 1) if MIDFIRST & 1 else (0, 1, 2, 3)
            r = {i: _nt(q[i], kt[i]) for i in order}
            return [r[i] for i in range(4)]

        lo_r = lax.broadcasted_iota(jnp.int32, (R, 128), 1) < 64

        def pv(s4, vt):
            sa, sb, s1, s2 = s4
            p, pa, pb, ra, rb = softmax2(jnp.where(is_a, sa, sb) + merge(s1, s2), is_a, allowed)
            if MIDFIRST & 2:
                om = merge(_nn(g1(p).astype(BF16), vt[2]), _nn(g2(p).astype(BF16), vt[3]))
                oa, ob = _nn(pa.astype(BF16), vt[0]), _nn(pb.astype(BF16), vt[1])
            else:
                oa, ob = _nn(pa.astype(BF16), vt[0]), _nn(pb.astype(BF16), vt[1])
                om = merge(_nn(g1(p).astype(BF16), vt[2]), _nn(g2(p).astype(BF16), vt[3]))
            return jnp.concatenate(
                [oa * ra, om * jnp.where(lo_r, ra, rb), ob * rb], axis=1).astype(BF16)

        return arrange_q, arrange, scores, pv

    def attn_one_layer():
        _, first, allowed = masks(R1)
        head_a = lax.broadcasted_iota(jnp.int32, (L, PW), 1) < DH

        def arrange(a):
            a1 = _cat0(a[0:M], a[2 * M:])
            return _cat0(jnp.where(head_a, a1, 0.0), jnp.where(head_a, 0.0, a1)).astype(BF16)

        head_a1 = lax.broadcasted_iota(jnp.int32, (R1, PW), 1) < DH

        def pv(s, vt):
            p, _, _, r0, r1 = softmax2(s, first, allowed)
            return (_nn(p.astype(BF16), vt) * jnp.where(head_a1, r0, r1)).astype(BF16)

        return lambda q: q.astype(BF16), arrange, _nt, pv

    def a_phase(h, attn, hooks, t=None):
        arrange_q, arrange, scores, pv = attn

        def proj(m, p):
            if p >= NPRE:
                return _nt(h, weights(m, p))
            c = p * 3 + m
            if t is None:
                return _nn(h, weights_nn(c, c + 1))
            y = _nn(_cat0(h[0:2 * M], h[R1:]), weights_nn(c, c + 1))
            pre = pre_ref[pl.ds(al(t * SEG, SEG), SEG), c * PW:(c + 1) * PW].astype(F32)
            return _cat0(y[0:2 * M], pre, y[2 * M:])

        proj_o = lambda o, p: _nn(o, weights(3, p))
        st = {'acc': None, 'o': {}, 'done': 0}

        def wo_upto(n):
            while st['done'] < n:
                pp = st['done']
                y = proj_o(st['o'].pop(pp), pp)
                st['acc'] = y if st['acc'] is None else st['acc'] + y
                st['done'] += 1

        q, kt = arrange_q(proj(0, 0)), arrange(proj(1, 0))
        vts = {0: arrange(proj(2, 0))}
        lim = NPAIR - 1 - HELD
        for p in range(NPAIR):
            last = p == NPAIR - 1
            for op in (ORDER_LAST if last else ORDER):
                if op == 'S':
                    s = scores(q, kt)
                    hooks(p - 0.5)
                elif op == 'Q':
                    qn = arrange_q(proj(0, p + 1))
                elif op == 'K':
                    ktn = arrange(proj(1, p + 1))
                elif op == 'V':
                    vts[p + 1] = arrange(proj(2, p + 1))
                elif op == 'P':
                    hooks(p)
                    st['o'][p] = pv(s, vts.pop(p))
                elif op == 'W':
                    wo_upto(p + 1 if last else min(p + 1, lim))
                elif op == 'w':
                    wo_upto(p if last else min(p, lim))
                elif op == 'x':
                    wo_upto(p - 1)
            q, kt = qn, ktn
        return st['acc']

    def b_phase1(t, layers=(0, 1)):
        w = jnp.concatenate([_cat0(*[pltpu.bitcast(pwqkv_ref[j * NC + c], BF16) for c in range(NC)])
                             for j in range(3)], axis=1)
        l0 = layers[0]
        qkv = _nn(_ln(xb_ref[l0 * SEG:(layers[-1] + 1) * SEG, :]).astype(BF16), w)
        for l in layers:
            rows = slice((l - l0) * SEG, (l - l0 + 1) * SEG)
            for c in range(NC):
                bq_ref[c, l * SEG:(l + 1) * SEG, :] = qkv[rows, c * 128:(c + 1) * 128]
                for j in range(2):
                    bkv_ref[l, j, c, 0:16, :] = bkv_ref[l, j, c, SEG:SEG + 16, :]
                    bkv_ref[l, j, c, 16:16 + SEG, :] = qkv[
                        rows, (j + 1) * D + c * 128:(j + 1) * D + (c + 1) * 128]
        bscale = BDH ** -0.5
        ri8 = lax.broadcasted_iota(jnp.int32, (8, 128), 0)
        for l in layers:
            seg = t - 1 - 2 * l
            for r in range(SEG // 8):
                pos = seg * SEG + r * 8 + ri8
                q = [bq_ref[c, l * SEG + r * 8:l * SEG + r * 8 + 8, :] for c in range(NC)]
                lg = []
                for w in range(BW):
                    o0 = 16 + r * 8 - BDIL * w
                    s = q[0] * bkv_ref[l, 0, 0, o0:o0 + 8, :]
                    for c in range(1, NC):
                        s = s + q[c] * bkv_ref[l, 0, c, o0:o0 + 8, :]
                    s = s + pltpu.roll(s, 64, 1)
                    s = s + pltpu.roll(s, 32, 1)
                    if r * 8 - BDIL * w < 0:
                        s = jnp.where(pos - BDIL * w >= 0, s, -1e9 / bscale)
                    lg.append(s)
                m = lg[0]
                for w in range(1, BW):
                    m = jnp.maximum(m, lg[w])
                e = [jnp.exp2((s - m) * (bscale * LOG2E)) for s in lg]
                den = e[0]
                for w in range(1, BW):
                    den = den + e[w]
                inv = pl.reciprocal(den, approx=True)
                for c in range(NC):
                    o = e[0] * bkv_ref[l, 1, c, 16 + r * 8:16 + r * 8 + 8, :]
                    for w in range(1, BW):
                        o0 = 16 + r * 8 - BDIL * w
                        o = o + e[w] * bkv_ref[l, 1, c, o0:o0 + 8, :]
                    bq_ref[c, l * SEG + r * 8:l * SEG + r * 8 + 8, :] = o * inv

    def b_phase2(t, layers=(0, 1)):
        rows = slice(layers[0] * SEG, (layers[-1] + 1) * SEG)
        w = jnp.concatenate([pltpu.bitcast(pwo_ref[c], BF16) for c in range(NC)], axis=1)
        o = jnp.concatenate([bq_ref[c, rows, :] for c in range(NC)], axis=1).astype(BF16)
        yb = xb_ref[rows, :] + _nn(o, w)
        if 1 in layers:
            row = al(max(t - 3, 0) * SEG if isinstance(t, int) else jnp.maximum(t - 3, 0) * SEG, SEG)
            out_ref[pl.ds(row, SEG), :] = yb[-SEG:].astype(out_ref.dtype)
        return yb[:SEG]

    def x_seg(s):
        row = s * SEG if isinstance(s, int) else pl.multiple_of(s * SEG, SEG)
        return x_ref[pl.ds(row, SEG), :].astype(F32)

    def with_b(t):
        box = {}

        def hooks(p):
            if p == BQKV_AT - 0.5:
                b_phase1(t)
            elif p == BWO_PAIR and BWO2_PAIR == BWO_PAIR:
                box['x2'] = b_phase2(t)
            elif p == BWO_PAIR:
                box['x2'] = b_phase2(t, (0,))
            elif p == BWO2_PAIR:
                b_phase2(t, (1,))
        return hooks, box

    def prepare_next(t, x2):
        sn = jnp.minimum(t + 1, NSEG - 1)
        hx_ref[0:SEG, :] = hxa_ref[pl.ds(al(sn * SEG, SEG), SEG), :]
        hx_ref[SEG:, :] = _ln(x2).astype(BF16)
        res_ref[...] = _cat0(x_seg(sn), x2)

    def permuted_rows(c):
        rows = [st_ref[c, pl.ds(d, H, stride=BDH), :] for d in range(BDH)]
        return _cat0(*rows).astype(BF16)

    mem0 = mem0_ref[...].astype(F32)
    mem_ref[...] = _cat0(mem0, mem0)
    bkv_ref[...] = jnp.zeros(bkv_ref.shape, F32)
    acc_ref[...] = jnp.zeros(acc_ref.shape, F32)
    eye = (lax.broadcasted_iota(jnp.int32, (128, 128), 0)
           == lax.broadcasted_iota(jnp.int32, (128, 128), 1)).astype(F32).astype(BF16)
    for p in range(NPRE):
        for cp in qkv_copies(p):
            cp.wait()
        if p == 0:
            hx_ref[0:SEG, :] = _ln(x_seg(0)).astype(BF16)
        for m in range(3):
            for c in range(NC):
                y = _nt(eye, wl_ref[m, p * PW:(p + 1) * PW, c * 128:(c + 1) * 128]).astype(BF16)
                wn_ref[c * 64:(c + 1) * 64, (p * 3 + m) * PW:(p * 3 + m + 1) * PW] = pltpu.bitcast(y, U32)

    def step0(p, carry):
        @pl.when(p >= NPRE)
        def _():
            for cp in qkv_copies(p):
                cp.wait()

        @pl.when(p < NU)
        def _():
            unit_copy(p).wait()

        wo_copy(p).wait()
        u = jnp.minimum(p, NU - 1)

        def wfirst(m):
            w = wl_ref[m, pl.ds(al(p * PW, 128), PW), :]
            w_ref[m, pl.ds(al(p * (PW // 2), 64), PW // 2), :] = pltpu.bitcast(w, U32)
            return w

        _, arrange, scores, pv = attn_one_layer()
        h = _cat0(mem_ref[...].astype(BF16), hx_ref[0:SEG, :])
        xrows = pl.ds(al(p * XB, XB), XB)
        xl = _ln(x_ref[xrows, :].astype(F32)).astype(BF16)
        hxa_ref[xrows, :] = xl

        def pre(c0, c1):
            pre_ref[xrows, c0 * PW:c1 * PW] = _nn(xl, weights_nn(c0, c1)).astype(BF16)

        q, kt, vt = _nt(h, wfirst(0)).astype(BF16), arrange(_nt(h, wfirst(1))), arrange(_nt(h, wfirst(2)))
        for c in range(NC):
            st_ref[0, c * 128:(c + 1) * 128, :] = _nt(eye, bwqkv_ref[u, :, c * 128:(c + 1) * 128])
        pre(0, 1)
        s = scores(q, kt)
        pre(1, 2 * NPRE)
        o = pv(s, vt)
        pwqkv_ref[u] = pltpu.bitcast(_nt(eye, permuted_rows(0)).astype(BF16), U32)
        pre(2 * NPRE, 3 * NPRE)
        acc_ref[...] += _nn(o, wfirst(3))
        issue_rest(p + WIN, 0)

        return carry

    lax.fori_loop(0, NPAIR, step0, 0)
    bw2.wait()
    for c in range(NC):
        st_ref[c] = bwo_ref[:, c * 128:(c + 1) * 128].astype(F32)
        pwo_ref[c] = pltpu.bitcast(permuted_rows(c), U32)
    zeros = jnp.zeros((SEG, D), F32)
    mem_ref[0:M, :] = acc_ref[0:M, :]
    xb_ref[...] = _cat0(x_seg(0) + acc_ref[2 * M:, :], zeros)
    prepare_next(0, zeros)

    def single(t, carry):
        @pl.when(t == NSEG + 1)
        def _():
            out_a.start()

        l = (t >= NSEG).astype(jnp.int32)
        mrows = pl.ds(al(l * M, M), M)
        xrows = pl.ds(al(l * SEG, SEG), SEG)
        hooks, box = with_b(t)
        mem = mem_ref[mrows, :]
        h = _cat0(_cat0(mem, mem).astype(BF16), hx_ref[xrows, :])
        acc = a_phase(h, attn_one_layer(), hooks)
        mem_ref[mrows, :] = acc[:M]
        xb_ref[xrows, :] = res_ref[xrows, :] + acc[2 * M:]
        prepare_next(t, box['x2'])
        return carry

    def step(t, carry):
        hooks, box = with_b(t)
        h = _cat0(mem_ref[...].astype(BF16), hx_ref[...])
        acc = a_phase(h, attn_two_layers(), hooks, t)
        mem_ref[...] = acc[:2 * M]
        xb_ref[...] = res_ref[...] + acc[2 * M:]
        prepare_next(t, box['x2'])
        return carry

    def outer(i, carry):
        lax.fori_loop(1 + (NSEG - 1) * i, 2 + NSEG * i, single, 0)
        lax.fori_loop(2, NSEG - (NSEG - 2) * i, step, 0)
        return carry

    lax.fori_loop(0, 2, outer, 0)
    b_phase1(NSEG + 2, (1,))
    b_phase2(NSEG + 2, (1,))
    out_b.start()
    out_a.wait()
    out_b.wait()


@jax.jit
def pallas_interleave_layers__memory_aug_recurrent_mem_tr__sliding_local_dilated__prompt_kernel(
    A_x, A_mem0, A_Wq, A_Wk, A_Wv, A_Wo, A_seg_len, B_x, B_wqkv, B_wo,
):
    del A_seg_len, B_x
    wt = lambda w: jnp.transpose(w, (1, 2, 0)).reshape(HD, D)
    vm = pl.BlockSpec(memory_space=pltpu.VMEM)
    hbm = pl.BlockSpec(memory_space=pl.ANY)
    out = pl.pallas_call(
        _kernel,
        out_shape=jax.ShapeDtypeStruct((S, D), A_x.dtype),
        in_specs=[hbm, vm, hbm, hbm, hbm, hbm, hbm, hbm],
        out_specs=hbm,
        scratch_shapes=[
            pltpu.VMEM((S, D), BF16),
            pltpu.VMEM((S, D), BF16),
            pltpu.VMEM((4, HD, D), BF16),
            pltpu.VMEM((4, HD // 2, D), U32),
            pltpu.VMEM((NU, 128, D), BF16),
            pltpu.VMEM((D, D), BF16),
            pltpu.VMEM((NU, 64, D), U32),
            pltpu.VMEM((NC, D // 2, 128), U32),
            pltpu.VMEM((NC, D, 128), F32),
            pltpu.VMEM((R1, D), F32),
            pltpu.VMEM((2 * M, D), F32),
            pltpu.VMEM((2 * SEG, D), BF16),
            pltpu.VMEM((2 * SEG, D), F32),
            pltpu.VMEM((2 * SEG, D), F32),
            pltpu.VMEM((NC, 2 * SEG, 128), F32),
            pltpu.VMEM((2, 2, NC, 16 + SEG, 128), F32),
            pltpu.VMEM((D // 2, NPRE * 3 * PW), U32),
            pltpu.VMEM((S, D), BF16),
            pltpu.VMEM((S, NPRE * 3 * PW), BF16),
            pltpu.SemaphoreType.DMA((NPAIR,)),
            pltpu.SemaphoreType.DMA((NPAIR,)),
            pltpu.SemaphoreType.DMA((3,)),
        ],
        compiler_params=pltpu.CompilerParams(vmem_limit_bytes=120 * 2 ** 20),
    )(A_x.reshape(S, D), A_mem0.reshape(M, D), wt(A_Wq), wt(A_Wk), wt(A_Wv),
      A_Wo.reshape(HD, D), B_wqkv, B_wo)
    return out.reshape(1, S, D)
```

```python
import jax
import jax.numpy as jnp
from jax import lax
import jax.experimental.pallas as pl
import jax.experimental.pallas.tpu as pltpu

S, D = 2048, 640
H, DH = 32, 192
HD = H * DH
M, SEG = 8, 32
L = M + SEG
NSEG = S // SEG
R = 2 * L
R1 = 2 * M + SEG
PW = 2 * DH
NPAIR = H // 2
BDH, BW, BDIL = 20, 8, 2
NC = D // 128
XB = 112
X0 = S - NPAIR * XB
NPRE = 9
XT = 7
TB = 0
BQKV_AT = 0
F32, BF16, U32 = jnp.float32, jnp.bfloat16, jnp.uint32
NT = (((1,), (1,)), ((), ()))
LOG2E = 1.4426950408889634
NU = 3 * NC
WIN = 4
ORDER = 'SQKPVW'
ORDER_LAST = 'SxPwW'
MIDFIRST = 3
HELD = 2
BWO2_PAIR = 10
BWO_PAIR = 10


def _ln(x):
    m = jnp.mean(x, axis=-1, keepdims=True)
    xc = x - m
    v = jnp.mean(xc * xc, axis=-1, keepdims=True)
    return xc * lax.rsqrt(v + 1e-5)


def _nt(a, b):
    return lax.dot_general(a, b, NT, preferred_element_type=F32)


def _nn(a, b):
    return jnp.dot(a, b, preferred_element_type=F32)


def _cat0(*a):
    return jnp.concatenate(a, axis=0)


def _kernel(x_hbm, mem0_ref, wq_hbm, wk_hbm, wv_hbm, wo_hbm, bwqkv_hbm, bwo_hbm,
            out_hbm,
            x_ref, out_ref, wl_ref, w_ref, wt_ref, bwqkv_ref, bwo_ref, pwqkv_ref, pwo_ref,
            st_ref, acc_ref, mem_ref, hx_ref, res_ref, xb_ref, bq_ref, bkv_ref, wn_ref, hxa_ref, pre_ref, qsem, wsem, sem):
    def al(v, n):
        return v if isinstance(v, int) else pl.multiple_of(v, n)

    w_hbm = (wq_hbm, wk_hbm, wv_hbm, wo_hbm)

    def w_copy(m, p, s):
        rows = pl.ds(al(p * PW, 128), PW)
        return pltpu.make_async_copy(w_hbm[m].at[rows, :], wl_ref.at[m, rows, :], s)

    def x_rows(p):
        return pl.ds(al(X0 + p * XB, 16), XB)

    def x_copy(p):
        return pltpu.make_async_copy(x_hbm.at[x_rows(p), :], x_ref.at[x_rows(p), :], wsem.at[p])

    first = [pltpu.make_async_copy(x_hbm.at[pl.ds(0, X0), :], x_ref.at[pl.ds(0, X0), :], qsem.at[NPRE])] + [
        w_copy(c % 3, c // 3, qsem.at[c]) for c in range(NPRE)]

    def unit_copy(u):
        src = bwqkv_hbm.at[pl.ds(al((u % NC) * 128, 128), 128), pl.ds(al((u // NC) * D, 128), D)]
        return pltpu.make_async_copy(src, bwqkv_ref.at[u], wsem.at[u])

    bw2 = pltpu.make_async_copy(bwo_hbm, bwo_ref, sem.at[0])
    osplit = (NSEG - 2) * SEG
    out_a = pltpu.make_async_copy(out_ref.at[pl.ds(0, osplit), :], out_hbm.at[pl.ds(0, osplit), :], sem.at[1])
    out_b = pltpu.make_async_copy(out_ref.at[pl.ds(osplit, S - osplit), :],
                                  out_hbm.at[pl.ds(osplit, S - osplit), :], sem.at[2])

    def issue_first(i, carry):
        for j, cp in enumerate(first):
            pl.when(i == j)(cp.start)
        return carry

    def group(p, act):
        for m in range(3):
            pl.when((p * 3 + m >= NPRE) & (p < NPAIR))(lambda m=m: act(w_copy(m, p, wsem.at[p])))
        pl.when(p < NU)(lambda: act(unit_copy(p)))

        @pl.when(p < NPAIR)
        def _():
            act(x_copy(p))
            act(w_copy(3, p, wsem.at[p]))

    def issue_rest(p, carry):
        group(p, lambda cp: cp.start())
        pl.when(p == NPAIR)(bw2.start)
        return carry

    lax.fori_loop(0, len(first), issue_first, 0)
    lax.fori_loop(0, WIN, issue_rest, 0)

    def weights(m, p):
        if m < 3:
            return pltpu.bitcast(wt_ref[p * 3 + m], BF16)
        return pltpu.bitcast(w_ref[pl.ds(p * PW // 2, PW // 2), :], BF16)

    def transposed(w):
        return w.T if TB else w.astype(F32).T.astype(BF16)

    def weights_nn(c0, c1):
        return pltpu.bitcast(wn_ref[:, c0 * PW:c1 * PW], BF16)

    scale = DH ** -0.5
    ninf = -jnp.inf

    def softmax2(s, sel, allowed):
        s = jnp.where(allowed, s, -1e9 / scale)
        m0 = jnp.max(jnp.where(sel, s, ninf), axis=-1, keepdims=True)
        m1 = jnp.max(jnp.where(sel, ninf, s), axis=-1, keepdims=True)
        e = jnp.exp2((s - jnp.where(sel, m0, m1)) * (scale * LOG2E))
        e0, e1 = jnp.where(sel, e, 0.0), jnp.where(sel, 0.0, e)
        d0 = jnp.sum(e0, axis=-1, keepdims=True)
        d1 = jnp.sum(e1, axis=-1, keepdims=True)
        return e, e0, e1, pl.reciprocal(d0, approx=True), pl.reciprocal(d1, approx=True)

    def masks(rows):
        qi = lax.broadcasted_iota(jnp.int32, (rows, R), 0)
        ki = lax.broadcasted_iota(jnp.int32, (rows, R), 1)
        first = ki < L
        kk = jnp.where(first, ki, ki - L)
        qq = M + ((qi - 2 * M) & (SEG - 1))
        allowed = (qi < 2 * M) | (kk <= qq)
        return qi, first, allowed

    def attn_two_layers():
        qi, first, allowed = masks(R)
        row_l1 = (qi < M) | ((qi >= 2 * M) & (qi < R1))
        is_a = first == row_l1
        lo = lax.broadcasted_iota(jnp.int32, (L, 128), 1) < 64

        def arrange(a):
            a1 = _cat0(a[0:M], a[2 * M:R1])
            a2 = _cat0(a[M:2 * M], a[R1:])
            cat = lambda u, w: _cat0(u, w).astype(BF16)
            m1, m2 = a1[:, 128:256], a2[:, 128:256]
            return (cat(a1[:, :128], a2[:, :128]), cat(a2[:, 256:], a1[:, 256:]),
                    cat(jnp.where(lo, m1, 0.0), jnp.where(lo, 0.0, m1)),
                    cat(jnp.where(lo, 0.0, m2), jnp.where(lo, m2, 0.0)))

        g1 = lambda a: a[0:R1]
        g2 = lambda a: _cat0(a[0:2 * M], a[R1:])
        merge = lambda u1, u2: _cat0(u1[0:M], u2[M:2 * M], u1[2 * M:], u2[2 * M:])

        def arrange_q(q):
            qm = q[:, 128:256]
            return [u.astype(BF16) for u in (q[:, :128], q[:, 256:], g1(qm), g2(qm))]

        def scores(q, kt):
            order = (2, 3, 0, 1) if MIDFIRST & 1 else (0, 1, 2, 3)
            r = {i: _nt(q[i], kt[i]) for i in order}
            return [r[i] for i in range(4)]

        lo_r = lax.broadcasted_iota(jnp.int32, (R, 128), 1) < 64

        def pv(s4, vt):
            sa, sb, s1, s2 = s4
            p, pa, pb, ra, rb = softmax2(jnp.where(is_a, sa, sb) + merge(s1, s2), is_a, allowed)
            if MIDFIRST & 2:
                om = merge(_nn(g1(p).astype(BF16), vt[2]), _nn(g2(p).astype(BF16), vt[3]))
                oa, ob = _nn(pa.astype(BF16), vt[0]), _nn(pb.astype(BF16), vt[1])
            else:
                oa, ob = _nn(pa.astype(BF16), vt[0]), _nn(pb.astype(BF16), vt[1])
                om = merge(_nn(g1(p).astype(BF16), vt[2]), _nn(g2(p).astype(BF16), vt[3]))
            return jnp.concatenate(
                [oa * ra, om * jnp.where(lo_r, ra, rb), ob * rb], axis=1).astype(BF16)

        return arrange_q, arrange, scores, pv

    def attn_one_layer():
        _, first, allowed = masks(R1)
        head_a = lax.broadcasted_iota(jnp.int32, (L, PW), 1) < DH

        def arrange(a):
            a1 = _cat0(a[0:M], a[2 * M:])
            return _cat0(jnp.where(head_a, a1, 0.0), jnp.where(head_a, 0.0, a1)).astype(BF16)

        head_a1 = lax.broadcasted_iota(jnp.int32, (R1, PW), 1) < DH

        def pv(s, vt):
            p, _, _, r0, r1 = softmax2(s, first, allowed)
            return (_nn(p.astype(BF16), vt) * jnp.where(head_a1, r0, r1)).astype(BF16)

        return lambda q: q.astype(BF16), arrange, _nt, pv

    def a_phase(h, attn, hooks, t=None):
        arrange_q, arrange, scores, pv = attn

        def proj(m, p):
            c = p * 3 + m
            if c >= NPRE or t is None:
                return _nn(h, weights(m, p))
            y = _nn(_cat0(h[0:2 * M], h[R1:]), weights(m, p))
            pre = pre_ref[pl.ds(al(t * SEG, SEG), SEG), c * PW:(c + 1) * PW].astype(F32)
            return _cat0(y[0:2 * M], pre, y[2 * M:])

        proj_o = lambda o, p: _nn(o, weights(3, p))
        st = {'acc': None, 'o': {}, 'done': 0}

        def wo_upto(n):
            while st['done'] < n:
                pp = st['done']
                y = proj_o(st['o'].pop(pp), pp)
                st['acc'] = y if st['acc'] is None else st['acc'] + y
                st['done'] += 1

        q, kt = arrange_q(proj(0, 0)), arrange(proj(1, 0))
        vts = {0: arrange(proj(2, 0))}
        lim = NPAIR - 1 - HELD
        for p in range(NPAIR):
            last = p == NPAIR - 1
            for op in (ORDER_LAST if last else ORDER):
                if op == 'S':
                    s = scores(q, kt)
                    hooks(p - 0.5)
                elif op == 'Q':
                    qn = arrange_q(proj(0, p + 1))
                elif op == 'K':
                    ktn = arrange(proj(1, p + 1))
                elif op == 'V':
                    vts[p + 1] = arrange(proj(2, p + 1))
                elif op == 'P':
                    hooks(p)
                    st['o'][p] = pv(s, vts.pop(p))
                elif op == 'W':
                    wo_upto(p + 1 if last else min(p + 1, lim))
                elif op == 'w':
                    wo_upto(p if last else min(p, lim))
                elif op == 'x':
                    wo_upto(p - 1)
            q, kt = qn, ktn
        return st['acc']

    def b_phase1(t, layers=(0, 1)):
        w = jnp.concatenate([_cat0(*[pltpu.bitcast(pwqkv_ref[j * NC + c], BF16) for c in range(NC)])
                             for j in range(3)], axis=1)
        l0 = layers[0]
        qkv = _nn(_ln(xb_ref[l0 * SEG:(layers[-1] + 1) * SEG, :]).astype(BF16), w)
        for l in layers:
            rows = slice((l - l0) * SEG, (l - l0 + 1) * SEG)
            for c in range(NC):
                bq_ref[c, l * SEG:(l + 1) * SEG, :] = qkv[rows, c * 128:(c + 1) * 128]
                for j in range(2):
                    bkv_ref[l, j, c, 0:16, :] = bkv_ref[l, j, c, SEG:SEG + 16, :]
                    bkv_ref[l, j, c, 16:16 + SEG, :] = qkv[
                        rows, (j + 1) * D + c * 128:(j + 1) * D + (c + 1) * 128]
        bscale = BDH ** -0.5
        ri8 = lax.broadcasted_iota(jnp.int32, (8, 128), 0)
        for l in layers:
            seg = t - 1 - 2 * l
            for r in range(SEG // 8):
                pos = seg * SEG + r * 8 + ri8
                q = [bq_ref[c, l * SEG + r * 8:l * SEG + r * 8 + 8, :] for c in range(NC)]
                lg = []
                for w in range(BW):
                    o0 = 16 + r * 8 - BDIL * w
                    s = q[0] * bkv_ref[l, 0, 0, o0:o0 + 8, :]
                    for c in range(1, NC):
                        s = s + q[c] * bkv_ref[l, 0, c, o0:o0 + 8, :]
                    s = s + pltpu.roll(s, 64, 1)
                    s = s + pltpu.roll(s, 32, 1)
                    if r * 8 - BDIL * w < 0:
                        s = jnp.where(pos - BDIL * w >= 0, s, -1e9 / bscale)
                    lg.append(s)
                m = lg[0]
                for w in range(1, BW):
                    m = jnp.maximum(m, lg[w])
                e = [jnp.exp2((s - m) * (bscale * LOG2E)) for s in lg]
                den = e[0]
                for w in range(1, BW):
                    den = den + e[w]
                inv = pl.reciprocal(den, approx=True)
                for c in range(NC):
                    o = e[0] * bkv_ref[l, 1, c, 16 + r * 8:16 + r * 8 + 8, :]
                    for w in range(1, BW):
                        o0 = 16 + r * 8 - BDIL * w
                        o = o + e[w] * bkv_ref[l, 1, c, o0:o0 + 8, :]
                    bq_ref[c, l * SEG + r * 8:l * SEG + r * 8 + 8, :] = o * inv

    def b_phase2(t, layers=(0, 1)):
        rows = slice(layers[0] * SEG, (layers[-1] + 1) * SEG)
        w = jnp.concatenate([pltpu.bitcast(pwo_ref[c], BF16) for c in range(NC)], axis=1)
        o = jnp.concatenate([bq_ref[c, rows, :] for c in range(NC)], axis=1).astype(BF16)
        yb = xb_ref[rows, :] + _nn(o, w)
        if 1 in layers:
            row = al(max(t - 3, 0) * SEG if isinstance(t, int) else jnp.maximum(t - 3, 0) * SEG, SEG)
            out_ref[pl.ds(row, SEG), :] = yb[-SEG:].astype(out_ref.dtype)
        return yb[:SEG]

    def x_seg(s):
        row = s * SEG if isinstance(s, int) else pl.multiple_of(s * SEG, SEG)
        return x_ref[pl.ds(row, SEG), :].astype(F32)

    def with_b(t):
        box = {}

        def hooks(p):
            if p == BQKV_AT - 0.5:
                b_phase1(t)
            elif p == BWO_PAIR and BWO2_PAIR == BWO_PAIR:
                box['x2'] = b_phase2(t)
            elif p == BWO_PAIR:
                box['x2'] = b_phase2(t, (0,))
            elif p == BWO2_PAIR:
                b_phase2(t, (1,))
        return hooks, box

    def prepare_next(t, x2):
        sn = jnp.minimum(t + 1, NSEG - 1)
        hx_ref[0:SEG, :] = hxa_ref[pl.ds(al(sn * SEG, SEG), SEG), :]
        hx_ref[SEG:, :] = _ln(x2).astype(BF16)
        res_ref[...] = _cat0(x_seg(sn), x2)

    def permuted_rows(c):
        rows = [st_ref[c, pl.ds(d, H, stride=BDH), :] for d in range(BDH)]
        return _cat0(*rows)

    mem0 = mem0_ref[...].astype(F32)
    mem_ref[...] = _cat0(mem0, mem0)
    bkv_ref[...] = jnp.zeros(bkv_ref.shape, F32)
    acc_ref[...] = jnp.zeros(acc_ref.shape, F32)
    eye = (lax.broadcasted_iota(jnp.int32, (128, 128), 0)
           == lax.broadcasted_iota(jnp.int32, (128, 128), 1)).astype(F32).astype(BF16)
    first[0].wait()
    xl0 = _ln(x_ref[0:X0, :].astype(F32)).astype(BF16)
    hxa_ref[0:X0, :] = xl0
    hx_ref[0:SEG, :] = xl0[0:SEG]
    for u in range(NPRE):
        first[1 + u].wait()
        w = wl_ref[u % 3, (u // 3) * PW:(u // 3 + 1) * PW, :]
        for c in range(NC):
            wc = w[:, c * 128:(c + 1) * 128]
            y = (wc.astype(F32).T if XT & 4 else _nt(eye, wc)).astype(BF16)
            wn_ref[c * 64:(c + 1) * 64, u * PW:(u + 1) * PW] = pltpu.bitcast(y, U32)
        pre_ref[2 * SEG:X0, u * PW:(u + 1) * PW] = _nt(hxa_ref[2 * SEG:X0, :], w).astype(BF16)

    def step0(p, carry):
        group(p, lambda cp: cp.wait())
        u = jnp.minimum(p, NU - 1)

        def wfirst(m):
            w = wl_ref[m, pl.ds(al(p * PW, 128), PW), :]
            if m < 3:
                for c in range(NC):
                    wt_ref[p * 3 + m, c * 64:(c + 1) * 64, :] = pltpu.bitcast(
                        transposed(w[:, c * 128:(c + 1) * 128]), U32)
            else:
                w_ref[pl.ds(al(p * (PW // 2), 64), PW // 2), :] = pltpu.bitcast(w, U32)
            return w

        _, arrange, scores, pv = attn_one_layer()
        h = _cat0(mem_ref[...].astype(BF16), hx_ref[0:SEG, :])
        xrows = x_rows(p)
        xl = _ln(x_ref[xrows, :].astype(F32)).astype(BF16)
        hxa_ref[xrows, :] = xl

        def pre(c0, c1):
            pre_ref[xrows, c0 * PW:c1 * PW] = _nn(xl, weights_nn(c0, c1)).astype(BF16)

        q, kt, vt = _nt(h, wfirst(0)).astype(BF16), arrange(_nt(h, wfirst(1))), arrange(_nt(h, wfirst(2)))
        for c in range(NC):
            bt = bwqkv_ref[u, :, c * 128:(c + 1) * 128]
            st_ref[0, c * 128:(c + 1) * 128, :] = bt.astype(F32).T if XT & 1 else _nt(eye, bt)
        pre(0, 1)
        s = scores(q, kt)
        pre(1, 4)
        o = pv(s, vt)
        pr = permuted_rows(0)
        pwqkv_ref[u] = pltpu.bitcast((pr.T if XT & 2 else _nt(eye, pr.astype(BF16))).astype(BF16), U32)
        pre(4, NPRE)
        acc_ref[...] += _nn(o, wfirst(3))
        issue_rest(p + WIN, 0)

        return carry

    lax.fori_loop(0, NPAIR, step0, 0)
    bw2.wait()
    for c in range(NC):
        st_ref[c] = bwo_ref[:, c * 128:(c + 1) * 128].astype(F32)
        pwo_ref[c] = pltpu.bitcast(permuted_rows(c).astype(BF16), U32)
    zeros = jnp.zeros((SEG, D), F32)
    mem_ref[0:M, :] = acc_ref[0:M, :]
    xb_ref[...] = _cat0(x_seg(0) + acc_ref[2 * M:, :], zeros)
    prepare_next(0, zeros)

    def single(t, carry):
        @pl.when(t == NSEG + 1)
        def _():
            out_a.start()

        l = (t >= NSEG).astype(jnp.int32)
        mrows = pl.ds(al(l * M, M), M)
        xrows = pl.ds(al(l * SEG, SEG), SEG)
        hooks, box = with_b(t)
        mem = mem_ref[mrows, :]
        h = _cat0(_cat0(mem, mem).astype(BF16), hx_ref[xrows, :])
        acc = a_phase(h, attn_one_layer(), hooks)
        mem_ref[mrows, :] = acc[:M]
        xb_ref[xrows, :] = res_ref[xrows, :] + acc[2 * M:]
        prepare_next(t, box['x2'])
        return carry

    def step(t, carry):
        hooks, box = with_b(t)
        h = _cat0(mem_ref[...].astype(BF16), hx_ref[...])
        acc = a_phase(h, attn_two_layers(), hooks, t)
        mem_ref[...] = acc[:2 * M]
        xb_ref[...] = res_ref[...] + acc[2 * M:]
        prepare_next(t, box['x2'])
        return carry

    def outer(i, carry):
        lax.fori_loop(1 + (NSEG - 1) * i, 2 + NSEG * i, single, 0)
        lax.fori_loop(2, NSEG - (NSEG - 2) * i, step, 0)
        return carry

    lax.fori_loop(0, 2, outer, 0)
    b_phase1(NSEG + 2, (1,))
    b_phase2(NSEG + 2, (1,))
    out_b.start()
    out_a.wait()
    out_b.wait()


@jax.jit
def pallas_interleave_layers__memory_aug_recurrent_mem_tr__sliding_local_dilated__prompt_kernel(
    A_x, A_mem0, A_Wq, A_Wk, A_Wv, A_Wo, A_seg_len, B_x, B_wqkv, B_wo,
):
    del A_seg_len, B_x
    wt = lambda w: jnp.transpose(w, (1, 2, 0)).reshape(HD, D)
    vm = pl.BlockSpec(memory_space=pltpu.VMEM)
    hbm = pl.BlockSpec(memory_space=pl.ANY)
    out = pl.pallas_call(
        _kernel,
        out_shape=jax.ShapeDtypeStruct((S, D), A_x.dtype),
        in_specs=[hbm, vm, hbm, hbm, hbm, hbm, hbm, hbm],
        out_specs=hbm,
        scratch_shapes=[
            pltpu.VMEM((S, D), BF16),
            pltpu.VMEM((S, D), BF16),
            pltpu.VMEM((4, HD, D), BF16),
            pltpu.VMEM((HD // 2, D), U32),
            pltpu.VMEM((3 * NPAIR, D // 2, PW), U32),
            pltpu.VMEM((NU, 128, D), BF16),
            pltpu.VMEM((D, D), BF16),
            pltpu.VMEM((NU, 64, D), U32),
            pltpu.VMEM((NC, D // 2, 128), U32),
            pltpu.VMEM((NC, D, 128), F32),
            pltpu.VMEM((R1, D), F32),
            pltpu.VMEM((2 * M, D), F32),
            pltpu.VMEM((2 * SEG, D), BF16),
            pltpu.VMEM((2 * SEG, D), F32),
            pltpu.VMEM((2 * SEG, D), F32),
            pltpu.VMEM((NC, 2 * SEG, 128), F32),
            pltpu.VMEM((2, 2, NC, 16 + SEG, 128), F32),
            pltpu.VMEM((D // 2, NPRE * PW), U32),
            pltpu.VMEM((S, D), BF16),
            pltpu.VMEM((S, NPRE * PW), BF16),
            pltpu.SemaphoreType.DMA((NPRE + 1,)),
            pltpu.SemaphoreType.DMA((NPAIR,)),
            pltpu.SemaphoreType.DMA((3,)),
        ],
        compiler_params=pltpu.CompilerParams(vmem_limit_bytes=120 * 2 ** 20),
    )(A_x.reshape(S, D), A_mem0.reshape(M, D), wt(A_Wq), wt(A_Wk), wt(A_Wv),
      A_Wo.reshape(HD, D), B_wqkv, B_wo)
    return out.reshape(1, S, D)
```

```python
import jax
import jax.numpy as jnp
from jax import lax
import jax.experimental.pallas as pl
import jax.experimental.pallas.tpu as pltpu

S, D = 2048, 640
H, DH = 32, 192
HD = H * DH
M, SEG = 8, 32
L = M + SEG
NSEG = S // SEG
R = 2 * L
R1 = 2 * M + SEG
PW = 2 * DH
NPAIR = H // 2
BDH, BW, BDIL = 20, 8, 2
NC = D // 128
XB = 112
X0 = S - NPAIR * XB
NPRE = 8
XT = 7
TB = 1
RELOAD = 0
S0 = (2, 1, 1, 2, 1)
BQKV_AT = 0
F32, BF16, U32 = jnp.float32, jnp.bfloat16, jnp.uint32
NT = (((1,), (1,)), ((), ()))
LOG2E = 1.4426950408889634
NU = 3 * NC
WIN = 4
ORDER = 'SQKPVW'
ORDER_LAST = 'SxPwW'
MIDFIRST = 3
HELD = 2
BWO2_PAIR = 10
BWO_PAIR = 10


def _ln(x):
    m = jnp.mean(x, axis=-1, keepdims=True)
    xc = x - m
    v = jnp.mean(xc * xc, axis=-1, keepdims=True)
    return xc * lax.rsqrt(v + 1e-5)


def _nt(a, b):
    return lax.dot_general(a, b, NT, preferred_element_type=F32)


def _nn(a, b):
    return jnp.dot(a, b, preferred_element_type=F32)


def _cat0(*a):
    return jnp.concatenate(a, axis=0)


def _kernel(x_hbm, mem0_ref, wq_hbm, wk_hbm, wv_hbm, wo_hbm, bwqkv_hbm, bwo_hbm,
            out_hbm,
            x_ref, out_ref, wl_ref, w_ref, wt_ref, bwqkv_ref, bwo_ref, pwqkv_ref, pwo_ref,
            st_ref, acc_ref, mem_ref, hx_ref, res_ref, xb_ref, bq_ref, bkv_ref, wn_ref, hxa_ref, pre_ref, qsem, wsem, sem):
    def al(v, n):
        return v if isinstance(v, int) else pl.multiple_of(v, n)

    w_hbm = (wq_hbm, wk_hbm, wv_hbm, wo_hbm)

    def w_copy(m, p, s):
        rows = pl.ds(al(p * PW, 128), PW)
        return pltpu.make_async_copy(w_hbm[m].at[rows, :], wl_ref.at[m, rows, :], s)

    def x_rows(p):
        return pl.ds(al(X0 + p * XB, 16), XB)

    def x_copy(p):
        return pltpu.make_async_copy(x_hbm.at[x_rows(p + 1), :], x_ref.at[x_rows(p + 1), :], wsem.at[p])

    first = [pltpu.make_async_copy(x_hbm.at[pl.ds(0, X0 + XB), :], x_ref.at[pl.ds(0, X0 + XB), :], qsem.at[NPRE])] + [
        w_copy(c % 3, c // 3, qsem.at[c]) for c in range(NPRE)]

    def unit_copy(u):
        src = bwqkv_hbm.at[pl.ds(al((u % NC) * 128, 128), 128), pl.ds(al((u // NC) * D, 128), D)]
        return pltpu.make_async_copy(src, bwqkv_ref.at[u], wsem.at[u])

    bw2 = pltpu.make_async_copy(bwo_hbm, bwo_ref, sem.at[0])
    osplit = (NSEG - 2) * SEG
    out_a = pltpu.make_async_copy(out_ref.at[pl.ds(0, osplit), :], out_hbm.at[pl.ds(0, osplit), :], sem.at[1])
    out_b = pltpu.make_async_copy(out_ref.at[pl.ds(osplit, S - osplit), :],
                                  out_hbm.at[pl.ds(osplit, S - osplit), :], sem.at[2])

    def issue_first(i, carry):
        for j, cp in enumerate(first):
            pl.when(i == j)(cp.start)
        return carry

    def group(p, act):
        for m in range(3):
            pl.when((p * 3 + m >= NPRE) & (p < NPAIR))(lambda m=m: act(w_copy(m, p, wsem.at[p])))

        @pl.when(p < NPAIR - 1)
        def _():
            act(unit_copy(p))
            act(x_copy(p))

        pl.when(p < NPAIR)(lambda: act(w_copy(3, p, wsem.at[p])))

    def issue_rest(p, carry):
        group(p, lambda cp: cp.start())
        pl.when(p == NPAIR)(bw2.start)
        return carry

    lax.fori_loop(0, len(first), issue_first, 0)
    lax.fori_loop(0, WIN, issue_rest, 0)

    def weights(m, p):
        if m < 3:
            return pltpu.bitcast(wt_ref[p * 3 + m], BF16)
        return pltpu.bitcast(w_ref[pl.ds(p * PW // 2, PW // 2), :], BF16)

    def transposed(w):
        return w.T if TB else w.astype(F32).T.astype(BF16)

    def weights_nn(c0, c1):
        return pltpu.bitcast(wn_ref[:, c0 * PW:c1 * PW], BF16)

    scale = DH ** -0.5
    ninf = -jnp.inf

    def softmax2(s, sel, allowed):
        s = jnp.where(allowed, s, -1e9 / scale)
        m0 = jnp.max(jnp.where(sel, s, ninf), axis=-1, keepdims=True)
        m1 = jnp.max(jnp.where(sel, ninf, s), axis=-1, keepdims=True)
        e = jnp.exp2((s - jnp.where(sel, m0, m1)) * (scale * LOG2E))
        e0, e1 = jnp.where(sel, e, 0.0), jnp.where(sel, 0.0, e)
        d0 = jnp.sum(e0, axis=-1, keepdims=True)
        d1 = jnp.sum(e1, axis=-1, keepdims=True)
        return e, e0, e1, pl.reciprocal(d0, approx=True), pl.reciprocal(d1, approx=True)

    def masks(rows):
        qi = lax.broadcasted_iota(jnp.int32, (rows, R), 0)
        ki = lax.broadcasted_iota(jnp.int32, (rows, R), 1)
        first = ki < L
        kk = jnp.where(first, ki, ki - L)
        qq = M + ((qi - 2 * M) & (SEG - 1))
        allowed = (qi < 2 * M) | (kk <= qq)
        return qi, first, allowed

    def attn_two_layers():
        qi, first, allowed = masks(R)
        row_l1 = (qi < M) | ((qi >= 2 * M) & (qi < R1))
        is_a = first == row_l1
        lo = lax.broadcasted_iota(jnp.int32, (L, 128), 1) < 64

        def arrange(a):
            a1 = _cat0(a[0:M], a[2 * M:R1])
            a2 = _cat0(a[M:2 * M], a[R1:])
            cat = lambda u, w: _cat0(u, w).astype(BF16)
            m1, m2 = a1[:, 128:256], a2[:, 128:256]
            return (cat(a1[:, :128], a2[:, :128]), cat(a2[:, 256:], a1[:, 256:]),
                    cat(jnp.where(lo, m1, 0.0), jnp.where(lo, 0.0, m1)),
                    cat(jnp.where(lo, 0.0, m2), jnp.where(lo, m2, 0.0)))

        g1 = lambda a: a[0:R1]
        g2 = lambda a: _cat0(a[0:2 * M], a[R1:])
        merge = lambda u1, u2: _cat0(u1[0:M], u2[M:2 * M], u1[2 * M:], u2[2 * M:])

        def arrange_q(q):
            qm = q[:, 128:256]
            return [u.astype(BF16) for u in (q[:, :128], q[:, 256:], g1(qm), g2(qm))]

        def scores(q, kt):
            order = (2, 3, 0, 1) if MIDFIRST & 1 else (0, 1, 2, 3)
            r = {i: _nt(q[i], kt[i]) for i in order}
            return [r[i] for i in range(4)]

        lo_r = lax.broadcasted_iota(jnp.int32, (R, 128), 1) < 64

        def pv(s4, vt):
            sa, sb, s1, s2 = s4
            p, pa, pb, ra, rb = softmax2(jnp.where(is_a, sa, sb) + merge(s1, s2), is_a, allowed)
            if MIDFIRST & 2:
                om = merge(_nn(g1(p).astype(BF16), vt[2]), _nn(g2(p).astype(BF16), vt[3]))
                oa, ob = _nn(pa.astype(BF16), vt[0]), _nn(pb.astype(BF16), vt[1])
            else:
                oa, ob = _nn(pa.astype(BF16), vt[0]), _nn(pb.astype(BF16), vt[1])
                om = merge(_nn(g1(p).astype(BF16), vt[2]), _nn(g2(p).astype(BF16), vt[3]))
            return jnp.concatenate(
                [oa * ra, om * jnp.where(lo_r, ra, rb), ob * rb], axis=1).astype(BF16)

        return arrange_q, arrange, scores, pv

    def attn_one_layer():
        _, first, allowed = masks(R1)
        head_a = lax.broadcasted_iota(jnp.int32, (L, PW), 1) < DH

        def arrange(a):
            a1 = _cat0(a[0:M], a[2 * M:])
            return _cat0(jnp.where(head_a, a1, 0.0), jnp.where(head_a, 0.0, a1)).astype(BF16)

        head_a1 = lax.broadcasted_iota(jnp.int32, (R1, PW), 1) < DH

        def pv(s, vt):
            p, _, _, r0, r1 = softmax2(s, first, allowed)
            return (_nn(p.astype(BF16), vt) * jnp.where(head_a1, r0, r1)).astype(BF16)

        return lambda q: q.astype(BF16), arrange, _nt, pv

    def a_phase(h, attn, hooks, t=None):
        arrange_q, arrange, scores, pv = attn

        def proj(m, p):
            c = p * 3 + m
            if c >= NPRE or t is None:
                return _nn(h, weights(m, p))
            y = _nn(_cat0(h[0:2 * M], h[R1:]), weights(m, p))
            pre = pre_ref[pl.ds(al(t * SEG, SEG), SEG), c * PW:(c + 1) * PW].astype(F32)
            return _cat0(y[0:2 * M], pre, y[2 * M:])

        proj_o = lambda o, p: _nn(o, weights(3, p))
        st = {'acc': None, 'o': {}, 'done': 0}

        def wo_upto(n):
            while st['done'] < n:
                pp = st['done']
                y = proj_o(st['o'].pop(pp), pp)
                st['acc'] = y if st['acc'] is None else st['acc'] + y
                st['done'] += 1

        q, kt = arrange_q(proj(0, 0)), arrange(proj(1, 0))
        vts = {0: arrange(proj(2, 0))}
        lim = NPAIR - 1 - HELD
        for p in range(NPAIR):
            last = p == NPAIR - 1
            for op in (ORDER_LAST if last else ORDER):
                if op == 'S':
                    s = scores(q, kt)
                    hooks(p - 0.5)
                elif op == 'Q':
                    qn = arrange_q(proj(0, p + 1))
                elif op == 'K':
                    ktn = arrange(proj(1, p + 1))
                elif op == 'V':
                    vts[p + 1] = arrange(proj(2, p + 1))
                elif op == 'P':
                    hooks(p)
                    st['o'][p] = pv(s, vts.pop(p))
                elif op == 'W':
                    wo_upto(p + 1 if last else min(p + 1, lim))
                elif op == 'w':
                    wo_upto(p if last else min(p, lim))
                elif op == 'x':
                    wo_upto(p - 1)
            q, kt = qn, ktn
        return st['acc']

    def b_phase1(t, layers=(0, 1)):
        w = jnp.concatenate([_cat0(*[pltpu.bitcast(pwqkv_ref[j * NC + c], BF16) for c in range(NC)])
                             for j in range(3)], axis=1)
        l0 = layers[0]
        qkv = _nn(_ln(xb_ref[l0 * SEG:(layers[-1] + 1) * SEG, :]).astype(BF16), w)
        for l in layers:
            rows = slice((l - l0) * SEG, (l - l0 + 1) * SEG)
            for c in range(NC):
                bq_ref[c, l * SEG:(l + 1) * SEG, :] = qkv[rows, c * 128:(c + 1) * 128]
                for j in range(2):
                    bkv_ref[l, j, c, 0:16, :] = bkv_ref[l, j, c, SEG:SEG + 16, :]
                    bkv_ref[l, j, c, 16:16 + SEG, :] = qkv[
                        rows, (j + 1) * D + c * 128:(j + 1) * D + (c + 1) * 128]
        bscale = BDH ** -0.5
        ri8 = lax.broadcasted_iota(jnp.int32, (8, 128), 0)
        for l in layers:
            seg = t - 1 - 2 * l
            for r in range(SEG // 8):
                pos = seg * SEG + r * 8 + ri8
                q = [bq_ref[c, l * SEG + r * 8:l * SEG + r * 8 + 8, :] for c in range(NC)]
                lg = []
                for w in range(BW):
                    o0 = 16 + r * 8 - BDIL * w
                    s = q[0] * bkv_ref[l, 0, 0, o0:o0 + 8, :]
                    for c in range(1, NC):
                        s = s + q[c] * bkv_ref[l, 0, c, o0:o0 + 8, :]
                    s = s + pltpu.roll(s, 64, 1)
                    s = s + pltpu.roll(s, 32, 1)
                    if r * 8 - BDIL * w < 0:
                        s = jnp.where(pos - BDIL * w >= 0, s, -1e9 / bscale)
                    lg.append(s)
                m = lg[0]
                for w in range(1, BW):
                    m = jnp.maximum(m, lg[w])
                e = [jnp.exp2((s - m) * (bscale * LOG2E)) for s in lg]
                den = e[0]
                for w in range(1, BW):
                    den = den + e[w]
                inv = pl.reciprocal(den, approx=True)
                for c in range(NC):
                    o = e[0] * bkv_ref[l, 1, c, 16 + r * 8:16 + r * 8 + 8, :]
                    for w in range(1, BW):
                        o0 = 16 + r * 8 - BDIL * w
                        o = o + e[w] * bkv_ref[l, 1, c, o0:o0 + 8, :]
                    bq_ref[c, l * SEG + r * 8:l * SEG + r * 8 + 8, :] = o * inv

    def b_phase2(t, layers=(0, 1)):
        rows = slice(layers[0] * SEG, (layers[-1] + 1) * SEG)
        w = jnp.concatenate([pltpu.bitcast(pwo_ref[c], BF16) for c in range(NC)], axis=1)
        o = jnp.concatenate([bq_ref[c, rows, :] for c in range(NC)], axis=1).astype(BF16)
        yb = xb_ref[rows, :] + _nn(o, w)
        if 1 in layers:
            row = al(max(t - 3, 0) * SEG if isinstance(t, int) else jnp.maximum(t - 3, 0) * SEG, SEG)
            out_ref[pl.ds(row, SEG), :] = yb[-SEG:].astype(out_ref.dtype)
        return yb[:SEG]

    def x_seg(s):
        row = s * SEG if isinstance(s, int) else pl.multiple_of(s * SEG, SEG)
        return x_ref[pl.ds(row, SEG), :].astype(F32)

    def with_b(t):
        box = {}

        def hooks(p):
            if p == BQKV_AT - 0.5:
                b_phase1(t)
            elif p == BWO_PAIR and BWO2_PAIR == BWO_PAIR:
                box['x2'] = b_phase2(t)
            elif p == BWO_PAIR:
                box['x2'] = b_phase2(t, (0,))
            elif p == BWO2_PAIR:
                b_phase2(t, (1,))
        return hooks, box

    def prepare_next(t, x2):
        sn = jnp.minimum(t + 1, NSEG - 1)
        hx_ref[0:SEG, :] = hxa_ref[pl.ds(al(sn * SEG, SEG), SEG), :]
        hx_ref[SEG:, :] = _ln(x2).astype(BF16)
        res_ref[...] = _cat0(x_seg(sn), x2)

    def permuted_rows(c):
        rows = [st_ref[c, pl.ds(d, H, stride=BDH), :] for d in range(BDH)]
        return _cat0(*rows)

    mem0 = mem0_ref[...].astype(F32)
    mem_ref[...] = _cat0(mem0, mem0)
    bkv_ref[...] = jnp.zeros(bkv_ref.shape, F32)
    acc_ref[...] = jnp.zeros(acc_ref.shape, F32)
    eye = (lax.broadcasted_iota(jnp.int32, (128, 128), 0)
           == lax.broadcasted_iota(jnp.int32, (128, 128), 1)).astype(F32).astype(BF16)
    first[0].wait()
    xl0 = _ln(x_ref[0:X0 + XB, :].astype(F32)).astype(BF16)
    hxa_ref[0:X0 + XB, :] = xl0
    hx_ref[0:SEG, :] = xl0[0:SEG]
    for u in range(NPRE):
        first[1 + u].wait()
        w = wl_ref[u % 3, (u // 3) * PW:(u // 3 + 1) * PW, :]
        for c in range(NC):
            wc = w[:, c * 128:(c + 1) * 128]
            y = (wc.astype(F32).T if XT & 4 else _nt(eye, wc)).astype(BF16)
            wn_ref[c * 64:(c + 1) * 64, u * PW:(u + 1) * PW] = pltpu.bitcast(y, U32)
        pre_ref[2 * SEG:X0, u * PW:(u + 1) * PW] = _nt(hxa_ref[2 * SEG:X0, :], w).astype(BF16)

    def step0(p, carry):
        group(p, lambda cp: cp.wait())
        u = jnp.minimum(p, NU - 1)

        def wfirst(m):
            w = wl_ref[m, pl.ds(al(p * PW, 128), PW), :]
            if m < 3:
                w = _cat0(*[transposed(w[:, c * 128:(c + 1) * 128]) for c in range(NC)])
                wt_ref[p * 3 + m] = pltpu.bitcast(w, U32)
                return weights(m, p) if RELOAD else w
            w_ref[pl.ds(al(p * (PW // 2), 64), PW // 2), :] = pltpu.bitcast(w, U32)
            return w

        _, arrange, scores, pv = attn_one_layer()
        h = _cat0(mem_ref[...].astype(BF16), hx_ref[0:SEG, :])
        xrows = x_rows(p)
        xl = hxa_ref[xrows, :]
        for c in range(NC):
            st_ref[0, c * 128:(c + 1) * 128, :] = bwqkv_ref[u, :, c * 128:(c + 1) * 128].astype(F32).T
        pwqkv_ref[u] = pltpu.bitcast(permuted_rows(0).T.astype(BF16), U32)
        done = [0]

        def pre(n):
            c0, c1 = done[0], min(done[0] + n, NPRE)
            done[0] = c1
            if c1 > c0:
                pre_ref[xrows, c0 * PW:c1 * PW] = _nn(xl, weights_nn(c0, c1)).astype(BF16)

        pre(S0[0])
        q = _nn(h, wfirst(0)).astype(BF16)
        pre(S0[1])
        kt = arrange(_nn(h, wfirst(1)))
        pre(S0[2])
        s = scores(q, kt)
        pre(S0[3])
        vt = arrange(_nn(h, wfirst(2)))
        pre(S0[4])
        o = pv(s, vt)
        pre(NPRE)
        acc_ref[...] += _nn(o, wfirst(3))
        nrows = x_rows(u + 1)
        hxa_ref[nrows, :] = _ln(x_ref[nrows, :].astype(F32)).astype(BF16)
        issue_rest(p + WIN, 0)

        return carry

    lax.fori_loop(0, NPAIR, step0, 0)
    bw2.wait()
    for c in range(NC):
        st_ref[c] = bwo_ref[:, c * 128:(c + 1) * 128].astype(F32)
        pwo_ref[c] = pltpu.bitcast(permuted_rows(c).astype(BF16), U32)
    zeros = jnp.zeros((SEG, D), F32)
    mem_ref[0:M, :] = acc_ref[0:M, :]
    xb_ref[...] = _cat0(x_seg(0) + acc_ref[2 * M:, :], zeros)
    prepare_next(0, zeros)

    def single(t, carry):
        @pl.when(t == NSEG + 1)
        def _():
            out_a.start()

        l = (t >= NSEG).astype(jnp.int32)
        mrows = pl.ds(al(l * M, M), M)
        xrows = pl.ds(al(l * SEG, SEG), SEG)
        hooks, box = with_b(t)
        mem = mem_ref[mrows, :]
        h = _cat0(_cat0(mem, mem).astype(BF16), hx_ref[xrows, :])
        acc = a_phase(h, attn_one_layer(), hooks)
        mem_ref[mrows, :] = acc[:M]
        xb_ref[xrows, :] = res_ref[xrows, :] + acc[2 * M:]
        prepare_next(t, box['x2'])
        return carry

    def step(t, carry):
        hooks, box = with_b(t)
        h = _cat0(mem_ref[...].astype(BF16), hx_ref[...])
        acc = a_phase(h, attn_two_layers(), hooks, t)
        mem_ref[...] = acc[:2 * M]
        xb_ref[...] = res_ref[...] + acc[2 * M:]
        prepare_next(t, box['x2'])
        return carry

    def outer(i, carry):
        lax.fori_loop(1 + (NSEG - 1) * i, 2 + NSEG * i, single, 0)
        lax.fori_loop(2, NSEG - (NSEG - 2) * i, step, 0)
        return carry

    lax.fori_loop(0, 2, outer, 0)
    b_phase1(NSEG + 2, (1,))
    b_phase2(NSEG + 2, (1,))
    out_b.start()
    out_a.wait()
    out_b.wait()


@jax.jit
def pallas_interleave_layers__memory_aug_recurrent_mem_tr__sliding_local_dilated__prompt_kernel(
    A_x, A_mem0, A_Wq, A_Wk, A_Wv, A_Wo, A_seg_len, B_x, B_wqkv, B_wo,
):
    del A_seg_len, B_x
    wt = lambda w: jnp.transpose(w, (1, 2, 0)).reshape(HD, D)
    vm = pl.BlockSpec(memory_space=pltpu.VMEM)
    hbm = pl.BlockSpec(memory_space=pl.ANY)
    out = pl.pallas_call(
        _kernel,
        out_shape=jax.ShapeDtypeStruct((S, D), A_x.dtype),
        in_specs=[hbm, vm, hbm, hbm, hbm, hbm, hbm, hbm],
        out_specs=hbm,
        scratch_shapes=[
            pltpu.VMEM((S, D), BF16),
            pltpu.VMEM((S, D), BF16),
            pltpu.VMEM((4, HD, D), BF16),
            pltpu.VMEM((HD // 2, D), U32),
            pltpu.VMEM((3 * NPAIR, D // 2, PW), U32),
            pltpu.VMEM((NU, 128, D), BF16),
            pltpu.VMEM((D, D), BF16),
            pltpu.VMEM((NU, 64, D), U32),
            pltpu.VMEM((NC, D // 2, 128), U32),
            pltpu.VMEM((NC, D, 128), F32),
            pltpu.VMEM((R1, D), F32),
            pltpu.VMEM((2 * M, D), F32),
            pltpu.VMEM((2 * SEG, D), BF16),
            pltpu.VMEM((2 * SEG, D), F32),
            pltpu.VMEM((2 * SEG, D), F32),
            pltpu.VMEM((NC, 2 * SEG, 128), F32),
            pltpu.VMEM((2, 2, NC, 16 + SEG, 128), F32),
            pltpu.VMEM((D // 2, NPRE * PW), U32),
            pltpu.VMEM((S, D), BF16),
            pltpu.VMEM((S, NPRE * PW), BF16),
            pltpu.SemaphoreType.DMA((NPRE + 1,)),
            pltpu.SemaphoreType.DMA((NPAIR,)),
            pltpu.SemaphoreType.DMA((3,)),
        ],
        compiler_params=pltpu.CompilerParams(vmem_limit_bytes=120 * 2 ** 20),
    )(A_x.reshape(S, D), A_mem0.reshape(M, D), wt(A_Wq), wt(A_Wk), wt(A_Wv),
      A_Wo.reshape(HD, D), B_wqkv, B_wo)
    return out.reshape(1, S, D)
```

```python
import jax
import jax.numpy as jnp
from jax import lax
import jax.experimental.pallas as pl
import jax.experimental.pallas.tpu as pltpu

S, D = 2048, 640
H, DH = 32, 192
HD = H * DH
M, SEG = 8, 32
L = M + SEG
NSEG = S // SEG
R = 2 * L
R1 = 2 * M + SEG
PW = 2 * DH
NPAIR = H // 2
BDH, BW, BDIL = 20, 8, 2
NC = D // 128
XB = 112
X0 = S - NPAIR * XB
NPRE = 8
XT = 7
TB = 1
RELOAD = 0
S0 = (2, 1, 1, 2, 1)
BQKV_AT = 0
F32, BF16, U32 = jnp.float32, jnp.bfloat16, jnp.uint32
NT = (((1,), (1,)), ((), ()))
LOG2E = 1.4426950408889634
NU = 3 * NC
WIN = 4
ORDER = 'SQKPVW'
ORDER_LAST = 'SxPwW'
MIDFIRST = 3
HELD = 2
BWO2_PAIR = 10
BWO_PAIR = 10


def _ln(x):
    m = jnp.mean(x, axis=-1, keepdims=True)
    xc = x - m
    v = jnp.mean(xc * xc, axis=-1, keepdims=True)
    return xc * lax.rsqrt(v + 1e-5)


def _nt(a, b):
    return lax.dot_general(a, b, NT, preferred_element_type=F32)


def _nn(a, b):
    return jnp.dot(a, b, preferred_element_type=F32)


def _cat0(*a):
    return jnp.concatenate(a, axis=0)


def _kernel(x_hbm, mem0_hbm, wq_hbm, wk_hbm, wv_hbm, wo_hbm, bwqkv_hbm, bwo_hbm,
            out_hbm,
            x_ref, out_ref, wl_ref, w_ref, wt_ref, bwqkv_ref, bwo_ref, pwqkv_ref, pwo_ref,
            st_ref, acc_ref, mem_ref, hx_ref, res_ref, xb_ref, bq_ref, bkv_ref, wn_ref, hxa_ref, pre_ref, mem0_ref, qsem, wsem, sem):
    def al(v, n):
        return v if isinstance(v, int) else pl.multiple_of(v, n)

    w_hbm = (wq_hbm, wk_hbm, wv_hbm, wo_hbm)

    def w_copy(m, p, s):
        rows = pl.ds(al(p * PW, 128), PW)
        return pltpu.make_async_copy(w_hbm[m].at[rows, :], wl_ref.at[m, rows, :], s)

    def x_rows(p):
        return pl.ds(al(X0 + p * XB, 16), XB)

    def x_copy(p):
        return pltpu.make_async_copy(x_hbm.at[x_rows(p + 1), :], x_ref.at[x_rows(p + 1), :], wsem.at[p])

    first = [pltpu.make_async_copy(x_hbm.at[pl.ds(0, X0 + XB), :], x_ref.at[pl.ds(0, X0 + XB), :], qsem.at[NPRE])] + [
        w_copy(c % 3, c // 3, qsem.at[c]) for c in range(NPRE)]

    def unit_copy(u):
        src = bwqkv_hbm.at[pl.ds(al((u % NC) * 128, 128), 128), pl.ds(al((u // NC) * D, 128), D)]
        return pltpu.make_async_copy(src, bwqkv_ref.at[u], wsem.at[u])

    bw2 = pltpu.make_async_copy(bwo_hbm, bwo_ref, sem.at[3])
    mem0_copy = pltpu.make_async_copy(mem0_hbm, mem0_ref, sem.at[0])
    osplit = (NSEG - 2) * SEG
    out_a = pltpu.make_async_copy(out_ref.at[pl.ds(0, osplit), :], out_hbm.at[pl.ds(0, osplit), :], sem.at[1])
    out_b = pltpu.make_async_copy(out_ref.at[pl.ds(osplit, S - osplit), :],
                                  out_hbm.at[pl.ds(osplit, S - osplit), :], sem.at[2])

    def issue_first(i, carry):
        for j, cp in enumerate(first):
            pl.when(i == j)(cp.start)
        return carry

    def group(p, act):
        for m in range(3):
            pl.when((p * 3 + m >= NPRE) & (p < NPAIR))(lambda m=m: act(w_copy(m, p, wsem.at[p])))

        @pl.when(p < NPAIR - 1)
        def _():
            act(unit_copy(p))
            act(x_copy(p))

        pl.when(p < NPAIR)(lambda: act(w_copy(3, p, wsem.at[p])))

    def issue_rest(p, carry):
        group(p, lambda cp: cp.start())
        pl.when(p == NPAIR)(bw2.start)
        return carry

    lax.fori_loop(0, len(first), issue_first, 0)
    mem0_copy.start()
    lax.fori_loop(0, WIN, issue_rest, 0)

    def weights(m, p):
        if m < 3:
            return pltpu.bitcast(wt_ref[p * 3 + m], BF16)
        return pltpu.bitcast(w_ref[pl.ds(p * PW // 2, PW // 2), :], BF16)

    def transposed(w):
        return w.T if TB else w.astype(F32).T.astype(BF16)

    def weights_nn(c0, c1):
        return pltpu.bitcast(wn_ref[:, c0 * PW:c1 * PW], BF16)

    scale = DH ** -0.5
    ninf = -jnp.inf

    def softmax2(s, sel, allowed):
        s = jnp.where(allowed, s, -1e9 / scale)
        m0 = jnp.max(jnp.where(sel, s, ninf), axis=-1, keepdims=True)
        m1 = jnp.max(jnp.where(sel, ninf, s), axis=-1, keepdims=True)
        e = jnp.exp2((s - jnp.where(sel, m0, m1)) * (scale * LOG2E))
        e0, e1 = jnp.where(sel, e, 0.0), jnp.where(sel, 0.0, e)
        d0 = jnp.sum(e0, axis=-1, keepdims=True)
        d1 = jnp.sum(e1, axis=-1, keepdims=True)
        return e, e0, e1, pl.reciprocal(d0, approx=True), pl.reciprocal(d1, approx=True)

    def masks(rows):
        qi = lax.broadcasted_iota(jnp.int32, (rows, R), 0)
        ki = lax.broadcasted_iota(jnp.int32, (rows, R), 1)
        first = ki < L
        kk = jnp.where(first, ki, ki - L)
        qq = M + ((qi - 2 * M) & (SEG - 1))
        allowed = (qi < 2 * M) | (kk <= qq)
        return qi, first, allowed

    def attn_two_layers():
        qi, first, allowed = masks(R)
        row_l1 = (qi < M) | ((qi >= 2 * M) & (qi < R1))
        is_a = first == row_l1
        lo = lax.broadcasted_iota(jnp.int32, (L, 128), 1) < 64

        def arrange(a):
            a1 = _cat0(a[0:M], a[2 * M:R1])
            a2 = _cat0(a[M:2 * M], a[R1:])
            cat = lambda u, w: _cat0(u, w).astype(BF16)
            m1, m2 = a1[:, 128:256], a2[:, 128:256]
            return (cat(a1[:, :128], a2[:, :128]), cat(a2[:, 256:], a1[:, 256:]),
                    cat(jnp.where(lo, m1, 0.0), jnp.where(lo, 0.0, m1)),
                    cat(jnp.where(lo, 0.0, m2), jnp.where(lo, m2, 0.0)))

        g1 = lambda a: a[0:R1]
        g2 = lambda a: _cat0(a[0:2 * M], a[R1:])
        merge = lambda u1, u2: _cat0(u1[0:M], u2[M:2 * M], u1[2 * M:], u2[2 * M:])

        def arrange_q(q):
            qm = q[:, 128:256]
            return [u.astype(BF16) for u in (q[:, :128], q[:, 256:], g1(qm), g2(qm))]

        def scores(q, kt):
            order = (2, 3, 0, 1) if MIDFIRST & 1 else (0, 1, 2, 3)
            r = {i: _nt(q[i], kt[i]) for i in order}
            return [r[i] for i in range(4)]

        lo_r = lax.broadcasted_iota(jnp.int32, (R, 128), 1) < 64

        def pv(s4, vt):
            sa, sb, s1, s2 = s4
            p, pa, pb, ra, rb = softmax2(jnp.where(is_a, sa, sb) + merge(s1, s2), is_a, allowed)
            if MIDFIRST & 2:
                om = merge(_nn(g1(p).astype(BF16), vt[2]), _nn(g2(p).astype(BF16), vt[3]))
                oa, ob = _nn(pa.astype(BF16), vt[0]), _nn(pb.astype(BF16), vt[1])
            else:
                oa, ob = _nn(pa.astype(BF16), vt[0]), _nn(pb.astype(BF16), vt[1])
                om = merge(_nn(g1(p).astype(BF16), vt[2]), _nn(g2(p).astype(BF16), vt[3]))
            return jnp.concatenate(
                [oa * ra, om * jnp.where(lo_r, ra, rb), ob * rb], axis=1).astype(BF16)

        return arrange_q, arrange, scores, pv

    def attn_one_layer():
        _, first, allowed = masks(R1)
        head_a = lax.broadcasted_iota(jnp.int32, (L, PW), 1) < DH

        def arrange(a):
            a1 = _cat0(a[0:M], a[2 * M:])
            return _cat0(jnp.where(head_a, a1, 0.0), jnp.where(head_a, 0.0, a1)).astype(BF16)

        head_a1 = lax.broadcasted_iota(jnp.int32, (R1, PW), 1) < DH

        def pv(s, vt):
            p, _, _, r0, r1 = softmax2(s, first, allowed)
            return (_nn(p.astype(BF16), vt) * jnp.where(head_a1, r0, r1)).astype(BF16)

        return lambda q: q.astype(BF16), arrange, _nt, pv

    def a_phase(h, attn, hooks, t=None):
        arrange_q, arrange, scores, pv = attn

        def proj(m, p):
            c = p * 3 + m
            if c >= NPRE or t is None:
                return _nn(h, weights(m, p))
            y = _nn(_cat0(h[0:2 * M], h[R1:]), weights(m, p))
            pre = pre_ref[pl.ds(al(t * SEG, SEG), SEG), c * PW:(c + 1) * PW].astype(F32)
            return _cat0(y[0:2 * M], pre, y[2 * M:])

        proj_o = lambda o, p: _nn(o, weights(3, p))
        st = {'acc': None, 'o': {}, 'done': 0}

        def wo_upto(n):
            while st['done'] < n:
                pp = st['done']
                y = proj_o(st['o'].pop(pp), pp)
                st['acc'] = y if st['acc'] is None else st['acc'] + y
                st['done'] += 1

        q, kt = arrange_q(proj(0, 0)), arrange(proj(1, 0))
        vts = {0: arrange(proj(2, 0))}
        lim = NPAIR - 1 - HELD
        for p in range(NPAIR):
            last = p == NPAIR - 1
            for op in (ORDER_LAST if last else ORDER):
                if op == 'S':
                    s = scores(q, kt)
                    hooks(p - 0.5)
                elif op == 'Q':
                    qn = arrange_q(proj(0, p + 1))
                elif op == 'K':
                    ktn = arrange(proj(1, p + 1))
                elif op == 'V':
                    vts[p + 1] = arrange(proj(2, p + 1))
                elif op == 'P':
                    hooks(p)
                    st['o'][p] = pv(s, vts.pop(p))
                elif op == 'W':
                    wo_upto(p + 1 if last else min(p + 1, lim))
                elif op == 'w':
                    wo_upto(p if last else min(p, lim))
                elif op == 'x':
                    wo_upto(p - 1)
            q, kt = qn, ktn
        return st['acc']

    def b_phase1(t, layers=(0, 1)):
        w = jnp.concatenate([_cat0(*[pltpu.bitcast(pwqkv_ref[j * NC + c], BF16) for c in range(NC)])
                             for j in range(3)], axis=1)
        l0 = layers[0]
        qkv = _nn(_ln(xb_ref[l0 * SEG:(layers[-1] + 1) * SEG, :]).astype(BF16), w)
        for l in layers:
            rows = slice((l - l0) * SEG, (l - l0 + 1) * SEG)
            for c in range(NC):
                bq_ref[c, l * SEG:(l + 1) * SEG, :] = qkv[rows, c * 128:(c + 1) * 128]
                for j in range(2):
                    bkv_ref[l, j, c, 0:16, :] = bkv_ref[l, j, c, SEG:SEG + 16, :]
                    bkv_ref[l, j, c, 16:16 + SEG, :] = qkv[
                        rows, (j + 1) * D + c * 128:(j + 1) * D + (c + 1) * 128]
        bscale = BDH ** -0.5
        ri8 = lax.broadcasted_iota(jnp.int32, (8, 128), 0)
        for l in layers:
            seg = t - 1 - 2 * l
            for r in range(SEG // 8):
                pos = seg * SEG + r * 8 + ri8
                q = [bq_ref[c, l * SEG + r * 8:l * SEG + r * 8 + 8, :] for c in range(NC)]
                lg = []
                for w in range(BW):
                    o0 = 16 + r * 8 - BDIL * w
                    s = q[0] * bkv_ref[l, 0, 0, o0:o0 + 8, :]
                    for c in range(1, NC):
                        s = s + q[c] * bkv_ref[l, 0, c, o0:o0 + 8, :]
                    s = s + pltpu.roll(s, 64, 1)
                    s = s + pltpu.roll(s, 32, 1)
                    if r * 8 - BDIL * w < 0:
                        s = jnp.where(pos - BDIL * w >= 0, s, -1e9 / bscale)
                    lg.append(s)
                m = lg[0]
                for w in range(1, BW):
                    m = jnp.maximum(m, lg[w])
                e = [jnp.exp2((s - m) * (bscale * LOG2E)) for s in lg]
                den = e[0]
                for w in range(1, BW):
                    den = den + e[w]
                inv = pl.reciprocal(den, approx=True)
                for c in range(NC):
                    o = e[0] * bkv_ref[l, 1, c, 16 + r * 8:16 + r * 8 + 8, :]
                    for w in range(1, BW):
                        o0 = 16 + r * 8 - BDIL * w
                        o = o + e[w] * bkv_ref[l, 1, c, o0:o0 + 8, :]
                    bq_ref[c, l * SEG + r * 8:l * SEG + r * 8 + 8, :] = o * inv

    def b_phase2(t, layers=(0, 1)):
        rows = slice(layers[0] * SEG, (layers[-1] + 1) * SEG)
        w = jnp.concatenate([pltpu.bitcast(pwo_ref[c], BF16) for c in range(NC)], axis=1)
        o = jnp.concatenate([bq_ref[c, rows, :] for c in range(NC)], axis=1).astype(BF16)
        yb = xb_ref[rows, :] + _nn(o, w)
        if 1 in layers:
            row = al(max(t - 3, 0) * SEG if isinstance(t, int) else jnp.maximum(t - 3, 0) * SEG, SEG)
            out_ref[pl.ds(row, SEG), :] = yb[-SEG:].astype(out_ref.dtype)
        return yb[:SEG]

    def x_seg(s):
        row = s * SEG if isinstance(s, int) else pl.multiple_of(s * SEG, SEG)
        return x_ref[pl.ds(row, SEG), :].astype(F32)

    def with_b(t):
        box = {}

        def hooks(p):
            if p == BQKV_AT - 0.5:
                b_phase1(t)
            elif p == BWO_PAIR and BWO2_PAIR == BWO_PAIR:
                box['x2'] = b_phase2(t)
            elif p == BWO_PAIR:
                box['x2'] = b_phase2(t, (0,))
            elif p == BWO2_PAIR:
                b_phase2(t, (1,))
        return hooks, box

    def prepare_next(t, x2):
        sn = jnp.minimum(t + 1, NSEG - 1)
        hx_ref[0:SEG, :] = hxa_ref[pl.ds(al(sn * SEG, SEG), SEG), :]
        hx_ref[SEG:, :] = _ln(x2).astype(BF16)
        res_ref[...] = _cat0(x_seg(sn), x2)

    def permuted_rows(c):
        rows = [st_ref[c, pl.ds(d, H, stride=BDH), :] for d in range(BDH)]
        return _cat0(*rows)

    bkv_ref[...] = jnp.zeros(bkv_ref.shape, F32)
    acc_ref[...] = jnp.zeros(acc_ref.shape, F32)
    eye = (lax.broadcasted_iota(jnp.int32, (128, 128), 0)
           == lax.broadcasted_iota(jnp.int32, (128, 128), 1)).astype(F32).astype(BF16)
    first[0].wait()
    xl0 = _ln(x_ref[0:X0 + XB, :].astype(F32)).astype(BF16)
    hxa_ref[0:X0 + XB, :] = xl0
    hx_ref[0:SEG, :] = xl0[0:SEG]
    for u in range(NPRE):
        first[1 + u].wait()
        w = wl_ref[u % 3, (u // 3) * PW:(u // 3 + 1) * PW, :]
        for c in range(NC):
            wc = w[:, c * 128:(c + 1) * 128]
            y = (wc.astype(F32).T if XT & 4 else _nt(eye, wc)).astype(BF16)
            wn_ref[c * 64:(c + 1) * 64, u * PW:(u + 1) * PW] = pltpu.bitcast(y, U32)
        pre_ref[2 * SEG:X0, u * PW:(u + 1) * PW] = _nt(hxa_ref[2 * SEG:X0, :], w).astype(BF16)

    mem0_copy.wait()
    mem0 = mem0_ref[...].astype(F32)
    mem_ref[...] = _cat0(mem0, mem0)

    def step0(p, carry):
        group(p, lambda cp: cp.wait())
        u = jnp.minimum(p, NU - 1)

        def wfirst(m):
            w = wl_ref[m, pl.ds(al(p * PW, 128), PW), :]
            if m < 3:
                w = _cat0(*[transposed(w[:, c * 128:(c + 1) * 128]) for c in range(NC)])
                wt_ref[p * 3 + m] = pltpu.bitcast(w, U32)
                return weights(m, p) if RELOAD else w
            w_ref[pl.ds(al(p * (PW // 2), 64), PW // 2), :] = pltpu.bitcast(w, U32)
            return w

        _, arrange, scores, pv = attn_one_layer()
        h = _cat0(mem_ref[...].astype(BF16), hx_ref[0:SEG, :])
        xrows = x_rows(p)
        xl = hxa_ref[xrows, :]
        for c in range(NC):
            st_ref[0, c * 128:(c + 1) * 128, :] = bwqkv_ref[u, :, c * 128:(c + 1) * 128].astype(F32).T
        pwqkv_ref[u] = pltpu.bitcast(permuted_rows(0).T.astype(BF16), U32)
        done = [0]

        def pre(n):
            c0, c1 = done[0], min(done[0] + n, NPRE)
            done[0] = c1
            if c1 > c0:
                pre_ref[xrows, c0 * PW:c1 * PW] = _nn(xl, weights_nn(c0, c1)).astype(BF16)

        pre(S0[0])
        q = _nn(h, wfirst(0)).astype(BF16)
        pre(S0[1])
        kt = arrange(_nn(h, wfirst(1)))
        pre(S0[2])
        s = scores(q, kt)
        pre(S0[3])
        vt = arrange(_nn(h, wfirst(2)))
        pre(S0[4])
        o = pv(s, vt)
        pre(NPRE)
        acc_ref[...] += _nn(o, wfirst(3))
        nrows = x_rows(u + 1)
        hxa_ref[nrows, :] = _ln(x_ref[nrows, :].astype(F32)).astype(BF16)
        issue_rest(p + WIN, 0)

        return carry

    lax.fori_loop(0, NPAIR, step0, 0)
    bw2.wait()
    for c in range(NC):
        st_ref[c] = bwo_ref[:, c * 128:(c + 1) * 128].astype(F32)
        pwo_ref[c] = pltpu.bitcast(permuted_rows(c).astype(BF16), U32)
    zeros = jnp.zeros((SEG, D), F32)
    mem_ref[0:M, :] = acc_ref[0:M, :]
    xb_ref[...] = _cat0(x_seg(0) + acc_ref[2 * M:, :], zeros)
    hx_ref[...] = _cat0(hxa_ref[SEG:2 * SEG, :], zeros.astype(BF16))
    res_ref[...] = _cat0(x_seg(1), zeros)

    def single(t, carry):
        @pl.when(t == NSEG + 1)
        def _():
            out_a.start()

        l = (t >= NSEG).astype(jnp.int32)
        mrows = pl.ds(al(l * M, M), M)
        xrows = pl.ds(al(l * SEG, SEG), SEG)
        hooks, box = with_b(t)
        mem = mem_ref[mrows, :]
        h = _cat0(_cat0(mem, mem).astype(BF16), hx_ref[xrows, :])
        acc = a_phase(h, attn_one_layer(), hooks)
        mem_ref[mrows, :] = acc[:M]
        xb_ref[xrows, :] = res_ref[xrows, :] + acc[2 * M:]
        prepare_next(t, box['x2'])
        return carry

    def step(t, carry):
        hooks, box = with_b(t)
        h = _cat0(mem_ref[...].astype(BF16), hx_ref[...])
        acc = a_phase(h, attn_two_layers(), hooks, t)
        mem_ref[...] = acc[:2 * M]
        xb_ref[...] = res_ref[...] + acc[2 * M:]
        prepare_next(t, box['x2'])
        return carry

    def outer(i, carry):
        lax.fori_loop(1 + (NSEG - 1) * i, 2 + NSEG * i, single, 0)
        lax.fori_loop(2, NSEG - (NSEG - 2) * i, step, 0)
        return carry

    lax.fori_loop(0, 2, outer, 0)
    b_phase1(NSEG + 2, (1,))
    b_phase2(NSEG + 2, (1,))
    out_b.start()
    out_a.wait()
    out_b.wait()


@jax.jit
def pallas_interleave_layers__memory_aug_recurrent_mem_tr__sliding_local_dilated__prompt_kernel(
    A_x, A_mem0, A_Wq, A_Wk, A_Wv, A_Wo, A_seg_len, B_x, B_wqkv, B_wo,
):
    del A_seg_len, B_x
    wt = lambda w: jnp.transpose(w, (1, 2, 0)).reshape(HD, D)
    hbm = pl.BlockSpec(memory_space=pl.ANY)
    out = pl.pallas_call(
        _kernel,
        out_shape=jax.ShapeDtypeStruct((S, D), A_x.dtype),
        in_specs=[hbm] * 8,
        out_specs=hbm,
        scratch_shapes=[
            pltpu.VMEM((S, D), BF16),
            pltpu.VMEM((S, D), BF16),
            pltpu.VMEM((4, HD, D), BF16),
            pltpu.VMEM((HD // 2, D), U32),
            pltpu.VMEM((3 * NPAIR, D // 2, PW), U32),
            pltpu.VMEM((NU, 128, D), BF16),
            pltpu.VMEM((D, D), BF16),
            pltpu.VMEM((NU, 64, D), U32),
            pltpu.VMEM((NC, D // 2, 128), U32),
            pltpu.VMEM((NC, D, 128), F32),
            pltpu.VMEM((R1, D), F32),
            pltpu.VMEM((2 * M, D), F32),
            pltpu.VMEM((2 * SEG, D), BF16),
            pltpu.VMEM((2 * SEG, D), F32),
            pltpu.VMEM((2 * SEG, D), F32),
            pltpu.VMEM((NC, 2 * SEG, 128), F32),
            pltpu.VMEM((2, 2, NC, 16 + SEG, 128), F32),
            pltpu.VMEM((D // 2, NPRE * PW), U32),
            pltpu.VMEM((S, D), BF16),
            pltpu.VMEM((S, NPRE * PW), BF16),
            pltpu.VMEM((M, D), BF16),
            pltpu.SemaphoreType.DMA((NPRE + 1,)),
            pltpu.SemaphoreType.DMA((NPAIR,)),
            pltpu.SemaphoreType.DMA((4,)),
        ],
        compiler_params=pltpu.CompilerParams(vmem_limit_bytes=120 * 2 ** 20),
    )(A_x.reshape(S, D), A_mem0.reshape(M, D), wt(A_Wq), wt(A_Wk), wt(A_Wv),
      A_Wo.reshape(HD, D), B_wqkv, B_wo)
    return out.reshape(1, S, D)
```

```python
import jax
import jax.numpy as jnp
from jax import lax
import jax.experimental.pallas as pl
import jax.experimental.pallas.tpu as pltpu

S, D = 2048, 640
H, DH = 32, 192
HD = H * DH
M, SEG = 8, 32
L = M + SEG
NSEG = S // SEG
R = 2 * L
R1 = 2 * M + SEG
PW = 2 * DH
NPAIR = H // 2
BDH, BW, BDIL = 20, 8, 2
NC = D // 128
XB = 112
X0 = S - NPAIR * XB
NPRE = 8
XT = 7
TB = 1
RELOAD = 0
S0 = (2, 1, 1, 2, 1)
BQKV_AT = 0
F32, BF16, U32 = jnp.float32, jnp.bfloat16, jnp.uint32
NT = (((1,), (1,)), ((), ()))
LOG2E = 1.4426950408889634
NU = 3 * NC
WIN = 4
ORDER = 'SQKPVW'
ORDER_LAST = 'SxPwW'
MIDFIRST = 3
HELD = 2
UNROLL = 2
BWO2_PAIR = 16
BWO_PAIR = 8


def _ln(x):
    m = jnp.mean(x, axis=-1, keepdims=True)
    xc = x - m
    v = jnp.mean(xc * xc, axis=-1, keepdims=True)
    return xc * lax.rsqrt(v + 1e-5)


def _nt(a, b):
    return lax.dot_general(a, b, NT, preferred_element_type=F32)


def _nn(a, b):
    return jnp.dot(a, b, preferred_element_type=F32)


def _cat0(*a):
    return jnp.concatenate(a, axis=0)


def _kernel(x_hbm, mem0_hbm, wq_hbm, wk_hbm, wv_hbm, wo_hbm, bwqkv_hbm, bwo_hbm,
            out_hbm,
            x_ref, out_ref, wl_ref, w_ref, wt_ref, bwqkv_ref, bwo_ref, pwqkv_ref, pwo_ref,
            st_ref, acc_ref, mem_ref, hx_ref, res_ref, xb_ref, bq_ref, bkv_ref, wn_ref, hxa_ref, pre_ref, mem0_ref, qsem, wsem, sem):
    def al(v, n):
        return v if isinstance(v, int) else pl.multiple_of(v, n)

    w_hbm = (wq_hbm, wk_hbm, wv_hbm, wo_hbm)

    def w_copy(m, p, s):
        rows = pl.ds(al(p * PW, 128), PW)
        return pltpu.make_async_copy(w_hbm[m].at[rows, :], wl_ref.at[m, rows, :], s)

    def x_rows(p):
        return pl.ds(al(X0 + p * XB, 16), XB)

    def x_copy(p):
        return pltpu.make_async_copy(x_hbm.at[x_rows(p + 1), :], x_ref.at[x_rows(p + 1), :], wsem.at[p])

    first = [pltpu.make_async_copy(x_hbm.at[pl.ds(0, X0 + XB), :], x_ref.at[pl.ds(0, X0 + XB), :], qsem.at[NPRE])] + [
        w_copy(c % 3, c // 3, qsem.at[c]) for c in range(NPRE)]

    def unit_copy(u):
        src = bwqkv_hbm.at[pl.ds(al((u % NC) * 128, 128), 128), pl.ds(al((u // NC) * D, 128), D)]
        return pltpu.make_async_copy(src, bwqkv_ref.at[u], wsem.at[u])

    bw2 = pltpu.make_async_copy(bwo_hbm, bwo_ref, sem.at[3])
    mem0_copy = pltpu.make_async_copy(mem0_hbm, mem0_ref, sem.at[0])
    osplit = (NSEG - 3) * SEG
    out_a = pltpu.make_async_copy(out_ref.at[pl.ds(0, osplit), :], out_hbm.at[pl.ds(0, osplit), :], sem.at[1])
    out_b = pltpu.make_async_copy(out_ref.at[pl.ds(osplit, S - osplit), :],
                                  out_hbm.at[pl.ds(osplit, S - osplit), :], sem.at[2])

    def issue_first(i, carry):
        for j, cp in enumerate(first):
            pl.when(i == j)(cp.start)
        return carry

    def group(p, act):
        for m in range(3):
            pl.when((p * 3 + m >= NPRE) & (p < NPAIR))(lambda m=m: act(w_copy(m, p, wsem.at[p])))

        @pl.when(p < NPAIR - 1)
        def _():
            act(unit_copy(p))
            act(x_copy(p))

        pl.when(p < NPAIR)(lambda: act(w_copy(3, p, wsem.at[p])))

    def issue_rest(p, carry):
        group(p, lambda cp: cp.start())
        pl.when(p == NPAIR)(bw2.start)
        return carry

    lax.fori_loop(0, len(first), issue_first, 0)
    mem0_copy.start()
    lax.fori_loop(0, WIN, issue_rest, 0)

    def weights(m, p):
        if m < 3:
            return pltpu.bitcast(wt_ref[p * 3 + m], BF16)
        return pltpu.bitcast(w_ref[pl.ds(p * PW // 2, PW // 2), :], BF16)

    def transposed(w):
        return w.T if TB else w.astype(F32).T.astype(BF16)


    scale = DH ** -0.5
    ninf = -jnp.inf

    def softmax2(s, sel, allowed):
        s = jnp.where(allowed, s, -1e9 / scale)
        m0 = jnp.max(jnp.where(sel, s, ninf), axis=-1, keepdims=True)
        m1 = jnp.max(jnp.where(sel, ninf, s), axis=-1, keepdims=True)
        e = jnp.exp2((s - jnp.where(sel, m0, m1)) * (scale * LOG2E))
        e0, e1 = jnp.where(sel, e, 0.0), jnp.where(sel, 0.0, e)
        d0 = jnp.sum(e0, axis=-1, keepdims=True)
        d1 = jnp.sum(e1, axis=-1, keepdims=True)
        return e, e0, e1, pl.reciprocal(d0, approx=True), pl.reciprocal(d1, approx=True)

    def masks(rows):
        qi = lax.broadcasted_iota(jnp.int32, (rows, R), 0)
        ki = lax.broadcasted_iota(jnp.int32, (rows, R), 1)
        first = ki < L
        kk = jnp.where(first, ki, ki - L)
        qq = M + ((qi - 2 * M) & (SEG - 1))
        allowed = (qi < 2 * M) | (kk <= qq)
        return qi, first, allowed

    def attn_two_layers():
        qi, first, allowed = masks(R)
        row_l1 = (qi < M) | ((qi >= 2 * M) & (qi < R1))
        is_a = first == row_l1
        lo = lax.broadcasted_iota(jnp.int32, (L, 128), 1) < 64

        def arrange(a):
            a1 = _cat0(a[0:M], a[2 * M:R1])
            a2 = _cat0(a[M:2 * M], a[R1:])
            cat = lambda u, w: _cat0(u, w).astype(BF16)
            m1, m2 = a1[:, 128:256], a2[:, 128:256]
            return (cat(a1[:, :128], a2[:, :128]), cat(a2[:, 256:], a1[:, 256:]),
                    cat(jnp.where(lo, m1, 0.0), jnp.where(lo, 0.0, m1)),
                    cat(jnp.where(lo, 0.0, m2), jnp.where(lo, m2, 0.0)))

        g1 = lambda a: a[0:R1]
        g2 = lambda a: _cat0(a[0:2 * M], a[R1:])
        merge = lambda u1, u2: _cat0(u1[0:M], u2[M:2 * M], u1[2 * M:], u2[2 * M:])

        def arrange_q(q):
            qm = q[:, 128:256]
            return [u.astype(BF16) for u in (q[:, :128], q[:, 256:], g1(qm), g2(qm))]

        def scores(q, kt):
            order = (2, 3, 0, 1) if MIDFIRST & 1 else (0, 1, 2, 3)
            r = {i: _nt(q[i], kt[i]) for i in order}
            return [r[i] for i in range(4)]

        lo_r = lax.broadcasted_iota(jnp.int32, (R, 128), 1) < 64

        def pv(s4, vt):
            sa, sb, s1, s2 = s4
            p, pa, pb, ra, rb = softmax2(jnp.where(is_a, sa, sb) + merge(s1, s2), is_a, allowed)
            if MIDFIRST & 2:
                om = merge(_nn(g1(p).astype(BF16), vt[2]), _nn(g2(p).astype(BF16), vt[3]))
                oa, ob = _nn(pa.astype(BF16), vt[0]), _nn(pb.astype(BF16), vt[1])
            else:
                oa, ob = _nn(pa.astype(BF16), vt[0]), _nn(pb.astype(BF16), vt[1])
                om = merge(_nn(g1(p).astype(BF16), vt[2]), _nn(g2(p).astype(BF16), vt[3]))
            return jnp.concatenate(
                [oa * ra, om * jnp.where(lo_r, ra, rb), ob * rb], axis=1).astype(BF16)

        return arrange_q, arrange, scores, pv

    def attn_one_layer():
        _, first, allowed = masks(R1)
        head_a = lax.broadcasted_iota(jnp.int32, (L, PW), 1) < DH

        def arrange(a):
            a1 = _cat0(a[0:M], a[2 * M:])
            return _cat0(jnp.where(head_a, a1, 0.0), jnp.where(head_a, 0.0, a1)).astype(BF16)

        head_a1 = lax.broadcasted_iota(jnp.int32, (R1, PW), 1) < DH

        def pv(s, vt):
            p, _, _, r0, r1 = softmax2(s, first, allowed)
            return (_nn(p.astype(BF16), vt) * jnp.where(head_a1, r0, r1)).astype(BF16)

        return lambda q: q.astype(BF16), arrange, _nt, pv

    def a_phase(h, attn, hooks, t=None):
        arrange_q, arrange, scores, pv = attn

        def proj(m, p):
            c = p * 3 + m
            if c >= NPRE or t is None:
                return _nn(h, weights(m, p))
            y = _nn(_cat0(h[0:2 * M], h[R1:]), weights(m, p))
            pre = pre_ref[c, pl.ds(al(t * SEG, SEG), SEG), :].astype(F32)
            return _cat0(y[0:2 * M], pre, y[2 * M:])

        proj_o = lambda o, p: _nn(o, weights(3, p))
        st = {'acc': None, 'o': {}, 'done': 0}

        def wo_upto(n):
            while st['done'] < n:
                pp = st['done']
                y = proj_o(st['o'].pop(pp), pp)
                st['acc'] = y if st['acc'] is None else st['acc'] + y
                st['done'] += 1

        q, kt = arrange_q(proj(0, 0)), arrange(proj(1, 0))
        vts = {0: arrange(proj(2, 0))}
        lim = NPAIR - 1 - HELD
        for p in range(NPAIR):
            last = p == NPAIR - 1
            for op in (ORDER_LAST if last else ORDER):
                if op == 'S':
                    s = scores(q, kt)
                    hooks(p - 0.5)
                elif op == 'Q':
                    qn = arrange_q(proj(0, p + 1))
                elif op == 'K':
                    ktn = arrange(proj(1, p + 1))
                elif op == 'V':
                    vts[p + 1] = arrange(proj(2, p + 1))
                elif op == 'P':
                    hooks(p)
                    st['o'][p] = pv(s, vts.pop(p))
                elif op == 'W':
                    wo_upto(p + 1 if last else min(p + 1, lim))
                elif op == 'w':
                    wo_upto(p if last else min(p, lim))
                elif op == 'x':
                    wo_upto(p - 1)
            q, kt = qn, ktn
        hooks(NPAIR)
        return st['acc']

    def b_phase1(t, layers=(0, 1)):
        w = jnp.concatenate([_cat0(*[pltpu.bitcast(pwqkv_ref[j * NC + c], BF16) for c in range(NC)])
                             for j in range(3)], axis=1)
        l0 = layers[0]
        qkv = _nn(_ln(xb_ref[l0 * SEG:(layers[-1] + 1) * SEG, :]).astype(BF16), w)
        for l in layers:
            rows = slice((l - l0) * SEG, (l - l0 + 1) * SEG)
            for c in range(NC):
                bq_ref[c, l * SEG:(l + 1) * SEG, :] = qkv[rows, c * 128:(c + 1) * 128]
                for j in range(2):
                    bkv_ref[l, j, c, 0:16, :] = bkv_ref[l, j, c, SEG:SEG + 16, :]
                    bkv_ref[l, j, c, 16:16 + SEG, :] = qkv[
                        rows, (j + 1) * D + c * 128:(j + 1) * D + (c + 1) * 128]
        bscale = BDH ** -0.5
        ri8 = lax.broadcasted_iota(jnp.int32, (8, 128), 0)
        for l in layers:
            seg = t - 1 - 2 * l
            for r in range(SEG // 8):
                pos = seg * SEG + r * 8 + ri8
                q = [bq_ref[c, l * SEG + r * 8:l * SEG + r * 8 + 8, :] for c in range(NC)]
                lg = []
                for w in range(BW):
                    o0 = 16 + r * 8 - BDIL * w
                    s = q[0] * bkv_ref[l, 0, 0, o0:o0 + 8, :]
                    for c in range(1, NC):
                        s = s + q[c] * bkv_ref[l, 0, c, o0:o0 + 8, :]
                    s = s + pltpu.roll(s, 64, 1)
                    s = s + pltpu.roll(s, 32, 1)
                    if r * 8 - BDIL * w < 0:
                        s = jnp.where(pos - BDIL * w >= 0, s, -1e9 / bscale)
                    lg.append(s)
                m = lg[0]
                for w in range(1, BW):
                    m = jnp.maximum(m, lg[w])
                e = [jnp.exp2((s - m) * (bscale * LOG2E)) for s in lg]
                den = e[0]
                for w in range(1, BW):
                    den = den + e[w]
                inv = pl.reciprocal(den, approx=True)
                for c in range(NC):
                    o = e[0] * bkv_ref[l, 1, c, 16 + r * 8:16 + r * 8 + 8, :]
                    for w in range(1, BW):
                        o0 = 16 + r * 8 - BDIL * w
                        o = o + e[w] * bkv_ref[l, 1, c, o0:o0 + 8, :]
                    bq_ref[c, l * SEG + r * 8:l * SEG + r * 8 + 8, :] = o * inv

    def b_phase2(t, layers=(0, 1)):
        rows = slice(layers[0] * SEG, (layers[-1] + 1) * SEG)
        w = jnp.concatenate([pltpu.bitcast(pwo_ref[c], BF16) for c in range(NC)], axis=1)
        o = jnp.concatenate([bq_ref[c, rows, :] for c in range(NC)], axis=1).astype(BF16)
        yb = xb_ref[rows, :] + _nn(o, w)
        if 1 in layers:
            row = al(max(t - 3, 0) * SEG if isinstance(t, int) else jnp.maximum(t - 3, 0) * SEG, SEG)
            out_ref[pl.ds(row, SEG), :] = yb[-SEG:].astype(out_ref.dtype)
        return yb[:SEG]

    def x_seg(s):
        row = s * SEG if isinstance(s, int) else pl.multiple_of(s * SEG, SEG)
        return x_ref[pl.ds(row, SEG), :].astype(F32)

    def with_b(t):
        box = {}

        def hooks(p):
            if p == BQKV_AT - 0.5:
                b_phase1(t)
            elif p == BWO_PAIR and BWO2_PAIR == BWO_PAIR:
                box['x2'] = b_phase2(t)
            elif p == BWO_PAIR:
                box['x2'] = b_phase2(t, (0,))
            elif p == BWO2_PAIR:
                b_phase2(t, (1,))
        return hooks, box

    def prepare_next(t, x2):
        sn = jnp.minimum(t + 1, NSEG - 1)
        hx_ref[0:SEG, :] = hxa_ref[pl.ds(al(sn * SEG, SEG), SEG), :]
        hx_ref[SEG:, :] = _ln(x2).astype(BF16)
        res_ref[...] = _cat0(x_seg(sn), x2)

    def permuted_rows(c):
        rows = [st_ref[c, pl.ds(d, H, stride=BDH), :] for d in range(BDH)]
        return _cat0(*rows)

    bkv_ref[...] = jnp.zeros(bkv_ref.shape, F32)
    acc_ref[...] = jnp.zeros(acc_ref.shape, F32)
    first[0].wait()
    xl0 = _ln(x_ref[0:X0 + XB, :].astype(F32)).astype(BF16)
    hxa_ref[0:X0 + XB, :] = xl0
    hx_ref[0:SEG, :] = xl0[0:SEG]

    def early(u, carry):
        rows = pl.ds(al((u // 3) * PW, 128), PW)
        pltpu.make_async_copy(wq_hbm.at[rows, :], wl_ref.at[u % 3, rows, :], qsem.at[u]).wait()
        w = wl_ref[u % 3, rows, :]
        wn_ref[u] = pltpu.bitcast(_cat0(*[transposed(w[:, c * 128:(c + 1) * 128]) for c in range(NC)]), U32)
        pre_ref[u, 2 * SEG:X0, :] = _nt(hxa_ref[2 * SEG:X0, :], w).astype(BF16)
        return carry

    lax.fori_loop(0, NPRE, early, 0)
    mem0_copy.wait()
    mem0 = mem0_ref[...].astype(F32)
    mem_ref[...] = _cat0(mem0, mem0)

    def step0(p, carry):
        group(p, lambda cp: cp.wait())
        u = jnp.minimum(p, NU - 1)

        def wfirst(m):
            w = wl_ref[m, pl.ds(al(p * PW, 128), PW), :]
            if m < 3:
                w = _cat0(*[transposed(w[:, c * 128:(c + 1) * 128]) for c in range(NC)])
                wt_ref[p * 3 + m] = pltpu.bitcast(w, U32)
                return weights(m, p) if RELOAD else w
            w_ref[pl.ds(al(p * (PW // 2), 64), PW // 2), :] = pltpu.bitcast(w, U32)
            return w

        _, arrange, scores, pv = attn_one_layer()
        h = _cat0(mem_ref[...].astype(BF16), hx_ref[0:SEG, :])
        xrows = x_rows(p)
        xl = hxa_ref[xrows, :]
        for c in range(NC):
            st_ref[0, c * 128:(c + 1) * 128, :] = bwqkv_ref[u, :, c * 128:(c + 1) * 128].astype(F32).T
        pwqkv_ref[u] = pltpu.bitcast(permuted_rows(0).T.astype(BF16), U32)
        done = [0]

        def pre(n):
            c0, c1 = done[0], min(done[0] + n, NPRE)
            done[0] = c1
            for c in range(c0, c1):
                pre_ref[c, xrows, :] = _nn(xl, pltpu.bitcast(wn_ref[c], BF16)).astype(BF16)

        pre(S0[0])
        q = _nn(h, wfirst(0)).astype(BF16)
        pre(S0[1])
        kt = arrange(_nn(h, wfirst(1)))
        pre(S0[2])
        s = scores(q, kt)
        pre(S0[3])
        vt = arrange(_nn(h, wfirst(2)))
        pre(S0[4])
        o = pv(s, vt)
        pre(NPRE)
        acc_ref[...] += _nn(o, wfirst(3))
        nrows = x_rows(u + 1)
        hxa_ref[nrows, :] = _ln(x_ref[nrows, :].astype(F32)).astype(BF16)
        issue_rest(p + WIN, 0)

        return carry

    lax.fori_loop(0, NPAIR, step0, 0)
    bw2.wait()
    for c in range(NC):
        st_ref[c] = bwo_ref[:, c * 128:(c + 1) * 128].astype(F32)
        pwo_ref[c] = pltpu.bitcast(permuted_rows(c).astype(BF16), U32)
    zeros = jnp.zeros((SEG, D), F32)
    mem_ref[0:M, :] = acc_ref[0:M, :]
    xb_ref[...] = _cat0(x_seg(0) + acc_ref[2 * M:, :], zeros)
    hx_ref[...] = _cat0(hxa_ref[SEG:2 * SEG, :], zeros.astype(BF16))
    res_ref[...] = _cat0(x_seg(1), zeros)

    def single(t, carry):
        l = (t >= NSEG).astype(jnp.int32)
        mrows = pl.ds(al(l * M, M), M)
        xrows = pl.ds(al(l * SEG, SEG), SEG)
        hooks, box = with_b(t)
        mem = mem_ref[mrows, :]
        h = _cat0(_cat0(mem, mem).astype(BF16), hx_ref[xrows, :])
        acc = a_phase(h, attn_one_layer(), hooks)
        mem_ref[mrows, :] = acc[:M]
        xb_ref[xrows, :] = res_ref[xrows, :] + acc[2 * M:]
        prepare_next(t, box['x2'])
        return carry

    def step(i, carry):
        for j in range(UNROLL):
            step1(i * UNROLL + j)
        return carry

    def step1(t):
        hooks, box = with_b(t)
        h = _cat0(mem_ref[...].astype(BF16), hx_ref[...])
        acc = a_phase(h, attn_two_layers(), hooks, t)
        mem_ref[...] = acc[:2 * M]
        xb_ref[...] = res_ref[...] + acc[2 * M:]
        prepare_next(t, box['x2'])

    def outer(i, carry):
        lax.fori_loop(1 + (NSEG - 1) * i, 2 + NSEG * i, single, 0)
        lax.fori_loop(2 // UNROLL, (NSEG - (NSEG - 2) * i) // UNROLL, step, 0)
        pl.when(i == 0)(out_a.start)
        return carry

    lax.fori_loop(0, 2, outer, 0)
    b_phase1(NSEG + 2, (1,))
    b_phase2(NSEG + 2, (1,))
    out_b.start()
    out_a.wait()
    out_b.wait()


@jax.jit
def pallas_interleave_layers__memory_aug_recurrent_mem_tr__sliding_local_dilated__prompt_kernel(
    A_x, A_mem0, A_Wq, A_Wk, A_Wv, A_Wo, A_seg_len, B_x, B_wqkv, B_wo,
):
    del A_seg_len, B_x
    wt = lambda w: jnp.transpose(w, (1, 2, 0)).reshape(HD, D)
    hbm = pl.BlockSpec(memory_space=pl.ANY)
    out = pl.pallas_call(
        _kernel,
        out_shape=jax.ShapeDtypeStruct((S, D), A_x.dtype),
        in_specs=[hbm] * 8,
        out_specs=hbm,
        scratch_shapes=[
            pltpu.VMEM((S, D), BF16),
            pltpu.VMEM((S, D), BF16),
            pltpu.VMEM((4, HD, D), BF16),
            pltpu.VMEM((HD // 2, D), U32),
            pltpu.VMEM((3 * NPAIR, D // 2, PW), U32),
            pltpu.VMEM((NU, 128, D), BF16),
            pltpu.VMEM((D, D), BF16),
            pltpu.VMEM((NU, 64, D), U32),
            pltpu.VMEM((NC, D // 2, 128), U32),
            pltpu.VMEM((NC, D, 128), F32),
            pltpu.VMEM((R1, D), F32),
            pltpu.VMEM((2 * M, D), F32),
            pltpu.VMEM((2 * SEG, D), BF16),
            pltpu.VMEM((2 * SEG, D), F32),
            pltpu.VMEM((2 * SEG, D), F32),
            pltpu.VMEM((NC, 2 * SEG, 128), F32),
            pltpu.VMEM((2, 2, NC, 16 + SEG, 128), F32),
            pltpu.VMEM((NPRE, D // 2, PW), U32),
            pltpu.VMEM((S, D), BF16),
            pltpu.VMEM((NPRE, S, PW), BF16),
            pltpu.VMEM((M, D), BF16),
            pltpu.SemaphoreType.DMA((NPRE + 1,)),
            pltpu.SemaphoreType.DMA((NPAIR,)),
            pltpu.SemaphoreType.DMA((4,)),
        ],
        compiler_params=pltpu.CompilerParams(vmem_limit_bytes=120 * 2 ** 20),
    )(A_x.reshape(S, D), A_mem0.reshape(M, D), wt(A_Wq), wt(A_Wk), wt(A_Wv),
      A_Wo.reshape(HD, D), B_wqkv, B_wo)
    return out.reshape(1, S, D)
```

```python
import jax
import jax.numpy as jnp
from jax import lax
import jax.experimental.pallas as pl
import jax.experimental.pallas.tpu as pltpu

S, D = 2048, 640
H, DH = 32, 192
HD = H * DH
M, SEG = 8, 32
L = M + SEG
NSEG = S // SEG
R = 2 * L
R1 = 2 * M + SEG
PW = 2 * DH
NPAIR = H // 2
BDH, BW, BDIL = 20, 8, 2
NC = D // 128
XB = 112
X0 = S - NPAIR * XB
NPRE = 8
XT = 7
TB = 1
RELOAD = 0
S0 = (2, 1, 1, 2, 1)
BQKV_AT = 0
F32, BF16, U32 = jnp.float32, jnp.bfloat16, jnp.uint32
NT = (((1,), (1,)), ((), ()))
LOG2E = 1.4426950408889634
NU = 3 * NC
WIN = 4
ORDER = 'SQKPVW'
ORDER_LAST = 'SxPwW'
MIDFIRST = 0
HELD = 2
UNROLL = 2
SB = (0, 15, 15)
SHELD = 2
BWO2_PAIR = 16
BWO_PAIR = 8


def _ln(x):
    m = jnp.mean(x, axis=-1, keepdims=True)
    xc = x - m
    v = jnp.mean(xc * xc, axis=-1, keepdims=True)
    return xc * lax.rsqrt(v + 1e-5)


def _nt(a, b):
    return lax.dot_general(a, b, NT, preferred_element_type=F32)


def _nn(a, b):
    return jnp.dot(a, b, preferred_element_type=F32)


def _cat0(*a):
    return jnp.concatenate(a, axis=0)


def _kernel(x_hbm, mem0_hbm, wq_hbm, wk_hbm, wv_hbm, wo_hbm, bwqkv_hbm, bwo_hbm,
            out_hbm,
            x_ref, out_ref, wl_ref, w_ref, wt_ref, bwqkv_ref, bwo_ref, pwqkv_ref, pwo_ref,
            st_ref, acc_ref, mem_ref, hx_ref, res_ref, xb_ref, bq_ref, bkv_ref, wn_ref, hxa_ref, pre_ref, mem0_ref, qsem, wsem, sem):
    def al(v, n):
        return v if isinstance(v, int) else pl.multiple_of(v, n)

    w_hbm = (wq_hbm, wk_hbm, wv_hbm, wo_hbm)

    def w_copy(m, p, s):
        rows = pl.ds(al(p * PW, 128), PW)
        return pltpu.make_async_copy(w_hbm[m].at[rows, :], wl_ref.at[m, rows, :], s)

    def x_rows(p):
        return pl.ds(al(X0 + p * XB, 16), XB)

    def x_copy(p):
        return pltpu.make_async_copy(x_hbm.at[x_rows(p + 1), :], x_ref.at[x_rows(p + 1), :], wsem.at[p])

    first = [pltpu.make_async_copy(x_hbm.at[pl.ds(0, X0 + XB), :], x_ref.at[pl.ds(0, X0 + XB), :], qsem.at[NPRE])] + [
        w_copy(c % 3, c // 3, qsem.at[c]) for c in range(NPRE)]

    def unit_copy(u):
        src = bwqkv_hbm.at[pl.ds(al((u % NC) * 128, 128), 128), pl.ds(al((u // NC) * D, 128), D)]
        return pltpu.make_async_copy(src, bwqkv_ref.at[u], wsem.at[u])

    bw2 = pltpu.make_async_copy(bwo_hbm, bwo_ref, sem.at[3])
    mem0_copy = pltpu.make_async_copy(mem0_hbm, mem0_ref, sem.at[0])
    osplit = (NSEG - 3) * SEG
    out_a = pltpu.make_async_copy(out_ref.at[pl.ds(0, osplit), :], out_hbm.at[pl.ds(0, osplit), :], sem.at[1])
    out_b = pltpu.make_async_copy(out_ref.at[pl.ds(osplit, S - osplit), :],
                                  out_hbm.at[pl.ds(osplit, S - osplit), :], sem.at[2])

    def issue_first(i, carry):
        for j, cp in enumerate(first):
            pl.when(i == j)(cp.start)
        return carry

    def group(p, act):
        for m in range(3):
            pl.when((p * 3 + m >= NPRE) & (p < NPAIR))(lambda m=m: act(w_copy(m, p, wsem.at[p])))

        @pl.when(p < NPAIR - 1)
        def _():
            act(unit_copy(p))
            act(x_copy(p))

        pl.when(p < NPAIR)(lambda: act(w_copy(3, p, wsem.at[p])))

    def issue_rest(p, carry):
        group(p, lambda cp: cp.start())
        pl.when(p == NPAIR)(bw2.start)
        return carry

    lax.fori_loop(0, len(first), issue_first, 0)
    mem0_copy.start()
    lax.fori_loop(0, WIN, issue_rest, 0)

    def weights(m, p):
        if m < 3:
            return pltpu.bitcast(wt_ref[p * 3 + m], BF16)
        return pltpu.bitcast(w_ref[pl.ds(p * PW // 2, PW // 2), :], BF16)

    def transposed(w):
        return w.T if TB else w.astype(F32).T.astype(BF16)


    scale = DH ** -0.5
    ninf = -jnp.inf

    def softmax2(s, sel, allowed):
        s = jnp.where(allowed, s, -1e9 / scale)
        m0 = jnp.max(jnp.where(sel, s, ninf), axis=-1, keepdims=True)
        m1 = jnp.max(jnp.where(sel, ninf, s), axis=-1, keepdims=True)
        e = jnp.exp2((s - jnp.where(sel, m0, m1)) * (scale * LOG2E))
        e0, e1 = jnp.where(sel, e, 0.0), jnp.where(sel, 0.0, e)
        d0 = jnp.sum(e0, axis=-1, keepdims=True)
        d1 = jnp.sum(e1, axis=-1, keepdims=True)
        return e, e0, e1, pl.reciprocal(d0, approx=True), pl.reciprocal(d1, approx=True)

    def masks(rows):
        qi = lax.broadcasted_iota(jnp.int32, (rows, R), 0)
        ki = lax.broadcasted_iota(jnp.int32, (rows, R), 1)
        first = ki < L
        kk = jnp.where(first, ki, ki - L)
        qq = M + ((qi - 2 * M) & (SEG - 1))
        allowed = (qi < 2 * M) | (kk <= qq)
        return qi, first, allowed

    def attn_two_layers():
        qi, first, allowed = masks(R)
        row_l1 = (qi < M) | ((qi >= 2 * M) & (qi < R1))
        is_a = first == row_l1
        lo = lax.broadcasted_iota(jnp.int32, (L, 128), 1) < 64

        def arrange(a):
            a1 = _cat0(a[0:M], a[2 * M:R1])
            a2 = _cat0(a[M:2 * M], a[R1:])
            cat = lambda u, w: _cat0(u, w).astype(BF16)
            m1, m2 = a1[:, 128:256], a2[:, 128:256]
            return (cat(a1[:, :128], a2[:, :128]), cat(a2[:, 256:], a1[:, 256:]),
                    cat(jnp.where(lo, m1, 0.0), jnp.where(lo, 0.0, m1)),
                    cat(jnp.where(lo, 0.0, m2), jnp.where(lo, m2, 0.0)))

        g1 = lambda a: a[0:R1]
        g2 = lambda a: _cat0(a[0:2 * M], a[R1:])
        merge = lambda u1, u2: _cat0(u1[0:M], u2[M:2 * M], u1[2 * M:], u2[2 * M:])

        def arrange_q(q):
            qm = q[:, 128:256]
            return [u.astype(BF16) for u in (q[:, :128], q[:, 256:], g1(qm), g2(qm))]

        def scores(q, kt):
            order = (2, 3, 0, 1) if MIDFIRST & 1 else (0, 1, 2, 3)
            r = {i: _nt(q[i], kt[i]) for i in order}
            return [r[i] for i in range(4)]

        lo_r = lax.broadcasted_iota(jnp.int32, (R, 128), 1) < 64

        def pv(s4, vt):
            sa, sb, s1, s2 = s4
            p, pa, pb, ra, rb = softmax2(jnp.where(is_a, sa, sb) + merge(s1, s2), is_a, allowed)
            if MIDFIRST & 2:
                om = merge(_nn(g1(p).astype(BF16), vt[2]), _nn(g2(p).astype(BF16), vt[3]))
                oa, ob = _nn(pa.astype(BF16), vt[0]), _nn(pb.astype(BF16), vt[1])
            else:
                oa, ob = _nn(pa.astype(BF16), vt[0]), _nn(pb.astype(BF16), vt[1])
                om = merge(_nn(g1(p).astype(BF16), vt[2]), _nn(g2(p).astype(BF16), vt[3]))
            return jnp.concatenate(
                [oa * ra, om * jnp.where(lo_r, ra, rb), ob * rb], axis=1).astype(BF16)

        return arrange_q, arrange, scores, pv

    def attn_one_layer():
        _, first, allowed = masks(R1)
        head_a = lax.broadcasted_iota(jnp.int32, (L, PW), 1) < DH

        def arrange(a):
            a1 = _cat0(a[0:M], a[2 * M:])
            return _cat0(jnp.where(head_a, a1, 0.0), jnp.where(head_a, 0.0, a1)).astype(BF16)

        head_a1 = lax.broadcasted_iota(jnp.int32, (R1, PW), 1) < DH

        def pv(s, vt):
            p, _, _, r0, r1 = softmax2(s, first, allowed)
            return (_nn(p.astype(BF16), vt) * jnp.where(head_a1, r0, r1)).astype(BF16)

        return lambda q: q.astype(BF16), arrange, _nt, pv

    def a_phase(h, attn, hooks, t=None):
        arrange_q, arrange, scores, pv = attn

        def proj(m, p):
            c = p * 3 + m
            if c >= NPRE or t is None:
                return _nn(h, weights(m, p))
            y = _nn(_cat0(h[0:2 * M], h[R1:]), weights(m, p))
            pre = pre_ref[c, pl.ds(al(t * SEG, SEG), SEG), :].astype(F32)
            return _cat0(y[0:2 * M], pre, y[2 * M:])

        proj_o = lambda o, p: _nn(o, weights(3, p))
        st = {'acc': None, 'o': {}, 'done': 0}

        def wo_upto(n):
            while st['done'] < n:
                pp = st['done']
                y = proj_o(st['o'].pop(pp), pp)
                st['acc'] = y if st['acc'] is None else st['acc'] + y
                st['done'] += 1

        q, kt = arrange_q(proj(0, 0)), arrange(proj(1, 0))
        vts = {0: arrange(proj(2, 0))}
        lim = NPAIR - 1 - (SHELD if t is None else HELD)
        for p in range(NPAIR):
            last = p == NPAIR - 1
            for op in (ORDER_LAST if last else ORDER):
                if op == 'S':
                    s = scores(q, kt)
                    hooks(p - 0.5)
                elif op == 'Q':
                    qn = arrange_q(proj(0, p + 1))
                elif op == 'K':
                    ktn = arrange(proj(1, p + 1))
                elif op == 'V':
                    vts[p + 1] = arrange(proj(2, p + 1))
                elif op == 'P':
                    hooks(p)
                    st['o'][p] = pv(s, vts.pop(p))
                elif op == 'W':
                    wo_upto(p + 1 if last else min(p + 1, lim))
                elif op == 'w':
                    wo_upto(p if last else min(p, lim))
                elif op == 'x':
                    wo_upto(p - 1)
            q, kt = qn, ktn
        hooks(NPAIR)
        return st['acc']

    def b_phase1(t, layers=(0, 1)):
        w = jnp.concatenate([_cat0(*[pltpu.bitcast(pwqkv_ref[j * NC + c], BF16) for c in range(NC)])
                             for j in range(3)], axis=1)
        l0 = layers[0]
        qkv = _nn(_ln(xb_ref[l0 * SEG:(layers[-1] + 1) * SEG, :]).astype(BF16), w)
        for l in layers:
            rows = slice((l - l0) * SEG, (l - l0 + 1) * SEG)
            for c in range(NC):
                bq_ref[c, l * SEG:(l + 1) * SEG, :] = qkv[rows, c * 128:(c + 1) * 128]
                for j in range(2):
                    bkv_ref[l, j, c, 0:16, :] = bkv_ref[l, j, c, SEG:SEG + 16, :]
                    bkv_ref[l, j, c, 16:16 + SEG, :] = qkv[
                        rows, (j + 1) * D + c * 128:(j + 1) * D + (c + 1) * 128]
        bscale = BDH ** -0.5
        ri8 = lax.broadcasted_iota(jnp.int32, (8, 128), 0)
        for l in layers:
            seg = t - 1 - 2 * l
            for r in range(SEG // 8):
                pos = seg * SEG + r * 8 + ri8
                q = [bq_ref[c, l * SEG + r * 8:l * SEG + r * 8 + 8, :] for c in range(NC)]
                lg = []
                for w in range(BW):
                    o0 = 16 + r * 8 - BDIL * w
                    s = q[0] * bkv_ref[l, 0, 0, o0:o0 + 8, :]
                    for c in range(1, NC):
                        s = s + q[c] * bkv_ref[l, 0, c, o0:o0 + 8, :]
                    s = s + pltpu.roll(s, 64, 1)
                    s = s + pltpu.roll(s, 32, 1)
                    if r * 8 - BDIL * w < 0:
                        s = jnp.where(pos - BDIL * w >= 0, s, -1e9 / bscale)
                    lg.append(s)
                m = lg[0]
                for w in range(1, BW):
                    m = jnp.maximum(m, lg[w])
                e = [jnp.exp2((s - m) * (bscale * LOG2E)) for s in lg]
                den = e[0]
                for w in range(1, BW):
                    den = den + e[w]
                inv = pl.reciprocal(den, approx=True)
                for c in range(NC):
                    o = e[0] * bkv_ref[l, 1, c, 16 + r * 8:16 + r * 8 + 8, :]
                    for w in range(1, BW):
                        o0 = 16 + r * 8 - BDIL * w
                        o = o + e[w] * bkv_ref[l, 1, c, o0:o0 + 8, :]
                    bq_ref[c, l * SEG + r * 8:l * SEG + r * 8 + 8, :] = o * inv

    def b_phase2(t, layers=(0, 1)):
        rows = slice(layers[0] * SEG, (layers[-1] + 1) * SEG)
        w = jnp.concatenate([pltpu.bitcast(pwo_ref[c], BF16) for c in range(NC)], axis=1)
        o = jnp.concatenate([bq_ref[c, rows, :] for c in range(NC)], axis=1).astype(BF16)
        yb = xb_ref[rows, :] + _nn(o, w)
        if 1 in layers:
            row = al(max(t - 3, 0) * SEG if isinstance(t, int) else jnp.maximum(t - 3, 0) * SEG, SEG)
            out_ref[pl.ds(row, SEG), :] = yb[-SEG:].astype(out_ref.dtype)
        return yb[:SEG]

    def x_seg(s):
        row = s * SEG if isinstance(s, int) else pl.multiple_of(s * SEG, SEG)
        return x_ref[pl.ds(row, SEG), :].astype(F32)

    def with_b(t, at_qkv, at_wo1, at_wo2):
        box = {}

        def hooks(p):
            if p == at_qkv - 0.5:
                b_phase1(t)
            elif p == at_wo1 and at_wo2 == at_wo1:
                box['x2'] = b_phase2(t)
            elif p == at_wo1:
                box['x2'] = b_phase2(t, (0,))
            elif p == at_wo2:
                b_phase2(t, (1,))
        return hooks, box

    def prepare_next(t, x2):
        sn = jnp.minimum(t + 1, NSEG - 1)
        hx_ref[0:SEG, :] = hxa_ref[pl.ds(al(sn * SEG, SEG), SEG), :]
        hx_ref[SEG:, :] = _ln(x2).astype(BF16)
        res_ref[...] = _cat0(x_seg(sn), x2)

    def permuted_rows(c):
        rows = [st_ref[c, pl.ds(d, H, stride=BDH), :] for d in range(BDH)]
        return _cat0(*rows)

    bkv_ref[...] = jnp.zeros(bkv_ref.shape, F32)
    acc_ref[...] = jnp.zeros(acc_ref.shape, F32)
    first[0].wait()
    xl0 = _ln(x_ref[0:X0 + XB, :].astype(F32)).astype(BF16)
    hxa_ref[0:X0 + XB, :] = xl0
    hx_ref[0:SEG, :] = xl0[0:SEG]

    def early(u, carry):
        rows = pl.ds(al((u // 3) * PW, 128), PW)
        pltpu.make_async_copy(wq_hbm.at[rows, :], wl_ref.at[u % 3, rows, :], qsem.at[u]).wait()
        w = wl_ref[u % 3, rows, :]
        wn_ref[u] = pltpu.bitcast(_cat0(*[transposed(w[:, c * 128:(c + 1) * 128]) for c in range(NC)]), U32)
        pre_ref[u, 2 * SEG:X0, :] = _nt(hxa_ref[2 * SEG:X0, :], w).astype(BF16)
        return carry

    lax.fori_loop(0, NPRE, early, 0)
    mem0_copy.wait()
    mem0 = mem0_ref[...].astype(F32)
    mem_ref[...] = _cat0(mem0, mem0)

    def step0(p, carry):
        group(p, lambda cp: cp.wait())
        u = jnp.minimum(p, NU - 1)

        def wfirst(m):
            w = wl_ref[m, pl.ds(al(p * PW, 128), PW), :]
            if m < 3:
                w = _cat0(*[transposed(w[:, c * 128:(c + 1) * 128]) for c in range(NC)])
                wt_ref[p * 3 + m] = pltpu.bitcast(w, U32)
                return weights(m, p) if RELOAD else w
            w_ref[pl.ds(al(p * (PW // 2), 64), PW // 2), :] = pltpu.bitcast(w, U32)
            return w

        _, arrange, scores, pv = attn_one_layer()
        h = _cat0(mem_ref[...].astype(BF16), hx_ref[0:SEG, :])
        xrows = x_rows(p)
        xl = hxa_ref[xrows, :]
        for c in range(NC):
            st_ref[0, c * 128:(c + 1) * 128, :] = bwqkv_ref[u, :, c * 128:(c + 1) * 128].astype(F32).T
        pwqkv_ref[u] = pltpu.bitcast(permuted_rows(0).T.astype(BF16), U32)
        done = [0]

        def pre(n):
            c0, c1 = done[0], min(done[0] + n, NPRE)
            done[0] = c1
            for c in range(c0, c1):
                pre_ref[c, xrows, :] = _nn(xl, pltpu.bitcast(wn_ref[c], BF16)).astype(BF16)

        pre(S0[0])
        q = _nn(h, wfirst(0)).astype(BF16)
        pre(S0[1])
        kt = arrange(_nn(h, wfirst(1)))
        pre(S0[2])
        s = scores(q, kt)
        pre(S0[3])
        vt = arrange(_nn(h, wfirst(2)))
        pre(S0[4])
        o = pv(s, vt)
        pre(NPRE)
        acc_ref[...] += _nn(o, wfirst(3))
        nrows = x_rows(u + 1)
        hxa_ref[nrows, :] = _ln(x_ref[nrows, :].astype(F32)).astype(BF16)
        issue_rest(p + WIN, 0)

        return carry

    lax.fori_loop(0, NPAIR, step0, 0)
    bw2.wait()
    for c in range(NC):
        st_ref[c] = bwo_ref[:, c * 128:(c + 1) * 128].astype(F32)
        pwo_ref[c] = pltpu.bitcast(permuted_rows(c).astype(BF16), U32)
    zeros = jnp.zeros((SEG, D), F32)
    mem_ref[0:M, :] = acc_ref[0:M, :]
    xb_ref[...] = _cat0(x_seg(0) + acc_ref[2 * M:, :], zeros)
    hx_ref[...] = _cat0(hxa_ref[SEG:2 * SEG, :], zeros.astype(BF16))
    res_ref[...] = _cat0(x_seg(1), zeros)

    def single(t, carry):
        l = (t >= NSEG).astype(jnp.int32)
        mrows = pl.ds(al(l * M, M), M)
        xrows = pl.ds(al(l * SEG, SEG), SEG)
        hooks, box = with_b(t, *SB)
        mem = mem_ref[mrows, :]
        h = _cat0(_cat0(mem, mem).astype(BF16), hx_ref[xrows, :])
        acc = a_phase(h, attn_one_layer(), hooks)
        mem_ref[mrows, :] = acc[:M]
        xb_ref[xrows, :] = res_ref[xrows, :] + acc[2 * M:]
        prepare_next(t, box['x2'])
        return carry

    def step(i, carry):
        for j in range(UNROLL):
            step1(i * UNROLL + j)
        return carry

    def step1(t):
        hooks, box = with_b(t, BQKV_AT, BWO_PAIR, BWO2_PAIR)
        h = _cat0(mem_ref[...].astype(BF16), hx_ref[...])
        acc = a_phase(h, attn_two_layers(), hooks, t)
        mem_ref[...] = acc[:2 * M]
        xb_ref[...] = res_ref[...] + acc[2 * M:]
        prepare_next(t, box['x2'])

    def outer(i, carry):
        lax.fori_loop(1 + (NSEG - 1) * i, 2 + NSEG * i, single, 0)
        lax.fori_loop(2 // UNROLL, (NSEG - (NSEG - 2) * i) // UNROLL, step, 0)
        pl.when(i == 0)(out_a.start)
        return carry

    lax.fori_loop(0, 2, outer, 0)
    b_phase1(NSEG + 2, (1,))
    b_phase2(NSEG + 2, (1,))
    out_b.start()
    out_a.wait()
    out_b.wait()


@jax.jit
def pallas_interleave_layers__memory_aug_recurrent_mem_tr__sliding_local_dilated__prompt_kernel(
    A_x, A_mem0, A_Wq, A_Wk, A_Wv, A_Wo, A_seg_len, B_x, B_wqkv, B_wo,
):
    del A_seg_len, B_x
    wt = lambda w: jnp.transpose(w, (1, 2, 0)).reshape(HD, D)
    hbm = pl.BlockSpec(memory_space=pl.ANY)
    out = pl.pallas_call(
        _kernel,
        out_shape=jax.ShapeDtypeStruct((S, D), A_x.dtype),
        in_specs=[hbm] * 8,
        out_specs=hbm,
        scratch_shapes=[
            pltpu.VMEM((S, D), BF16),
            pltpu.VMEM((S, D), BF16),
            pltpu.VMEM((4, HD, D), BF16),
            pltpu.VMEM((HD // 2, D), U32),
            pltpu.VMEM((3 * NPAIR, D // 2, PW), U32),
            pltpu.VMEM((NU, 128, D), BF16),
            pltpu.VMEM((D, D), BF16),
            pltpu.VMEM((NU, 64, D), U32),
            pltpu.VMEM((NC, D // 2, 128), U32),
            pltpu.VMEM((NC, D, 128), F32),
            pltpu.VMEM((R1, D), F32),
            pltpu.VMEM((2 * M, D), F32),
            pltpu.VMEM((2 * SEG, D), BF16),
            pltpu.VMEM((2 * SEG, D), F32),
            pltpu.VMEM((2 * SEG, D), F32),
            pltpu.VMEM((NC, 2 * SEG, 128), F32),
            pltpu.VMEM((2, 2, NC, 16 + SEG, 128), F32),
            pltpu.VMEM((NPRE, D // 2, PW), U32),
            pltpu.VMEM((S, D), BF16),
            pltpu.VMEM((NPRE, S, PW), BF16),
            pltpu.VMEM((M, D), BF16),
            pltpu.SemaphoreType.DMA((NPRE + 1,)),
            pltpu.SemaphoreType.DMA((NPAIR,)),
            pltpu.SemaphoreType.DMA((4,)),
        ],
        compiler_params=pltpu.CompilerParams(vmem_limit_bytes=120 * 2 ** 20),
    )(A_x.reshape(S, D), A_mem0.reshape(M, D), wt(A_Wq), wt(A_Wk), wt(A_Wv),
      A_Wo.reshape(HD, D), B_wqkv, B_wo)
    return out.reshape(1, S, D)
```

```python
import jax
import jax.numpy as jnp
from jax import lax
import jax.experimental.pallas as pl
import jax.experimental.pallas.tpu as pltpu

S, D = 2048, 640
H, DH = 32, 192
HD = H * DH
M, SEG = 8, 32
L = M + SEG
NSEG = S // SEG
R = 2 * L
NK = R + 4 * M
R1 = 2 * M + SEG
PW = 2 * DH
NPAIR = H // 2
BDH, BW, BDIL = 20, 8, 2
NC = D // 128
XB = 112
X0 = S - NPAIR * XB
NPRE = 8
XT = 7
TB = 1
RELOAD = 0
S0 = (2, 1, 1, 2, 1)
BQKV_AT = 0
F32, BF16, U32 = jnp.float32, jnp.bfloat16, jnp.uint32
NT = (((1,), (1,)), ((), ()))
LOG2E = 1.4426950408889634
NU = 3 * NC
WIN = 4
ORDER = 'SQKPVW'
ORDER_LAST = 'SxPwW'
MIDFIRST = 0
HELD = 2
UNROLL = 2
SB = (0, 15, 15)
SHELD = 2
BWO2_PAIR = 16
BWO_PAIR = 8


def _ln(x):
    m = jnp.mean(x, axis=-1, keepdims=True)
    xc = x - m
    v = jnp.mean(xc * xc, axis=-1, keepdims=True)
    return xc * lax.rsqrt(v + 1e-5)


def _nt(a, b):
    return lax.dot_general(a, b, NT, preferred_element_type=F32)


def _nn(a, b):
    return jnp.dot(a, b, preferred_element_type=F32)


def _cat0(*a):
    return jnp.concatenate(a, axis=0)


def _kernel(x_hbm, mem0_hbm, wq_hbm, wk_hbm, wv_hbm, wo_hbm, bwqkv_hbm, bwo_hbm,
            out_hbm,
            x_ref, out_ref, wl_ref, w_ref, wt_ref, bwqkv_ref, bwo_ref, pwqkv_ref, pwo_ref,
            st_ref, acc_ref, mem_ref, hx_ref, res_ref, xb_ref, bq_ref, bkv_ref, wn_ref, hxa_ref, pre_ref, mem0_ref, qsem, wsem, sem):
    def al(v, n):
        return v if isinstance(v, int) else pl.multiple_of(v, n)

    w_hbm = (wq_hbm, wk_hbm, wv_hbm, wo_hbm)

    def w_copy(m, p, s):
        rows = pl.ds(al(p * PW, 128), PW)
        return pltpu.make_async_copy(w_hbm[m].at[rows, :], wl_ref.at[m, rows, :], s)

    def x_rows(p):
        return pl.ds(al(X0 + p * XB, 16), XB)

    def x_copy(p):
        return pltpu.make_async_copy(x_hbm.at[x_rows(p + 1), :], x_ref.at[x_rows(p + 1), :], wsem.at[p])

    first = [pltpu.make_async_copy(x_hbm.at[pl.ds(0, X0 + XB), :], x_ref.at[pl.ds(0, X0 + XB), :], qsem.at[NPRE])] + [
        w_copy(c % 3, c // 3, qsem.at[c]) for c in range(NPRE)]

    def unit_copy(u):
        src = bwqkv_hbm.at[pl.ds(al((u % NC) * 128, 128), 128), pl.ds(al((u // NC) * D, 128), D)]
        return pltpu.make_async_copy(src, bwqkv_ref.at[u], wsem.at[u])

    bw2 = pltpu.make_async_copy(bwo_hbm, bwo_ref, sem.at[3])
    mem0_copy = pltpu.make_async_copy(mem0_hbm, mem0_ref, sem.at[0])
    osplit = (NSEG - 3) * SEG
    out_a = pltpu.make_async_copy(out_ref.at[pl.ds(0, osplit), :], out_hbm.at[pl.ds(0, osplit), :], sem.at[1])
    out_b = pltpu.make_async_copy(out_ref.at[pl.ds(osplit, S - osplit), :],
                                  out_hbm.at[pl.ds(osplit, S - osplit), :], sem.at[2])

    def issue_first(i, carry):
        for j, cp in enumerate(first):
            pl.when(i == j)(cp.start)
        return carry

    def group(p, act):
        for m in range(3):
            pl.when((p * 3 + m >= NPRE) & (p < NPAIR))(lambda m=m: act(w_copy(m, p, wsem.at[p])))

        @pl.when(p < NPAIR - 1)
        def _():
            act(unit_copy(p))
            act(x_copy(p))

        pl.when(p < NPAIR)(lambda: act(w_copy(3, p, wsem.at[p])))

    def issue_rest(p, carry):
        group(p, lambda cp: cp.start())
        pl.when(p == NPAIR)(bw2.start)
        return carry

    lax.fori_loop(0, len(first), issue_first, 0)
    mem0_copy.start()
    lax.fori_loop(0, WIN, issue_rest, 0)

    def weights(m, p):
        if m < 3:
            return pltpu.bitcast(wt_ref[p * 3 + m], BF16)
        return pltpu.bitcast(w_ref[pl.ds(p * PW // 2, PW // 2), :], BF16)

    def transposed(w):
        return w.T if TB else w.astype(F32).T.astype(BF16)


    scale = DH ** -0.5
    ninf = -jnp.inf

    def softmax2(s, sel, allowed):
        s = jnp.where(allowed, s, -1e9 / scale)
        m0 = jnp.max(jnp.where(sel, s, ninf), axis=-1, keepdims=True)
        m1 = jnp.max(jnp.where(sel, ninf, s), axis=-1, keepdims=True)
        e = jnp.exp2((s - jnp.where(sel, m0, m1)) * (scale * LOG2E))
        e0, e1 = jnp.where(sel, e, 0.0), jnp.where(sel, 0.0, e)
        d0 = jnp.sum(e0, axis=-1, keepdims=True)
        d1 = jnp.sum(e1, axis=-1, keepdims=True)
        return e, e0, e1, pl.reciprocal(d0, approx=True), pl.reciprocal(d1, approx=True)

    def masks(rows):
        qi = lax.broadcasted_iota(jnp.int32, (rows, R), 0)
        ki = lax.broadcasted_iota(jnp.int32, (rows, R), 1)
        first = ki < L
        kk = jnp.where(first, ki, ki - L)
        qq = M + ((qi - 2 * M) & (SEG - 1))
        allowed = (qi < 2 * M) | (kk <= qq)
        return qi, first, allowed

    def attn_two_layers():
        qi = lax.broadcasted_iota(jnp.int32, (R, NK), 0)
        ki = lax.broadcasted_iota(jnp.int32, (R, NK), 1)
        special = (qi >= R1) & (qi < R1 + M)
        kk = jnp.where(ki < L, ki, jnp.where(ki < R, ki - L, (ki - R) & (2 * M - 1)))
        qq = M + ((qi - 2 * M) & (SEG - 1))
        allowed = (special == (ki >= R)) & ((qi < 2 * M) | (kk <= qq))
        row_l1 = (qi < M) | ((qi >= 2 * M) & (qi < R1))
        is_a = jnp.where(special, ki - (R + 2 * M), jnp.where(row_l1, L - 1 - ki, ki - L)) >= 0
        lo = lax.broadcasted_iota(jnp.int32, (L, 128), 1) < 64

        def arrange(a):
            a1 = _cat0(a[0:M], a[2 * M:R1])
            a2 = _cat0(a[M:2 * M], a[R1:])
            cat = lambda *u: _cat0(*u).astype(BF16)
            m1, m2 = a1[:, 128:256], a2[:, 128:256]
            m2b, m2a = jnp.where(lo, 0.0, m2), jnp.where(lo, m2, 0.0)
            e = 2 * M
            return (cat(a1[:, :128], a2[:, :128], a2[:e, :128], a2[:e, :128]),
                    cat(a2[:, 256:], a1[:, 256:], a2[:e, 256:], a2[:e, 256:]),
                    cat(jnp.where(lo, m1, 0.0), jnp.where(lo, 0.0, m1), m2b[:e], m2a[:e]),
                    cat(m2b, m2a, m2b[:e], m2b[:e]))

        g1 = lambda a: _cat0(a[0:M], a[2 * M:R1 + M])
        g2 = lambda a: _cat0(a[M:2 * M], a[R1 + M:])
        merge = lambda u1, u2: _cat0(u1[0:M], u2[0:M], u1[M:], u2[M:])

        def arrange_q(q):
            qm = q[:, 128:256]
            return [u.astype(BF16) for u in (q[:, :128], q[:, 256:], g1(qm), g2(qm))]

        def scores(q, kt):
            order = (2, 3, 0, 1) if MIDFIRST & 1 else (0, 1, 2, 3)
            r = {i: _nt(q[i], kt[i]) for i in order}
            return [r[i] for i in range(4)]

        lo_r = lax.broadcasted_iota(jnp.int32, (R, 128), 1) < 64

        def pv(s4, vt):
            sa, sb, s1, s2 = s4
            p, pa, pb, ra, rb = softmax2(jnp.where(is_a, sa, sb) + merge(s1, s2), is_a, allowed)
            if MIDFIRST & 2:
                om = merge(_nn(g1(p).astype(BF16), vt[2]), _nn(g2(p).astype(BF16), vt[3]))
                oa, ob = _nn(pa.astype(BF16), vt[0]), _nn(pb.astype(BF16), vt[1])
            else:
                oa, ob = _nn(pa.astype(BF16), vt[0]), _nn(pb.astype(BF16), vt[1])
                om = merge(_nn(g1(p).astype(BF16), vt[2]), _nn(g2(p).astype(BF16), vt[3]))
            return jnp.concatenate(
                [oa * ra, om * jnp.where(lo_r, ra, rb), ob * rb], axis=1).astype(BF16)

        return arrange_q, arrange, scores, pv

    def attn_one_layer():
        _, first, allowed = masks(R1)
        head_a = lax.broadcasted_iota(jnp.int32, (L, PW), 1) < DH

        def arrange(a):
            a1 = _cat0(a[0:M], a[2 * M:])
            return _cat0(jnp.where(head_a, a1, 0.0), jnp.where(head_a, 0.0, a1)).astype(BF16)

        head_a1 = lax.broadcasted_iota(jnp.int32, (R1, PW), 1) < DH

        def pv(s, vt):
            p, _, _, r0, r1 = softmax2(s, first, allowed)
            return (_nn(p.astype(BF16), vt) * jnp.where(head_a1, r0, r1)).astype(BF16)

        return lambda q: q.astype(BF16), arrange, _nt, pv

    def a_phase(h, attn, hooks, t=None):
        arrange_q, arrange, scores, pv = attn

        def proj(m, p):
            c = p * 3 + m
            if c >= NPRE or t is None:
                return _nn(h, weights(m, p))
            y = _nn(_cat0(h[0:2 * M], h[R1:]), weights(m, p))
            pre = pre_ref[c, pl.ds(al(t * SEG, SEG), SEG), :].astype(F32)
            return _cat0(y[0:2 * M], pre, y[2 * M:])

        proj_o = lambda o, p: _nn(o, weights(3, p))
        st = {'acc': None, 'o': {}, 'done': 0}

        def wo_upto(n):
            while st['done'] < n:
                pp = st['done']
                y = proj_o(st['o'].pop(pp), pp)
                st['acc'] = y if st['acc'] is None else st['acc'] + y
                st['done'] += 1

        q, kt = arrange_q(proj(0, 0)), arrange(proj(1, 0))
        vts = {0: arrange(proj(2, 0))}
        lim = NPAIR - 1 - (SHELD if t is None else HELD)
        for p in range(NPAIR):
            last = p == NPAIR - 1
            for op in (ORDER_LAST if last else ORDER):
                if op == 'S':
                    s = scores(q, kt)
                    hooks(p - 0.5)
                elif op == 'Q':
                    qn = arrange_q(proj(0, p + 1))
                elif op == 'K':
                    ktn = arrange(proj(1, p + 1))
                elif op == 'V':
                    vts[p + 1] = arrange(proj(2, p + 1))
                elif op == 'P':
                    hooks(p)
                    st['o'][p] = pv(s, vts.pop(p))
                elif op == 'W':
                    wo_upto(p + 1 if last else min(p + 1, lim))
                elif op == 'w':
                    wo_upto(p if last else min(p, lim))
                elif op == 'x':
                    wo_upto(p - 1)
            q, kt = qn, ktn
        hooks(NPAIR)
        return st['acc']

    def b_phase1(t, layers=(0, 1)):
        w = jnp.concatenate([_cat0(*[pltpu.bitcast(pwqkv_ref[j * NC + c], BF16) for c in range(NC)])
                             for j in range(3)], axis=1)
        l0 = layers[0]
        qkv = _nn(_ln(xb_ref[l0 * SEG:(layers[-1] + 1) * SEG, :]).astype(BF16), w)
        for l in layers:
            rows = slice((l - l0) * SEG, (l - l0 + 1) * SEG)
            for c in range(NC):
                bq_ref[c, l * SEG:(l + 1) * SEG, :] = qkv[rows, c * 128:(c + 1) * 128]
                for j in range(2):
                    bkv_ref[l, j, c, 0:16, :] = bkv_ref[l, j, c, SEG:SEG + 16, :]
                    bkv_ref[l, j, c, 16:16 + SEG, :] = qkv[
                        rows, (j + 1) * D + c * 128:(j + 1) * D + (c + 1) * 128]
        bscale = BDH ** -0.5
        ri8 = lax.broadcasted_iota(jnp.int32, (8, 128), 0)
        for l in layers:
            seg = t - 1 - 2 * l
            for r in range(SEG // 8):
                pos = seg * SEG + r * 8 + ri8
                q = [bq_ref[c, l * SEG + r * 8:l * SEG + r * 8 + 8, :] for c in range(NC)]
                lg = []
                for w in range(BW):
                    o0 = 16 + r * 8 - BDIL * w
                    s = q[0] * bkv_ref[l, 0, 0, o0:o0 + 8, :]
                    for c in range(1, NC):
                        s = s + q[c] * bkv_ref[l, 0, c, o0:o0 + 8, :]
                    s = s + pltpu.roll(s, 64, 1)
                    s = s + pltpu.roll(s, 32, 1)
                    if r * 8 - BDIL * w < 0:
                        s = jnp.where(pos - BDIL * w >= 0, s, -1e9 / bscale)
                    lg.append(s)
                m = lg[0]
                for w in range(1, BW):
                    m = jnp.maximum(m, lg[w])
                e = [jnp.exp2((s - m) * (bscale * LOG2E)) for s in lg]
                den = e[0]
                for w in range(1, BW):
                    den = den + e[w]
                inv = pl.reciprocal(den, approx=True)
                for c in range(NC):
                    o = e[0] * bkv_ref[l, 1, c, 16 + r * 8:16 + r * 8 + 8, :]
                    for w in range(1, BW):
                        o0 = 16 + r * 8 - BDIL * w
                        o = o + e[w] * bkv_ref[l, 1, c, o0:o0 + 8, :]
                    bq_ref[c, l * SEG + r * 8:l * SEG + r * 8 + 8, :] = o * inv

    def b_phase2(t, layers=(0, 1)):
        rows = slice(layers[0] * SEG, (layers[-1] + 1) * SEG)
        w = jnp.concatenate([pltpu.bitcast(pwo_ref[c], BF16) for c in range(NC)], axis=1)
        o = jnp.concatenate([bq_ref[c, rows, :] for c in range(NC)], axis=1).astype(BF16)
        yb = xb_ref[rows, :] + _nn(o, w)
        if 1 in layers:
            row = al(max(t - 3, 0) * SEG if isinstance(t, int) else jnp.maximum(t - 3, 0) * SEG, SEG)
            out_ref[pl.ds(row, SEG), :] = yb[-SEG:].astype(out_ref.dtype)
        return yb[:SEG]

    def x_seg(s):
        row = s * SEG if isinstance(s, int) else pl.multiple_of(s * SEG, SEG)
        return x_ref[pl.ds(row, SEG), :].astype(F32)

    def with_b(t, at_qkv, at_wo1, at_wo2):
        box = {}

        def hooks(p):
            if p == at_qkv - 0.5:
                b_phase1(t)
            elif p == at_wo1 and at_wo2 == at_wo1:
                box['x2'] = b_phase2(t)
            elif p == at_wo1:
                box['x2'] = b_phase2(t, (0,))
            elif p == at_wo2:
                b_phase2(t, (1,))
        return hooks, box

    def prepare_next(t, x2):
        sn = jnp.minimum(t + 1, NSEG - 1)
        hx_ref[0:SEG, :] = hxa_ref[pl.ds(al(sn * SEG, SEG), SEG), :]
        hx_ref[SEG:, :] = _ln(x2).astype(BF16)
        res_ref[...] = _cat0(x_seg(sn), x2)

    def permuted_rows(c):
        rows = [st_ref[c, pl.ds(d, H, stride=BDH), :] for d in range(BDH)]
        return _cat0(*rows)

    bkv_ref[...] = jnp.zeros(bkv_ref.shape, F32)
    acc_ref[...] = jnp.zeros(acc_ref.shape, F32)
    first[0].wait()
    xl0 = _ln(x_ref[0:X0 + XB, :].astype(F32)).astype(BF16)
    hxa_ref[0:X0 + XB, :] = xl0
    hx_ref[0:SEG, :] = xl0[0:SEG]

    def early(u, carry):
        rows = pl.ds(al((u // 3) * PW, 128), PW)
        pltpu.make_async_copy(wq_hbm.at[rows, :], wl_ref.at[u % 3, rows, :], qsem.at[u]).wait()
        w = wl_ref[u % 3, rows, :]
        wn_ref[u] = pltpu.bitcast(_cat0(*[transposed(w[:, c * 128:(c + 1) * 128]) for c in range(NC)]), U32)
        pre_ref[u, 2 * SEG:X0, :] = _nt(hxa_ref[2 * SEG:X0, :], w).astype(BF16)
        return carry

    lax.fori_loop(0, NPRE, early, 0)
    mem0_copy.wait()
    mem0 = mem0_ref[...].astype(F32)
    mem_ref[...] = _cat0(mem0, mem0)

    def step0(p, carry):
        group(p, lambda cp: cp.wait())
        u = jnp.minimum(p, NU - 1)

        def wfirst(m):
            w = wl_ref[m, pl.ds(al(p * PW, 128), PW), :]
            if m < 3:
                w = _cat0(*[transposed(w[:, c * 128:(c + 1) * 128]) for c in range(NC)])
                wt_ref[p * 3 + m] = pltpu.bitcast(w, U32)
                return weights(m, p) if RELOAD else w
            w_ref[pl.ds(al(p * (PW // 2), 64), PW // 2), :] = pltpu.bitcast(w, U32)
            return w

        _, arrange, scores, pv = attn_one_layer()
        h = _cat0(mem_ref[...].astype(BF16), hx_ref[0:SEG, :])
        xrows = x_rows(p)
        xl = hxa_ref[xrows, :]
        for c in range(NC):
            st_ref[0, c * 128:(c + 1) * 128, :] = bwqkv_ref[u, :, c * 128:(c + 1) * 128].astype(F32).T
        pwqkv_ref[u] = pltpu.bitcast(permuted_rows(0).T.astype(BF16), U32)
        done = [0]

        def pre(n):
            c0, c1 = done[0], min(done[0] + n, NPRE)
            done[0] = c1
            for c in range(c0, c1):
                pre_ref[c, xrows, :] = _nn(xl, pltpu.bitcast(wn_ref[c], BF16)).astype(BF16)

        pre(S0[0])
        q = _nn(h, wfirst(0)).astype(BF16)
        pre(S0[1])
        kt = arrange(_nn(h, wfirst(1)))
        pre(S0[2])
        s = scores(q, kt)
        pre(S0[3])
        vt = arrange(_nn(h, wfirst(2)))
        pre(S0[4])
        o = pv(s, vt)
        pre(NPRE)
        acc_ref[...] += _nn(o, wfirst(3))
        nrows = x_rows(u + 1)
        hxa_ref[nrows, :] = _ln(x_ref[nrows, :].astype(F32)).astype(BF16)
        issue_rest(p + WIN, 0)

        return carry

    lax.fori_loop(0, NPAIR, step0, 0)
    bw2.wait()
    for c in range(NC):
        st_ref[c] = bwo_ref[:, c * 128:(c + 1) * 128].astype(F32)
        pwo_ref[c] = pltpu.bitcast(permuted_rows(c).astype(BF16), U32)
    zeros = jnp.zeros((SEG, D), F32)
    mem_ref[0:M, :] = acc_ref[0:M, :]
    xb_ref[...] = _cat0(x_seg(0) + acc_ref[2 * M:, :], zeros)
    hx_ref[...] = _cat0(hxa_ref[SEG:2 * SEG, :], zeros.astype(BF16))
    res_ref[...] = _cat0(x_seg(1), zeros)

    def single(t, carry):
        l = (t >= NSEG).astype(jnp.int32)
        mrows = pl.ds(al(l * M, M), M)
        xrows = pl.ds(al(l * SEG, SEG), SEG)
        hooks, box = with_b(t, *SB)
        mem = mem_ref[mrows, :]
        h = _cat0(_cat0(mem, mem).astype(BF16), hx_ref[xrows, :])
        acc = a_phase(h, attn_one_layer(), hooks)
        mem_ref[mrows, :] = acc[:M]
        xb_ref[xrows, :] = res_ref[xrows, :] + acc[2 * M:]
        prepare_next(t, box['x2'])
        return carry

    def step(i, carry):
        for j in range(UNROLL):
            step1(i * UNROLL + j)
        return carry

    def step1(t):
        hooks, box = with_b(t, BQKV_AT, BWO_PAIR, BWO2_PAIR)
        h = _cat0(mem_ref[...].astype(BF16), hx_ref[...])
        acc = a_phase(h, attn_two_layers(), hooks, t)
        mem_ref[...] = acc[:2 * M]
        xb_ref[...] = res_ref[...] + acc[2 * M:]
        prepare_next(t, box['x2'])

    def outer(i, carry):
        lax.fori_loop(1 + (NSEG - 1) * i, 2 + NSEG * i, single, 0)
        lax.fori_loop(2 // UNROLL, (NSEG - (NSEG - 2) * i) // UNROLL, step, 0)
        pl.when(i == 0)(out_a.start)
        return carry

    lax.fori_loop(0, 2, outer, 0)
    b_phase1(NSEG + 2, (1,))
    b_phase2(NSEG + 2, (1,))
    out_b.start()
    out_a.wait()
    out_b.wait()


@jax.jit
def pallas_interleave_layers__memory_aug_recurrent_mem_tr__sliding_local_dilated__prompt_kernel(
    A_x, A_mem0, A_Wq, A_Wk, A_Wv, A_Wo, A_seg_len, B_x, B_wqkv, B_wo,
):
    del A_seg_len, B_x
    wt = lambda w: jnp.transpose(w, (1, 2, 0)).reshape(HD, D)
    hbm = pl.BlockSpec(memory_space=pl.ANY)
    out = pl.pallas_call(
        _kernel,
        out_shape=jax.ShapeDtypeStruct((S, D), A_x.dtype),
        in_specs=[hbm] * 8,
        out_specs=hbm,
        scratch_shapes=[
            pltpu.VMEM((S, D), BF16),
            pltpu.VMEM((S, D), BF16),
            pltpu.VMEM((4, HD, D), BF16),
            pltpu.VMEM((HD // 2, D), U32),
            pltpu.VMEM((3 * NPAIR, D // 2, PW), U32),
            pltpu.VMEM((NU, 128, D), BF16),
            pltpu.VMEM((D, D), BF16),
            pltpu.VMEM((NU, 64, D), U32),
            pltpu.VMEM((NC, D // 2, 128), U32),
            pltpu.VMEM((NC, D, 128), F32),
            pltpu.VMEM((R1, D), F32),
            pltpu.VMEM((2 * M, D), F32),
            pltpu.VMEM((2 * SEG, D), BF16),
            pltpu.VMEM((2 * SEG, D), F32),
            pltpu.VMEM((2 * SEG, D), F32),
            pltpu.VMEM((NC, 2 * SEG, 128), F32),
            pltpu.VMEM((2, 2, NC, 16 + SEG, 128), F32),
            pltpu.VMEM((NPRE, D // 2, PW), U32),
            pltpu.VMEM((S, D), BF16),
            pltpu.VMEM((NPRE, S, PW), BF16),
            pltpu.VMEM((M, D), BF16),
            pltpu.SemaphoreType.DMA((NPRE + 1,)),
            pltpu.SemaphoreType.DMA((NPAIR,)),
            pltpu.SemaphoreType.DMA((4,)),
        ],
        compiler_params=pltpu.CompilerParams(vmem_limit_bytes=120 * 2 ** 20),
    )(A_x.reshape(S, D), A_mem0.reshape(M, D), wt(A_Wq), wt(A_Wk), wt(A_Wv),
      A_Wo.reshape(HD, D), B_wqkv, B_wo)
    return out.reshape(1, S, D)
```

```python
import jax
import jax.numpy as jnp
from jax import lax
import jax.experimental.pallas as pl
import jax.experimental.pallas.tpu as pltpu

S, D = 2048, 640
H, DH = 32, 192
HD = H * DH
M, SEG = 8, 32
L = M + SEG
NSEG = S // SEG
R = 2 * L
NK = R + 4 * M
R1 = 2 * M + SEG
PW = 2 * DH
NPAIR = H // 2
BDH, BW, BDIL = 20, 8, 2
NC = D // 128
XB = 112
X0 = S - NPAIR * XB
NPRE = 8
XT = 7
TB = 1
RELOAD = 0
S0 = (2, 1, 1, 2, 1)
BQKV_AT = 0
F32, BF16, U32 = jnp.float32, jnp.bfloat16, jnp.uint32
NT = (((1,), (1,)), ((), ()))
LOG2E = 1.4426950408889634
NU = 3 * NC
WIN = 4
ORDER = 'SQKPVW'
ORDER_LAST = 'SxPwW'
SORD = (0, 1, 2, 3)
PORD = (0, 1, 2, 3)
HELD = 2
UNROLL = 2
PINS = (2, 4, 6, 7, 9, 11, 13, 14)
SB = (0, 15, 15)
SHELD = 2
BWO2_PAIR = 16
BWO_PAIR = 8


def _ln(x):
    m = jnp.mean(x, axis=-1, keepdims=True)
    xc = x - m
    v = jnp.mean(xc * xc, axis=-1, keepdims=True)
    return xc * lax.rsqrt(v + 1e-5)


def _nt(a, b):
    return lax.dot_general(a, b, NT, preferred_element_type=F32)


def _nn(a, b):
    return jnp.dot(a, b, preferred_element_type=F32)


def _cat0(*a):
    return jnp.concatenate(a, axis=0)


def _kernel(x_hbm, mem0_hbm, wq_hbm, wk_hbm, wv_hbm, wo_hbm, bwqkv_hbm, bwo_hbm,
            out_hbm,
            x_ref, out_ref, wl_ref, w_ref, wt_ref, bwqkv_ref, bwo_ref, pwqkv_ref, pwo_ref,
            st_ref, acc_ref, mem_ref, hx_ref, res_ref, xb_ref, bq_ref, bkv_ref, wn_ref, hxa_ref, pre_ref, mem0_ref, zero_ref, qsem, wsem, sem):
    def al(v, n):
        return v if isinstance(v, int) else pl.multiple_of(v, n)

    w_hbm = (wq_hbm, wk_hbm, wv_hbm, wo_hbm)

    def w_copy(m, p, s):
        rows = pl.ds(al(p * PW, 128), PW)
        return pltpu.make_async_copy(w_hbm[m].at[rows, :], wl_ref.at[m, rows, :], s)

    def x_rows(p):
        return pl.ds(al(X0 + p * XB, 16), XB)

    def x_copy(p):
        return pltpu.make_async_copy(x_hbm.at[x_rows(p + 1), :], x_ref.at[x_rows(p + 1), :], wsem.at[p])

    first = [pltpu.make_async_copy(x_hbm.at[pl.ds(0, X0 + XB), :], x_ref.at[pl.ds(0, X0 + XB), :], qsem.at[NPRE])] + [
        w_copy(c % 3, c // 3, qsem.at[c]) for c in range(NPRE)]

    def unit_copy(u):
        src = bwqkv_hbm.at[pl.ds(al((u % NC) * 128, 128), 128), pl.ds(al((u // NC) * D, 128), D)]
        return pltpu.make_async_copy(src, bwqkv_ref.at[u], wsem.at[u])

    bw2 = pltpu.make_async_copy(bwo_hbm, bwo_ref, sem.at[3])
    mem0_copy = pltpu.make_async_copy(mem0_hbm, mem0_ref, sem.at[0])
    osplit = (NSEG - 3) * SEG
    out_a = pltpu.make_async_copy(out_ref.at[pl.ds(0, osplit), :], out_hbm.at[pl.ds(0, osplit), :], sem.at[1])
    out_b = pltpu.make_async_copy(out_ref.at[pl.ds(osplit, S - osplit), :],
                                  out_hbm.at[pl.ds(osplit, S - osplit), :], sem.at[2])

    def issue_first(i, carry):
        for j, cp in enumerate(first):
            pl.when(i == j)(cp.start)
        return carry

    def group(p, act):
        for m in range(3):
            pl.when((p * 3 + m >= NPRE) & (p < NPAIR))(lambda m=m: act(w_copy(m, p, wsem.at[p])))

        @pl.when(p < NPAIR - 1)
        def _():
            act(unit_copy(p))
            act(x_copy(p))

        pl.when(p < NPAIR)(lambda: act(w_copy(3, p, wsem.at[p])))

    def issue_rest(p, carry):
        group(p, lambda cp: cp.start())
        pl.when(p == NPAIR)(bw2.start)
        return carry

    lax.fori_loop(0, len(first), issue_first, 0)
    mem0_copy.start()
    lax.fori_loop(0, WIN, issue_rest, 0)

    def weights(m, p):
        if m < 3:
            return pltpu.bitcast(wt_ref[p * 3 + m], BF16)
        return pltpu.bitcast(w_ref[pl.ds(p * PW // 2, PW // 2), :], BF16)

    def transposed(w):
        return w.T if TB else w.astype(F32).T.astype(BF16)


    scale = DH ** -0.5
    ninf = -jnp.inf

    def softmax2(s, sel, allowed):
        s = jnp.where(allowed, s, -1e9 / scale)
        m0 = jnp.max(jnp.where(sel, s, ninf), axis=-1, keepdims=True)
        m1 = jnp.max(jnp.where(sel, ninf, s), axis=-1, keepdims=True)
        e = jnp.exp2((s - jnp.where(sel, m0, m1)) * (scale * LOG2E))
        e0, e1 = jnp.where(sel, e, 0.0), jnp.where(sel, 0.0, e)
        d0 = jnp.sum(e0, axis=-1, keepdims=True)
        d1 = jnp.sum(e1, axis=-1, keepdims=True)
        return e, e0, e1, pl.reciprocal(d0, approx=True), pl.reciprocal(d1, approx=True)

    def masks(rows):
        qi = lax.broadcasted_iota(jnp.int32, (rows, R), 0)
        ki = lax.broadcasted_iota(jnp.int32, (rows, R), 1)
        first = ki < L
        kk = jnp.where(first, ki, ki - L)
        qq = M + ((qi - 2 * M) & (SEG - 1))
        allowed = (qi < 2 * M) | (kk <= qq)
        return qi, first, allowed

    def attn_two_layers():
        qi = lax.broadcasted_iota(jnp.int32, (R, NK), 0)
        ki = lax.broadcasted_iota(jnp.int32, (R, NK), 1)
        special = (qi >= R1) & (qi < R1 + M)
        kk = jnp.where(ki < L, ki, jnp.where(ki < R, ki - L, (ki - R) & (2 * M - 1)))
        qq = M + ((qi - 2 * M) & (SEG - 1))
        allowed = (special == (ki >= R)) & ((qi < 2 * M) | (kk <= qq))
        row_l1 = (qi < M) | ((qi >= 2 * M) & (qi < R1))
        is_a = jnp.where(special, ki - (R + 2 * M), jnp.where(row_l1, L - 1 - ki, ki - L)) >= 0
        lo = lax.broadcasted_iota(jnp.int32, (L, 128), 1) < 64

        def arrange(a):
            a1 = _cat0(a[0:M], a[2 * M:R1])
            a2 = _cat0(a[M:2 * M], a[R1:])
            cat = lambda *u: _cat0(*u).astype(BF16)
            m1, m2 = a1[:, 128:256], a2[:, 128:256]
            m2b, m2a = jnp.where(lo, 0.0, m2), jnp.where(lo, m2, 0.0)
            e = 2 * M
            return (cat(a1[:, :128], a2[:, :128], a2[:e, :128], a2[:e, :128]),
                    cat(a2[:, 256:], a1[:, 256:], a2[:e, 256:], a2[:e, 256:]),
                    cat(jnp.where(lo, m1, 0.0), jnp.where(lo, 0.0, m1), m2b[:e], m2a[:e]),
                    cat(m2b, m2a, m2b[:e], m2b[:e]))

        g1 = lambda a: _cat0(a[0:M], a[2 * M:R1 + M])
        g2 = lambda a: _cat0(a[M:2 * M], a[R1 + M:])
        merge = lambda u1, u2: _cat0(u1[0:M], u2[0:M], u1[M:], u2[M:])

        def arrange_q(q):
            qm = q[:, 128:256]
            return [u.astype(BF16) for u in (q[:, :128], q[:, 256:], g1(qm), g2(qm))]

        def scores(q, kt):
            r = {i: _nt(q[i], kt[i]) for i in SORD}
            return [r[i] for i in range(4)]

        lo_r = lax.broadcasted_iota(jnp.int32, (R, 128), 1) < 64

        def pv(s4, vt, pin=None):
            sa, sb, s1, s2 = s4
            if pin is not None:
                s1 = _cat0(s1[0:M] + pin[:, :NK], s1[M:])
            p, pa, pb, ra, rb = softmax2(jnp.where(is_a, sa, sb) + merge(s1, s2), is_a, allowed)
            lhs = (pa, pb, g1(p), g2(p))
            r = {i: _nn(lhs[i].astype(BF16), vt[i]) for i in PORD}
            oa, ob, om = r[0], r[1], merge(r[2], r[3])
            return jnp.concatenate(
                [oa * ra, om * jnp.where(lo_r, ra, rb), ob * rb], axis=1).astype(BF16)

        return arrange_q, arrange, scores, pv

    def attn_one_layer():
        _, first, allowed = masks(R1)
        head_a = lax.broadcasted_iota(jnp.int32, (L, PW), 1) < DH

        def arrange(a):
            a1 = _cat0(a[0:M], a[2 * M:])
            return _cat0(jnp.where(head_a, a1, 0.0), jnp.where(head_a, 0.0, a1)).astype(BF16)

        head_a1 = lax.broadcasted_iota(jnp.int32, (R1, PW), 1) < DH

        def pv(s, vt, pin=None):
            p, _, _, r0, r1 = softmax2(s, first, allowed)
            return (_nn(p.astype(BF16), vt) * jnp.where(head_a1, r0, r1)).astype(BF16)

        return lambda q: q.astype(BF16), arrange, _nt, pv

    def a_phase(h, attn, hooks, t=None):
        arrange_q, arrange, scores, pv = attn

        def proj(m, p):
            c = p * 3 + m
            if c >= NPRE or t is None:
                return _nn(h, weights(m, p))
            y = _nn(_cat0(h[0:2 * M], h[R1:]), weights(m, p))
            pre = pre_ref[c, pl.ds(al(t * SEG, SEG), SEG), :].astype(F32)
            return _cat0(y[0:2 * M], pre, y[2 * M:])

        proj_o = lambda o, p: _nn(o, weights(3, p))
        st = {'acc': None, 'o': {}, 'done': 0}

        def wo_upto(n):
            while st['done'] < n:
                pp = st['done']
                y = proj_o(st['o'].pop(pp), pp)
                st['acc'] = y if st['acc'] is None else st['acc'] + y
                st['done'] += 1

        q, kt = arrange_q(proj(0, 0)), arrange(proj(1, 0))
        vts = {0: arrange(proj(2, 0))}
        lim = NPAIR - 1 - (SHELD if t is None else HELD)
        for p in range(NPAIR):
            last = p == NPAIR - 1
            for op in (ORDER_LAST if last else ORDER):
                if op == 'S':
                    s = scores(q, kt)
                    hooks(p - 0.5)
                elif op == 'Q':
                    qn = arrange_q(proj(0, p + 1))
                elif op == 'K':
                    ktn = arrange(proj(1, p + 1))
                elif op == 'V':
                    vts[p + 1] = arrange(proj(2, p + 1))
                elif op == 'P':
                    st['o'][p] = pv(s, vts.pop(p), hooks(p))
                elif op == 'W':
                    wo_upto(p + 1 if last else min(p + 1, lim))
                elif op == 'w':
                    wo_upto(p if last else min(p, lim))
                elif op == 'x':
                    wo_upto(p - 1)
            q, kt = qn, ktn
        hooks(NPAIR)
        return st['acc']

    def b_phase1(t, layers=(0, 1), pins=None):
        w = jnp.concatenate([_cat0(*[pltpu.bitcast(pwqkv_ref[j * NC + c], BF16) for c in range(NC)])
                             for j in range(3)], axis=1)
        l0 = layers[0]
        qkv = _nn(_ln(xb_ref[l0 * SEG:(layers[-1] + 1) * SEG, :]).astype(BF16), w)
        for l in layers:
            rows = slice((l - l0) * SEG, (l - l0 + 1) * SEG)
            for c in range(NC):
                bq_ref[c, l * SEG:(l + 1) * SEG, :] = qkv[rows, c * 128:(c + 1) * 128]
                for j in range(2):
                    bkv_ref[l, j, c, 0:16, :] = bkv_ref[l, j, c, SEG:SEG + 16, :]
                    bkv_ref[l, j, c, 16:16 + SEG, :] = qkv[
                        rows, (j + 1) * D + c * 128:(j + 1) * D + (c + 1) * 128]
        bscale = BDH ** -0.5
        ri8 = lax.broadcasted_iota(jnp.int32, (8, 128), 0)
        for l in layers:
            seg = t - 1 - 2 * l
            for r in range(SEG // 8):
                pos = seg * SEG + r * 8 + ri8
                q = [bq_ref[c, l * SEG + r * 8:l * SEG + r * 8 + 8, :] for c in range(NC)]
                lg = []
                for w in range(BW):
                    o0 = 16 + r * 8 - BDIL * w
                    s = q[0] * bkv_ref[l, 0, 0, o0:o0 + 8, :]
                    for c in range(1, NC):
                        s = s + q[c] * bkv_ref[l, 0, c, o0:o0 + 8, :]
                    s = s + pltpu.roll(s, 64, 1)
                    s = s + pltpu.roll(s, 32, 1)
                    if r * 8 - BDIL * w < 0:
                        s = jnp.where(pos - BDIL * w >= 0, s, -1e9 / bscale)
                    lg.append(s)
                m = lg[0]
                for w in range(1, BW):
                    m = jnp.maximum(m, lg[w])
                e = [jnp.exp2((s - m) * (bscale * LOG2E)) for s in lg]
                den = e[0]
                for w in range(1, BW):
                    den = den + e[w]
                inv = pl.reciprocal(den, approx=True)
                bits = None
                for c in range(NC):
                    o = e[0] * bkv_ref[l, 1, c, 16 + r * 8:16 + r * 8 + 8, :]
                    for w in range(1, BW):
                        o0 = 16 + r * 8 - BDIL * w
                        o = o + e[w] * bkv_ref[l, 1, c, o0:o0 + 8, :]
                    o = o * inv
                    bq_ref[c, l * SEG + r * 8:l * SEG + r * 8 + 8, :] = o
                    ob = pltpu.bitcast(o, jnp.int32)
                    bits = ob if bits is None else bits | ob
                if pins is not None:
                    pins[PINS[l * 4 + r]] = pltpu.bitcast(bits & zero_ref[0], F32)

    def b_phase2(t, layers=(0, 1)):
        rows = slice(layers[0] * SEG, (layers[-1] + 1) * SEG)
        w = jnp.concatenate([pltpu.bitcast(pwo_ref[c], BF16) for c in range(NC)], axis=1)
        o = jnp.concatenate([bq_ref[c, rows, :] for c in range(NC)], axis=1).astype(BF16)
        yb = xb_ref[rows, :] + _nn(o, w)
        if 1 in layers:
            row = al(max(t - 3, 0) * SEG if isinstance(t, int) else jnp.maximum(t - 3, 0) * SEG, SEG)
            out_ref[pl.ds(row, SEG), :] = yb[-SEG:].astype(out_ref.dtype)
        return yb[:SEG]

    def x_seg(s):
        row = s * SEG if isinstance(s, int) else pl.multiple_of(s * SEG, SEG)
        return x_ref[pl.ds(row, SEG), :].astype(F32)

    def with_b(t, at_qkv, at_wo1, at_wo2, pin=False):
        box = {}
        pins = {}

        def hooks(p):
            if p == at_qkv - 0.5:
                b_phase1(t, pins=pins if pin and PINS else None)
            elif p == at_wo1 and at_wo2 == at_wo1:
                box['x2'] = b_phase2(t)
            elif p == at_wo1:
                box['x2'] = b_phase2(t, (0,))
            elif p == at_wo2:
                b_phase2(t, (1,))
            return pins.get(p)
        return hooks, box

    def prepare_next(t, x2):
        sn = jnp.minimum(t + 1, NSEG - 1)
        hx_ref[0:SEG, :] = hxa_ref[pl.ds(al(sn * SEG, SEG), SEG), :]
        hx_ref[SEG:, :] = _ln(x2).astype(BF16)
        res_ref[...] = _cat0(x_seg(sn), x2)

    def permuted_rows(c):
        rows = [st_ref[c, pl.ds(d, H, stride=BDH), :] for d in range(BDH)]
        return _cat0(*rows)

    bkv_ref[...] = jnp.zeros(bkv_ref.shape, F32)
    acc_ref[...] = jnp.zeros(acc_ref.shape, F32)
    zero_ref[0] = 0
    first[0].wait()
    xl0 = _ln(x_ref[0:X0 + XB, :].astype(F32)).astype(BF16)
    hxa_ref[0:X0 + XB, :] = xl0
    hx_ref[0:SEG, :] = xl0[0:SEG]

    def early(u, carry):
        rows = pl.ds(al((u // 3) * PW, 128), PW)
        pltpu.make_async_copy(wq_hbm.at[rows, :], wl_ref.at[u % 3, rows, :], qsem.at[u]).wait()
        w = wl_ref[u % 3, rows, :]
        wn_ref[u] = pltpu.bitcast(_cat0(*[transposed(w[:, c * 128:(c + 1) * 128]) for c in range(NC)]), U32)
        pre_ref[u, 2 * SEG:X0, :] = _nt(hxa_ref[2 * SEG:X0, :], w).astype(BF16)
        return carry

    lax.fori_loop(0, NPRE, early, 0)
    mem0_copy.wait()
    mem0 = mem0_ref[...].astype(F32)
    mem_ref[...] = _cat0(mem0, mem0)

    def step0(p, carry):
        group(p, lambda cp: cp.wait())
        u = jnp.minimum(p, NU - 1)

        def wfirst(m):
            w = wl_ref[m, pl.ds(al(p * PW, 128), PW), :]
            if m < 3:
                w = _cat0(*[transposed(w[:, c * 128:(c + 1) * 128]) for c in range(NC)])
                wt_ref[p * 3 + m] = pltpu.bitcast(w, U32)
                return weights(m, p) if RELOAD else w
            w_ref[pl.ds(al(p * (PW // 2), 64), PW // 2), :] = pltpu.bitcast(w, U32)
            return w

        _, arrange, scores, pv = attn_one_layer()
        h = _cat0(mem_ref[...].astype(BF16), hx_ref[0:SEG, :])
        xrows = x_rows(p)
        xl = hxa_ref[xrows, :]
        for c in range(NC):
            st_ref[0, c * 128:(c + 1) * 128, :] = bwqkv_ref[u, :, c * 128:(c + 1) * 128].astype(F32).T
        pwqkv_ref[u] = pltpu.bitcast(permuted_rows(0).T.astype(BF16), U32)
        done = [0]

        def pre(n):
            c0, c1 = done[0], min(done[0] + n, NPRE)
            done[0] = c1
            for c in range(c0, c1):
                pre_ref[c, xrows, :] = _nn(xl, pltpu.bitcast(wn_ref[c], BF16)).astype(BF16)

        pre(S0[0])
        q = _nn(h, wfirst(0)).astype(BF16)
        pre(S0[1])
        kt = arrange(_nn(h, wfirst(1)))
        pre(S0[2])
        s = scores(q, kt)
        pre(S0[3])
        vt = arrange(_nn(h, wfirst(2)))
        pre(S0[4])
        o = pv(s, vt)
        pre(NPRE)
        acc_ref[...] += _nn(o, wfirst(3))
        nrows = x_rows(u + 1)
        hxa_ref[nrows, :] = _ln(x_ref[nrows, :].astype(F32)).astype(BF16)
        issue_rest(p + WIN, 0)

        return carry

    lax.fori_loop(0, NPAIR, step0, 0)
    bw2.wait()
    for c in range(NC):
        st_ref[c] = bwo_ref[:, c * 128:(c + 1) * 128].astype(F32)
        pwo_ref[c] = pltpu.bitcast(permuted_rows(c).astype(BF16), U32)
    zeros = jnp.zeros((SEG, D), F32)
    mem_ref[0:M, :] = acc_ref[0:M, :]
    xb_ref[...] = _cat0(x_seg(0) + acc_ref[2 * M:, :], zeros)
    hx_ref[...] = _cat0(hxa_ref[SEG:2 * SEG, :], zeros.astype(BF16))
    res_ref[...] = _cat0(x_seg(1), zeros)

    def single(t, carry):
        l = (t >= NSEG).astype(jnp.int32)
        mrows = pl.ds(al(l * M, M), M)
        xrows = pl.ds(al(l * SEG, SEG), SEG)
        hooks, box = with_b(t, *SB)
        mem = mem_ref[mrows, :]
        h = _cat0(_cat0(mem, mem).astype(BF16), hx_ref[xrows, :])
        acc = a_phase(h, attn_one_layer(), hooks)
        mem_ref[mrows, :] = acc[:M]
        xb_ref[xrows, :] = res_ref[xrows, :] + acc[2 * M:]
        prepare_next(t, box['x2'])
        return carry

    def step(i, carry):
        for j in range(UNROLL):
            step1(i * UNROLL + j)
        return carry

    def step1(t):
        hooks, box = with_b(t, BQKV_AT, BWO_PAIR, BWO2_PAIR, True)
        h = _cat0(mem_ref[...].astype(BF16), hx_ref[...])
        acc = a_phase(h, attn_two_layers(), hooks, t)
        mem_ref[...] = acc[:2 * M]
        xb_ref[...] = res_ref[...] + acc[2 * M:]
        prepare_next(t, box['x2'])

    def outer(i, carry):
        lax.fori_loop(1 + (NSEG - 1) * i, 2 + NSEG * i, single, 0)
        lax.fori_loop(2 // UNROLL, (NSEG - (NSEG - 2) * i) // UNROLL, step, 0)
        pl.when(i == 0)(out_a.start)
        return carry

    lax.fori_loop(0, 2, outer, 0)
    b_phase1(NSEG + 2, (1,))
    b_phase2(NSEG + 2, (1,))
    out_b.start()
    out_a.wait()
    out_b.wait()


@jax.jit
def pallas_interleave_layers__memory_aug_recurrent_mem_tr__sliding_local_dilated__prompt_kernel(
    A_x, A_mem0, A_Wq, A_Wk, A_Wv, A_Wo, A_seg_len, B_x, B_wqkv, B_wo,
):
    del A_seg_len, B_x
    wt = lambda w: jnp.transpose(w, (1, 2, 0)).reshape(HD, D)
    hbm = pl.BlockSpec(memory_space=pl.ANY)
    out = pl.pallas_call(
        _kernel,
        out_shape=jax.ShapeDtypeStruct((S, D), A_x.dtype),
        in_specs=[hbm] * 8,
        out_specs=hbm,
        scratch_shapes=[
            pltpu.VMEM((S, D), BF16),
            pltpu.VMEM((S, D), BF16),
            pltpu.VMEM((4, HD, D), BF16),
            pltpu.VMEM((HD // 2, D), U32),
            pltpu.VMEM((3 * NPAIR, D // 2, PW), U32),
            pltpu.VMEM((NU, 128, D), BF16),
            pltpu.VMEM((D, D), BF16),
            pltpu.VMEM((NU, 64, D), U32),
            pltpu.VMEM((NC, D // 2, 128), U32),
            pltpu.VMEM((NC, D, 128), F32),
            pltpu.VMEM((R1, D), F32),
            pltpu.VMEM((2 * M, D), F32),
            pltpu.VMEM((2 * SEG, D), BF16),
            pltpu.VMEM((2 * SEG, D), F32),
            pltpu.VMEM((2 * SEG, D), F32),
            pltpu.VMEM((NC, 2 * SEG, 128), F32),
            pltpu.VMEM((2, 2, NC, 16 + SEG, 128), F32),
            pltpu.VMEM((NPRE, D // 2, PW), U32),
            pltpu.VMEM((S, D), BF16),
            pltpu.VMEM((NPRE, S, PW), BF16),
            pltpu.VMEM((M, D), BF16),
            pltpu.SMEM((1,), jnp.int32),
            pltpu.SemaphoreType.DMA((NPRE + 1,)),
            pltpu.SemaphoreType.DMA((NPAIR,)),
            pltpu.SemaphoreType.DMA((4,)),
        ],
        compiler_params=pltpu.CompilerParams(vmem_limit_bytes=120 * 2 ** 20),
    )(A_x.reshape(S, D), A_mem0.reshape(M, D), wt(A_Wq), wt(A_Wk), wt(A_Wv),
      A_Wo.reshape(HD, D), B_wqkv, B_wo)
    return out.reshape(1, S, D)
```

```python
import jax
import jax.numpy as jnp
from jax import lax
import jax.experimental.pallas as pl
import jax.experimental.pallas.tpu as pltpu

S, D = 2048, 640
H, DH = 32, 192
HD = H * DH
M, SEG = 8, 32
L = M + SEG
NSEG = S // SEG
R = 2 * L
R1 = 2 * M + SEG
NK = R + 4 * M
PW = 2 * DH
NPAIR = H // 2
BDH, BW, BDIL = 20, 8, 2
NC = D // 128
NU = 3 * NC
NPRE = 8
XB = 96
X0 = S - NPAIR * XB
WIN = 4
UNROLL = 2
HELD = 2
S0 = (2, 1, 1, 2, 1)
B_AT = (0, 7, 16)
B_AT1 = (0, 15, 15)
PINS = (2, 3, 4, 5, 8, 9, 10, 11)
F32, BF16, U32 = jnp.float32, jnp.bfloat16, jnp.uint32
LOG2E = 1.4426950408889634


def _ln(x):
    m = jnp.mean(x, axis=-1, keepdims=True)
    xc = x - m
    v = jnp.mean(xc * xc, axis=-1, keepdims=True)
    return xc * lax.rsqrt(v + 1e-5)


def _nt(a, b):
    return lax.dot_general(a, b, (((1,), (1,)), ((), ())), preferred_element_type=F32)


def _nn(a, b):
    return jnp.dot(a, b, preferred_element_type=F32)


def _cat0(*a):
    return jnp.concatenate(a, axis=0)


def _al(v, n):
    return v if isinstance(v, int) else pl.multiple_of(v, n)


def _iota(shape, dim):
    return lax.broadcasted_iota(jnp.int32, shape, dim)


def _transposed(w):
    return _cat0(*[w[:, c * 128:(c + 1) * 128].T for c in range(NC)])


def _kernel(x_hbm, mem0_hbm, wq_hbm, wk_hbm, wv_hbm, wo_hbm, bwqkv_hbm, bwo_hbm,
            out_hbm,
            x_ref, out_ref, wl_ref, wo_ref, wt_ref, bwqkv_ref, bwo_ref, pwqkv_ref, pwo_ref,
            st_ref, acc_ref, mem_ref, hx_ref, res_ref, xb_ref, bq_ref, bkv_ref, wn_ref,
            hxa_ref, pre_ref, mem0_ref, zero_ref, qsem, wsem, sem):
    w_hbm = (wq_hbm, wk_hbm, wv_hbm, wo_hbm)

    def w_copy(m, p, s):
        rows = pl.ds(_al(p * PW, 128), PW)
        return pltpu.make_async_copy(w_hbm[m].at[rows, :], wl_ref.at[m, rows, :], s)

    def x_rows(p):
        return pl.ds(_al(X0 + p * XB, 16), XB)

    def x_copy(p):
        return pltpu.make_async_copy(x_hbm.at[x_rows(p + 1), :], x_ref.at[x_rows(p + 1), :], wsem.at[p])

    def unit_copy(u):
        src = bwqkv_hbm.at[pl.ds(_al((u % NC) * 128, 128), 128), pl.ds(_al((u // NC) * D, 128), D)]
        return pltpu.make_async_copy(src, bwqkv_ref.at[u], wsem.at[u])

    def out_copy(r0, r1, s):
        return pltpu.make_async_copy(out_ref.at[pl.ds(r0, r1 - r0), :], out_hbm.at[pl.ds(r0, r1 - r0), :], s)

    x_head = pl.ds(0, X0 + XB)
    first = [pltpu.make_async_copy(x_hbm.at[x_head, :], x_ref.at[x_head, :], qsem.at[NPRE])] + [
        w_copy(c % 3, c // 3, qsem.at[c]) for c in range(NPRE)]
    mem0_copy = pltpu.make_async_copy(mem0_hbm, mem0_ref, sem.at[0])
    bwo_copy = pltpu.make_async_copy(bwo_hbm, bwo_ref, sem.at[1])
    out_a = out_copy(0, (NSEG - 3) * SEG, sem.at[2])
    out_b = out_copy((NSEG - 3) * SEG, S, sem.at[3])

    def issue_first(i, carry):
        for j, cp in enumerate(first):
            pl.when(i == j)(cp.start)
        return carry

    def group(p, act):
        for m in range(3):
            pl.when((p * 3 + m >= NPRE) & (p < NPAIR))(lambda m=m: act(w_copy(m, p, wsem.at[p])))

        @pl.when(p < NPAIR - 1)
        def _():
            act(unit_copy(p))
            act(x_copy(p))

        pl.when(p < NPAIR)(lambda: act(w_copy(3, p, wsem.at[p])))

    def issue_rest(p, carry):
        group(p, lambda cp: cp.start())
        pl.when(p == NPAIR)(bwo_copy.start)
        return carry

    lax.fori_loop(0, len(first), issue_first, 0)
    mem0_copy.start()
    lax.fori_loop(0, WIN, issue_rest, 0)

    scale = DH ** -0.5
    ninf = -jnp.inf

    def softmax2(s, sel, allowed):
        s = jnp.where(allowed, s, -1e9 / scale)
        m0 = jnp.max(jnp.where(sel, s, ninf), axis=-1, keepdims=True)
        m1 = jnp.max(jnp.where(sel, ninf, s), axis=-1, keepdims=True)
        e = jnp.exp2((s - jnp.where(sel, m0, m1)) * (scale * LOG2E))
        e0, e1 = jnp.where(sel, e, 0.0), jnp.where(sel, 0.0, e)
        d0 = jnp.sum(e0, axis=-1, keepdims=True)
        d1 = jnp.sum(e1, axis=-1, keepdims=True)
        return e, e0, e1, 1.0 / d0, 1.0 / d1

    def attn_two_layers():
        qi, ki = _iota((R, NK), 0), _iota((R, NK), 1)
        special = (qi >= R1) & (qi < R1 + M)
        kk = jnp.where(ki < L, ki, jnp.where(ki < R, ki - L, (ki - R) & (2 * M - 1)))
        qq = M + ((qi - 2 * M) & (SEG - 1))
        allowed = (special == (ki >= R)) & ((qi < 2 * M) | (kk <= qq))
        row_l1 = (qi < M) | ((qi >= 2 * M) & (qi < R1))
        is_a = jnp.where(special, ki - (R + 2 * M), jnp.where(row_l1, L - 1 - ki, ki - L)) >= 0
        lo = _iota((L, 128), 1) < 64
        lo_r = _iota((R, 128), 1) < 64
        g1 = lambda a: _cat0(a[0:M], a[2 * M:R1 + M])
        g2 = lambda a: _cat0(a[M:2 * M], a[R1 + M:])
        merge = lambda u1, u2: _cat0(u1[0:M], u2[0:M], u1[M:], u2[M:])

        def arrange_q(q):
            qm = q[:, 128:256]
            return [u.astype(BF16) for u in (q[:, :128], q[:, 256:], g1(qm), g2(qm))]

        def arrange(a):
            a1 = _cat0(a[0:M], a[2 * M:R1])
            a2 = _cat0(a[M:2 * M], a[R1:])
            cat = lambda *u: _cat0(*u).astype(BF16)
            m1, m2 = a1[:, 128:256], a2[:, 128:256]
            m2b, m2a = jnp.where(lo, 0.0, m2), jnp.where(lo, m2, 0.0)
            e = 2 * M
            return (cat(a1[:, :128], a2[:, :128], a2[:e, :128], a2[:e, :128]),
                    cat(a2[:, 256:], a1[:, 256:], a2[:e, 256:], a2[:e, 256:]),
                    cat(jnp.where(lo, m1, 0.0), jnp.where(lo, 0.0, m1), m2b[:e], m2a[:e]),
                    cat(m2b, m2a, m2b[:e], m2b[:e]))

        def scores(q, kt):
            return [_nt(u, w) for u, w in zip(q, kt)]

        def pv(s4, vt, pin):
            sa, sb, s1, s2 = s4
            if pin is not None:
                s1 = _cat0(s1[0:M] + pin[:, :NK], s1[M:])
            p, pa, pb, ra, rb = softmax2(jnp.where(is_a, sa, sb) + merge(s1, s2), is_a, allowed)
            oa, ob, o1, o2 = [_nn(u.astype(BF16), w) for u, w in zip((pa, pb, g1(p), g2(p)), vt)]
            return jnp.concatenate(
                [oa * ra, merge(o1, o2) * jnp.where(lo_r, ra, rb), ob * rb], axis=1).astype(BF16)

        return arrange_q, arrange, scores, pv

    def attn_one_layer():
        qi, ki = _iota((R1, R), 0), _iota((R1, R), 1)
        is_a = ki < L
        allowed = (qi < 2 * M) | (jnp.where(is_a, ki, ki - L) <= qi - M)
        head_a = _iota((L, PW), 1) < DH
        head_a1 = _iota((R1, PW), 1) < DH

        def arrange(a):
            a1 = _cat0(a[0:M], a[2 * M:])
            return _cat0(jnp.where(head_a, a1, 0.0), jnp.where(head_a, 0.0, a1)).astype(BF16)

        def pv(s, vt, pin=None):
            p, _, _, r0, r1 = softmax2(s, is_a, allowed)
            return (_nn(p.astype(BF16), vt) * jnp.where(head_a1, r0, r1)).astype(BF16)

        return lambda q: q.astype(BF16), arrange, _nt, pv

    def a_phase(h, attn, hooks, t=None):
        arrange_q, arrange, scores, pv = attn

        def proj(m, p):
            c = p * 3 + m
            w = pltpu.bitcast(wt_ref[c], BF16)
            if c >= NPRE or t is None:
                return _nn(h, w)
            y = _nn(_cat0(h[0:2 * M], h[R1:]), w)
            pre = pre_ref[c, pl.ds(_al(t * SEG, SEG), SEG), :].astype(F32)
            return _cat0(y[0:2 * M], pre, y[2 * M:])

        st = {'acc': None, 'o': {}, 'done': 0}

        def wo_upto(n):
            while st['done'] < n:
                pp = st['done']
                w = pltpu.bitcast(wo_ref[pp * PW // 2:(pp + 1) * PW // 2, :], BF16)
                y = _nn(st['o'].pop(pp), w)
                st['acc'] = y if st['acc'] is None else st['acc'] + y
                st['done'] += 1

        q, kt = arrange_q(proj(0, 0)), arrange(proj(1, 0))
        vt = arrange(proj(2, 0))
        for p in range(NPAIR):
            last = p == NPAIR - 1
            s = scores(q, kt)
            hooks(p - 0.5)
            if last:
                wo_upto(p - 1)
            else:
                q, kt = arrange_q(proj(0, p + 1)), arrange(proj(1, p + 1))
            st['o'][p] = pv(s, vt, hooks(p))
            if last:
                wo_upto(NPAIR)
            else:
                vt = arrange(proj(2, p + 1))
                wo_upto(min(p + 1, NPAIR - 1 - HELD))
        hooks(NPAIR)
        return st['acc']

    def b_phase1(t, layers=(0, 1), pins=None):
        w = jnp.concatenate([_cat0(*[pltpu.bitcast(pwqkv_ref[j * NC + c], BF16) for c in range(NC)])
                             for j in range(3)], axis=1)
        l0 = layers[0]
        qkv = _nn(_ln(xb_ref[l0 * SEG:(layers[-1] + 1) * SEG, :]).astype(BF16), w)
        for l in layers:
            rows = slice((l - l0) * SEG, (l - l0 + 1) * SEG)
            for c in range(NC):
                bq_ref[c, l * SEG:(l + 1) * SEG, :] = qkv[rows, c * 128:(c + 1) * 128]
                for j in range(2):
                    bkv_ref[l, j, c, 0:16, :] = bkv_ref[l, j, c, SEG:SEG + 16, :]
                    bkv_ref[l, j, c, 16:16 + SEG, :] = qkv[
                        rows, (j + 1) * D + c * 128:(j + 1) * D + (c + 1) * 128]
        bscale = BDH ** -0.5
        for l in layers:
            seg = t - 1 - 2 * l
            for r in range(SEG // 8):
                pos = seg * SEG + r * 8 + _iota((8, 128), 0)
                qrows = slice(l * SEG + r * 8, l * SEG + r * 8 + 8)
                kv = lambda j, c, w: bkv_ref[l, j, c, 16 + r * 8 - BDIL * w:24 + r * 8 - BDIL * w, :]
                q = [bq_ref[c, qrows, :] for c in range(NC)]
                lg = []
                for w in range(BW):
                    s = q[0] * kv(0, 0, w)
                    for c in range(1, NC):
                        s = s + q[c] * kv(0, c, w)
                    s = s + pltpu.roll(s, 64, 1)
                    s = s + pltpu.roll(s, 32, 1)
                    if r * 8 - BDIL * w < 0:
                        s = jnp.where(pos - BDIL * w >= 0, s, -1e9 / bscale)
                    lg.append(s)
                m = lg[0]
                for w in range(1, BW):
                    m = jnp.maximum(m, lg[w])
                e = [jnp.exp2((s - m) * (bscale * LOG2E)) for s in lg]
                den = e[0]
                for w in range(1, BW):
                    den = den + e[w]
                inv = 1.0 / den
                bits = None
                for c in range(NC):
                    o = e[0] * kv(1, c, 0)
                    for w in range(1, BW):
                        o = o + e[w] * kv(1, c, w)
                    o = o * inv
                    bq_ref[c, qrows, :] = o
                    ob = pltpu.bitcast(o, jnp.int32)
                    bits = ob if bits is None else bits | ob
                if pins is not None:
                    pins[PINS[l * 4 + r]] = pltpu.bitcast(bits & zero_ref[0], F32)

    def b_phase2(t, layers=(0, 1)):
        rows = slice(layers[0] * SEG, (layers[-1] + 1) * SEG)
        w = jnp.concatenate([pltpu.bitcast(pwo_ref[c], BF16) for c in range(NC)], axis=1)
        o = jnp.concatenate([bq_ref[c, rows, :] for c in range(NC)], axis=1).astype(BF16)
        yb = xb_ref[rows, :] + _nn(o, w)
        if 1 in layers:
            row = max(t - 3, 0) * SEG if isinstance(t, int) else jnp.maximum(t - 3, 0) * SEG
            out_ref[pl.ds(_al(row, SEG), SEG), :] = yb[-SEG:].astype(out_ref.dtype)
        return yb[:SEG]

    def with_b(t, at, pin):
        at_qkv, at_wo1, at_wo2 = at
        box, pins = {}, {}

        def hooks(p):
            if p == at_qkv - 0.5:
                b_phase1(t, pins=pins if pin else None)
            elif p == at_wo1 and at_wo2 == at_wo1:
                box['x2'] = b_phase2(t)
            elif p == at_wo1:
                box['x2'] = b_phase2(t, (0,))
            elif p == at_wo2:
                b_phase2(t, (1,))
            return pins.get(p)
        return hooks, box

    def x_seg(s):
        return x_ref[pl.ds(_al(s * SEG, SEG), SEG), :].astype(F32)

    def prepare_next(t, x2):
        sn = jnp.minimum(t + 1, NSEG - 1)
        hx_ref[0:SEG, :] = hxa_ref[pl.ds(_al(sn * SEG, SEG), SEG), :]
        hx_ref[SEG:, :] = _ln(x2).astype(BF16)
        res_ref[...] = _cat0(x_seg(sn), x2)

    def permuted_rows(c):
        return _cat0(*[st_ref[c, pl.ds(d, H, stride=BDH), :] for d in range(BDH)])

    bkv_ref[...] = jnp.zeros(bkv_ref.shape, F32)
    acc_ref[...] = jnp.zeros(acc_ref.shape, F32)
    st_ref[:, D:, :] = jnp.zeros((NC, st_ref.shape[1] - D, 128), F32)
    zero_ref[0] = 0
    first[0].wait()
    xl0 = _ln(x_ref[0:X0 + XB, :].astype(F32)).astype(BF16)
    hxa_ref[0:X0 + XB, :] = xl0
    hx_ref[0:SEG, :] = xl0[0:SEG]

    def early(u, carry):
        rows = pl.ds(_al((u // 3) * PW, 128), PW)
        dst = wl_ref.at[u % 3, rows, :]
        pltpu.make_async_copy(dst, dst, qsem.at[u]).wait()
        w = wl_ref[u % 3, rows, :]
        wn_ref[u] = pltpu.bitcast(_transposed(w), U32)
        pre_ref[u, 2 * SEG:X0, :] = _nt(hxa_ref[2 * SEG:X0, :], w).astype(BF16)
        return carry

    lax.fori_loop(0, NPRE, early, 0)
    mem0_copy.wait()
    mem0 = mem0_ref[...].astype(F32)
    mem_ref[...] = _cat0(mem0, mem0)

    def step0(p, carry):
        group(p, lambda cp: cp.wait())
        u = jnp.minimum(p, NU - 1)

        def wfirst(m):
            w = wl_ref[m, pl.ds(_al(p * PW, 128), PW), :]
            if m < 3:
                w = _transposed(w)
                wt_ref[p * 3 + m] = pltpu.bitcast(w, U32)
            else:
                wo_ref[pl.ds(_al(p * (PW // 2), 64), PW // 2), :] = pltpu.bitcast(w, U32)
            return w

        _, arrange, scores, pv = attn_one_layer()
        h = _cat0(mem_ref[...].astype(BF16), hx_ref[0:SEG, :])
        xrows = x_rows(p)
        xl = hxa_ref[xrows, :]
        for c in range(NC):
            st_ref[0, c * 128:(c + 1) * 128, :] = bwqkv_ref[u, :, c * 128:(c + 1) * 128].astype(F32).T
        pwqkv_ref[u] = pltpu.bitcast(permuted_rows(0).T.astype(BF16), U32)
        done = [0]

        def pre(n):
            c0, c1 = done[0], min(done[0] + n, NPRE)
            done[0] = c1
            for c in range(c0, c1):
                pre_ref[c, xrows, :] = _nn(xl, pltpu.bitcast(wn_ref[c], BF16)).astype(BF16)

        pre(S0[0])
        q = _nn(h, wfirst(0)).astype(BF16)
        pre(S0[1])
        kt = arrange(_nn(h, wfirst(1)))
        pre(S0[2])
        s = scores(q, kt)
        pre(S0[3])
        vt = arrange(_nn(h, wfirst(2)))
        pre(S0[4])
        o = pv(s, vt)
        pre(NPRE)
        acc_ref[...] += _nn(o, wfirst(3))
        nrows = x_rows(u + 1)
        hxa_ref[nrows, :] = _ln(x_ref[nrows, :].astype(F32)).astype(BF16)
        issue_rest(p + WIN, 0)
        return carry

    lax.fori_loop(0, NPAIR, step0, 0)
    bwo_copy.wait()
    for c in range(NC):
        st_ref[c, 0:D, :] = bwo_ref[:, c * 128:(c + 1) * 128].astype(F32)
        pwo_ref[c] = pltpu.bitcast(permuted_rows(c).astype(BF16), U32)
    zeros = jnp.zeros((SEG, D), F32)
    mem_ref[0:M, :] = acc_ref[0:M, :]
    xb_ref[...] = _cat0(x_seg(0) + acc_ref[2 * M:, :], zeros)
    hx_ref[...] = _cat0(hxa_ref[SEG:2 * SEG, :], zeros.astype(BF16))
    res_ref[...] = _cat0(x_seg(1), zeros)

    def single(t, carry):
        l = (t >= NSEG).astype(jnp.int32)
        mrows = pl.ds(_al(l * M, M), M)
        xrows = pl.ds(_al(l * SEG, SEG), SEG)
        hooks, box = with_b(t, B_AT1, False)
        mem = mem_ref[mrows, :]
        h = _cat0(_cat0(mem, mem).astype(BF16), hx_ref[xrows, :])
        acc = a_phase(h, attn_one_layer(), hooks)
        mem_ref[mrows, :] = acc[:M]
        xb_ref[xrows, :] = res_ref[xrows, :] + acc[2 * M:]
        prepare_next(t, box['x2'])
        return carry

    def step(i, carry):
        for j in range(UNROLL):
            t = i * UNROLL + j
            hooks, box = with_b(t, B_AT, True)
            h = _cat0(mem_ref[...].astype(BF16), hx_ref[...])
            acc = a_phase(h, attn_two_layers(), hooks, t)
            mem_ref[...] = acc[:2 * M]
            xb_ref[...] = res_ref[...] + acc[2 * M:]
            prepare_next(t, box['x2'])
        return carry

    def outer(i, carry):
        lax.fori_loop(1 + (NSEG - 1) * i, 2 + NSEG * i, single, 0)
        lax.fori_loop(2 // UNROLL, (NSEG - (NSEG - 2) * i) // UNROLL, step, 0)
        pl.when(i == 0)(out_a.start)
        return carry

    lax.fori_loop(0, 2, outer, 0)
    b_phase1(NSEG + 2, (1,))
    b_phase2(NSEG + 2, (1,))
    out_b.start()
    out_a.wait()
    out_b.wait()


@jax.jit
def pallas_interleave_layers__memory_aug_recurrent_mem_tr__sliding_local_dilated__prompt_kernel(
    A_x, A_mem0, A_Wq, A_Wk, A_Wv, A_Wo, A_seg_len, B_x, B_wqkv, B_wo,
):
    del A_seg_len, B_x
    wt = lambda w: jnp.transpose(w, (1, 2, 0)).reshape(HD, D)
    hbm = pl.BlockSpec(memory_space=pl.ANY)
    out = pl.pallas_call(
        _kernel,
        out_shape=jax.ShapeDtypeStruct((S, D), A_x.dtype),
        in_specs=[hbm] * 8,
        out_specs=hbm,
        scratch_shapes=[
            pltpu.VMEM((S, D), BF16),
            pltpu.VMEM((S, D), BF16),
            pltpu.VMEM((4, HD, D), BF16),
            pltpu.VMEM((HD // 2, D), U32),
            pltpu.VMEM((3 * NPAIR, D // 2, PW), U32),
            pltpu.VMEM((NU, 128, D), BF16),
            pltpu.VMEM((D, D), BF16),
            pltpu.VMEM((NU, 64, D), U32),
            pltpu.VMEM((NC, D // 2, 128), U32),
            pltpu.VMEM((NC, D + 32, 128), F32),
            pltpu.VMEM((R1, D), F32),
            pltpu.VMEM((2 * M, D), F32),
            pltpu.VMEM((2 * SEG, D), BF16),
            pltpu.VMEM((2 * SEG, D), F32),
            pltpu.VMEM((2 * SEG, D), F32),
            pltpu.VMEM((NC, 2 * SEG, 128), F32),
            pltpu.VMEM((2, 2, NC, 16 + SEG, 128), F32),
            pltpu.VMEM((NPRE, D // 2, PW), U32),
            pltpu.VMEM((S, D), BF16),
            pltpu.VMEM((NPRE, S, PW), BF16),
            pltpu.VMEM((M, D), BF16),
            pltpu.SMEM((1,), jnp.int32),
            pltpu.SemaphoreType.DMA((NPRE + 1,)),
            pltpu.SemaphoreType.DMA((NPAIR,)),
            pltpu.SemaphoreType.DMA((4,)),
        ],
        compiler_params=pltpu.CompilerParams(vmem_limit_bytes=120 * 2 ** 20, disable_bounds_checks=True),
    )(A_x.reshape(S, D), A_mem0.reshape(M, D), wt(A_Wq), wt(A_Wk), wt(A_Wv),
      A_Wo.reshape(HD, D), B_wqkv, B_wo)
    return out.reshape(1, S, D)
```

```python
import jax
import jax.numpy as jnp
from jax import lax
import jax.experimental.pallas as pl
import jax.experimental.pallas.tpu as pltpu

S, D = 2048, 640
H, DH = 32, 192
HD = H * DH
M, SEG = 8, 32
L = M + SEG
NSEG = S // SEG
R = 2 * L
R1 = 2 * M + SEG
NK = R + 4 * M
PW = 2 * DH
NPAIR = H // 2
BDH, BW, BDIL = 20, 8, 2
NC = D // 128
NU = 3 * NC
NPRE = 8
XB = 96
X0 = S - NPAIR * XB
WIN = 4
UNROLL = 2
HELD = 2
S0 = (2, 1, 1, 2, 1)
B_AT = (0, 15, 16)
B_AT1 = (0, 15, 15)
PINS = (2, 3, 4, 5, 8, 9, 10, 11)
F32, BF16, U32 = jnp.float32, jnp.bfloat16, jnp.uint32
LOG2E = 1.4426950408889634


def _ln(x):
    m = jnp.mean(x, axis=-1, keepdims=True)
    xc = x - m
    v = jnp.mean(xc * xc, axis=-1, keepdims=True)
    return xc * lax.rsqrt(v + 1e-5)


def _nt(a, b):
    return lax.dot_general(a, b, (((1,), (1,)), ((), ())), preferred_element_type=F32)


def _nn(a, b):
    return jnp.dot(a, b, preferred_element_type=F32)


def _cat0(*a):
    return jnp.concatenate(a, axis=0)


def _al(v, n):
    return v if isinstance(v, int) else pl.multiple_of(v, n)


def _iota(shape, dim):
    return lax.broadcasted_iota(jnp.int32, shape, dim)


def _transposed(w):
    return _cat0(*[w[:, c * 128:(c + 1) * 128].T for c in range(NC)])


def _kernel(x_hbm, mem0_hbm, wq_hbm, wk_hbm, wv_hbm, wo_hbm, bwqkv_hbm, bwo_hbm,
            out_hbm,
            x_ref, out_ref, wl_ref, wo_ref, wt_ref, bwqkv_ref, bwo_ref, pwqkv_ref, pwo_ref,
            st_ref, acc_ref, mem_ref, hx_ref, res_ref, xb_ref, bq_ref, bkv_ref, wn_ref,
            hxa_ref, pre_ref, mem0_ref, zero_ref, qsem, wsem, sem):
    w_hbm = (wq_hbm, wk_hbm, wv_hbm, wo_hbm)

    def w_copy(m, p, s):
        rows = pl.ds(_al(p * PW, 128), PW)
        return pltpu.make_async_copy(w_hbm[m].at[rows, :], wl_ref.at[m, rows, :], s)

    def x_rows(p):
        return pl.ds(_al(X0 + p * XB, 16), XB)

    def x_copy(p):
        return pltpu.make_async_copy(x_hbm.at[x_rows(p + 1), :], x_ref.at[x_rows(p + 1), :], wsem.at[p])

    def unit_copy(u):
        src = bwqkv_hbm.at[pl.ds(_al((u % NC) * 128, 128), 128), pl.ds(_al((u // NC) * D, 128), D)]
        return pltpu.make_async_copy(src, bwqkv_ref.at[u], wsem.at[u])

    def out_copy(r0, r1, s):
        return pltpu.make_async_copy(out_ref.at[pl.ds(r0, r1 - r0), :], out_hbm.at[pl.ds(r0, r1 - r0), :], s)

    x_head = pl.ds(0, X0 + XB)
    first = [pltpu.make_async_copy(x_hbm.at[x_head, :], x_ref.at[x_head, :], qsem.at[NPRE])] + [
        w_copy(c % 3, c // 3, qsem.at[c]) for c in range(NPRE)]
    mem0_copy = pltpu.make_async_copy(mem0_hbm, mem0_ref, sem.at[0])
    bwo_copy = pltpu.make_async_copy(bwo_hbm, bwo_ref, sem.at[1])
    out_a = out_copy(0, (NSEG - 3) * SEG, sem.at[2])
    out_b = out_copy((NSEG - 3) * SEG, S, sem.at[3])

    def issue_first(i, carry):
        for j, cp in enumerate(first):
            pl.when(i == j)(cp.start)
        return carry

    def group(p, act):
        for m in range(3):
            pl.when((p * 3 + m >= NPRE) & (p < NPAIR))(lambda m=m: act(w_copy(m, p, wsem.at[p])))

        @pl.when(p < NPAIR - 1)
        def _():
            act(unit_copy(p))
            act(x_copy(p))

        pl.when(p < NPAIR)(lambda: act(w_copy(3, p, wsem.at[p])))

    def issue_rest(p, carry):
        group(p, lambda cp: cp.start())
        pl.when(p == NPAIR)(bwo_copy.start)
        return carry

    lax.fori_loop(0, len(first), issue_first, 0)
    mem0_copy.start()
    lax.fori_loop(0, WIN, issue_rest, 0)

    scale = DH ** -0.5
    ninf = -jnp.inf

    def softmax2(s, sel, allowed):
        s = jnp.where(allowed, s, -1e9 / scale)
        m0 = jnp.max(jnp.where(sel, s, ninf), axis=-1, keepdims=True)
        m1 = jnp.max(jnp.where(sel, ninf, s), axis=-1, keepdims=True)
        e = jnp.exp2((s - jnp.where(sel, m0, m1)) * (scale * LOG2E))
        e0, e1 = jnp.where(sel, e, 0.0), jnp.where(sel, 0.0, e)
        d0 = jnp.sum(e0, axis=-1, keepdims=True)
        d1 = jnp.sum(e1, axis=-1, keepdims=True)
        return e, e0, e1, 1.0 / d0, 1.0 / d1

    def attn_two_layers():
        qi, ki = _iota((R, NK), 0), _iota((R, NK), 1)
        special = (qi >= R1) & (qi < R1 + M)
        kk = jnp.where(ki < L, ki, jnp.where(ki < R, ki - L, (ki - R) & (2 * M - 1)))
        qq = M + ((qi - 2 * M) & (SEG - 1))
        allowed = (special == (ki >= R)) & ((qi < 2 * M) | (kk <= qq))
        row_l1 = (qi < M) | ((qi >= 2 * M) & (qi < R1))
        is_a = jnp.where(special, ki - (R + 2 * M), jnp.where(row_l1, L - 1 - ki, ki - L)) >= 0
        lo = _iota((L, 128), 1) < 64
        lo_r = _iota((R, 128), 1) < 64
        g1 = lambda a: _cat0(a[0:M], a[2 * M:R1 + M])
        g2 = lambda a: _cat0(a[M:2 * M], a[R1 + M:])
        merge = lambda u1, u2: _cat0(u1[0:M], u2[0:M], u1[M:], u2[M:])

        def arrange_q(q):
            qm = q[:, 128:256]
            return [u.astype(BF16) for u in (q[:, :128], q[:, 256:], g1(qm), g2(qm))]

        def arrange(a):
            a1 = _cat0(a[0:M], a[2 * M:R1])
            a2 = _cat0(a[M:2 * M], a[R1:])
            cat = lambda *u: _cat0(*u).astype(BF16)
            m1, m2 = a1[:, 128:256], a2[:, 128:256]
            m2b, m2a = jnp.where(lo, 0.0, m2), jnp.where(lo, m2, 0.0)
            e = 2 * M
            return (cat(a1[:, :128], a2[:, :128], a2[:e, :128], a2[:e, :128]),
                    cat(a2[:, 256:], a1[:, 256:], a2[:e, 256:], a2[:e, 256:]),
                    cat(jnp.where(lo, m1, 0.0), jnp.where(lo, 0.0, m1), m2b[:e], m2a[:e]),
                    cat(m2b, m2a, m2b[:e], m2b[:e]))

        def scores(q, kt):
            return [_nt(u, w) for u, w in zip(q, kt)]

        def pv(s4, vt, pin):
            sa, sb, s1, s2 = s4
            if pin is not None:
                s1 = _cat0(s1[0:M] + pin[:, :NK], s1[M:])
            p, pa, pb, ra, rb = softmax2(jnp.where(is_a, sa, sb) + merge(s1, s2), is_a, allowed)
            oa, ob, o1, o2 = [_nn(u.astype(BF16), w) for u, w in zip((pa, pb, g1(p), g2(p)), vt)]
            return jnp.concatenate(
                [oa * ra, merge(o1, o2) * jnp.where(lo_r, ra, rb), ob * rb], axis=1).astype(BF16)

        return arrange_q, arrange, scores, pv

    def attn_one_layer():
        qi, ki = _iota((R1, R), 0), _iota((R1, R), 1)
        is_a = ki < L
        allowed = (qi < 2 * M) | (jnp.where(is_a, ki, ki - L) <= qi - M)
        head_a = _iota((L, PW), 1) < DH
        head_a1 = _iota((R1, PW), 1) < DH

        def arrange(a):
            a1 = _cat0(a[0:M], a[2 * M:])
            return _cat0(jnp.where(head_a, a1, 0.0), jnp.where(head_a, 0.0, a1)).astype(BF16)

        def pv(s, vt, pin=None):
            if pin is not None:
                s = _cat0(s[0:M] + pin[:, :R], s[M:])
            p, _, _, r0, r1 = softmax2(s, is_a, allowed)
            return (_nn(p.astype(BF16), vt) * jnp.where(head_a1, r0, r1)).astype(BF16)

        return lambda q: q.astype(BF16), arrange, _nt, pv

    def a_phase(h, attn, hooks, t=None):
        arrange_q, arrange, scores, pv = attn

        def proj(m, p):
            c = p * 3 + m
            w = pltpu.bitcast(wt_ref[c], BF16)
            if c >= NPRE or t is None:
                return _nn(h, w)
            y = _nn(_cat0(h[0:2 * M], h[R1:]), w)
            pre = pre_ref[c, pl.ds(_al(t * SEG, SEG), SEG), :].astype(F32)
            return _cat0(y[0:2 * M], pre, y[2 * M:])

        st = {'acc': None, 'o': {}, 'done': 0}

        def wo_upto(n):
            while st['done'] < n:
                pp = st['done']
                w = pltpu.bitcast(wo_ref[pp * PW // 2:(pp + 1) * PW // 2, :], BF16)
                y = _nn(st['o'].pop(pp), w)
                st['acc'] = y if st['acc'] is None else st['acc'] + y
                st['done'] += 1

        q, kt = arrange_q(proj(0, 0)), arrange(proj(1, 0))
        vt = arrange(proj(2, 0))
        for p in range(NPAIR):
            last = p == NPAIR - 1
            s = scores(q, kt)
            hooks(p - 0.5)
            if last:
                wo_upto(p - 1)
            else:
                q, kt = arrange_q(proj(0, p + 1)), arrange(proj(1, p + 1))
            st['o'][p] = pv(s, vt, hooks(p))
            if last:
                wo_upto(NPAIR)
            else:
                vt = arrange(proj(2, p + 1))
                wo_upto(min(p + 1, NPAIR - 1 - HELD))
        hooks(NPAIR)
        return st['acc']

    def b_phase1(t, layers=(0, 1), pins=None):
        w = jnp.concatenate([_cat0(*[pltpu.bitcast(pwqkv_ref[j * NC + c], BF16) for c in range(NC)])
                             for j in range(3)], axis=1)
        l0 = layers[0]
        qkv = _nn(_ln(xb_ref[l0 * SEG:(layers[-1] + 1) * SEG, :]).astype(BF16), w)
        for l in layers:
            rows = slice((l - l0) * SEG, (l - l0 + 1) * SEG)
            for c in range(NC):
                bq_ref[c, l * SEG:(l + 1) * SEG, :] = qkv[rows, c * 128:(c + 1) * 128]
                for j in range(2):
                    bkv_ref[l, j, c, 0:16, :] = bkv_ref[l, j, c, SEG:SEG + 16, :]
                    bkv_ref[l, j, c, 16:16 + SEG, :] = qkv[
                        rows, (j + 1) * D + c * 128:(j + 1) * D + (c + 1) * 128]
        bscale = BDH ** -0.5
        for l in layers:
            seg = t - 1 - 2 * l
            for r in range(SEG // 8):
                pos = seg * SEG + r * 8 + _iota((8, 128), 0)
                qrows = slice(l * SEG + r * 8, l * SEG + r * 8 + 8)
                kv = lambda j, c, w: bkv_ref[l, j, c, 16 + r * 8 - BDIL * w:24 + r * 8 - BDIL * w, :]
                q = [bq_ref[c, qrows, :] for c in range(NC)]
                lg = []
                for w in range(BW):
                    s = q[0] * kv(0, 0, w)
                    for c in range(1, NC):
                        s = s + q[c] * kv(0, c, w)
                    s = s + pltpu.roll(s, 64, 1)
                    s = s + pltpu.roll(s, 32, 1)
                    if r * 8 - BDIL * w < 0:
                        s = jnp.where(pos - BDIL * w >= 0, s, -1e9 / bscale)
                    lg.append(s)
                m = lg[0]
                for w in range(1, BW):
                    m = jnp.maximum(m, lg[w])
                e = [jnp.exp2((s - m) * (bscale * LOG2E)) for s in lg]
                den = e[0]
                for w in range(1, BW):
                    den = den + e[w]
                inv = 1.0 / den
                bits = None
                for c in range(NC):
                    o = e[0] * kv(1, c, 0)
                    for w in range(1, BW):
                        o = o + e[w] * kv(1, c, w)
                    o = o * inv
                    bq_ref[c, qrows, :] = o
                    ob = pltpu.bitcast(o, jnp.int32)
                    bits = ob if bits is None else bits | ob
                if pins is not None:
                    pins[PINS[l * 4 + r]] = pltpu.bitcast(bits & zero_ref[0], F32)

    def b_phase2(t, layers=(0, 1)):
        rows = slice(layers[0] * SEG, (layers[-1] + 1) * SEG)
        w = jnp.concatenate([pltpu.bitcast(pwo_ref[c], BF16) for c in range(NC)], axis=1)
        o = jnp.concatenate([bq_ref[c, rows, :] for c in range(NC)], axis=1).astype(BF16)
        yb = xb_ref[rows, :] + _nn(o, w)
        if 1 in layers:
            row = max(t - 3, 0) * SEG if isinstance(t, int) else jnp.maximum(t - 3, 0) * SEG
            out_ref[pl.ds(_al(row, SEG), SEG), :] = yb[-SEG:].astype(out_ref.dtype)
        return yb[:SEG]

    def with_b(t, at):
        at_qkv, at_wo1, at_wo2 = at
        box, pins = {}, {}

        def hooks(p):
            if p == at_qkv - 0.5:
                b_phase1(t, pins=pins)
            elif p == at_wo1 and at_wo2 == at_wo1:
                box['x2'] = b_phase2(t)
            elif p == at_wo1:
                box['x2'] = b_phase2(t, (0,))
            elif p == at_wo2:
                b_phase2(t, (1,))
            return pins.get(p)
        return hooks, box

    def x_seg(s):
        return x_ref[pl.ds(_al(s * SEG, SEG), SEG), :].astype(F32)

    def prepare_next(t, x2):
        sn = jnp.minimum(t + 1, NSEG - 1)
        hx_ref[0:SEG, :] = hxa_ref[pl.ds(_al(sn * SEG, SEG), SEG), :]
        hx_ref[SEG:, :] = _ln(x2).astype(BF16)
        res_ref[...] = _cat0(x_seg(sn), x2)

    def permuted_rows(c):
        return _cat0(*[st_ref[c, pl.ds(d, H, stride=BDH), :] for d in range(BDH)])

    bkv_ref[...] = jnp.zeros(bkv_ref.shape, F32)
    acc_ref[...] = jnp.zeros(acc_ref.shape, F32)
    st_ref[:, D:, :] = jnp.zeros((NC, st_ref.shape[1] - D, 128), F32)
    zero_ref[0] = 0
    first[0].wait()
    xl0 = _ln(x_ref[0:X0 + XB, :].astype(F32)).astype(BF16)
    hxa_ref[0:X0 + XB, :] = xl0
    hx_ref[0:SEG, :] = xl0[0:SEG]

    def early(u, carry):
        rows = pl.ds(_al((u // 3) * PW, 128), PW)
        dst = wl_ref.at[u % 3, rows, :]
        pltpu.make_async_copy(dst, dst, qsem.at[u]).wait()
        w = wl_ref[u % 3, rows, :]
        wn_ref[u] = pltpu.bitcast(_transposed(w), U32)
        pre_ref[u, 2 * SEG:X0, :] = _nt(hxa_ref[2 * SEG:X0, :], w).astype(BF16)
        return carry

    lax.fori_loop(0, NPRE, early, 0)
    mem0_copy.wait()
    mem0 = mem0_ref[...].astype(F32)
    mem_ref[...] = _cat0(mem0, mem0)

    def step0(p, carry):
        group(p, lambda cp: cp.wait())
        u = jnp.minimum(p, NU - 1)

        def wfirst(m):
            w = wl_ref[m, pl.ds(_al(p * PW, 128), PW), :]
            if m < 3:
                w = _transposed(w)
                wt_ref[p * 3 + m] = pltpu.bitcast(w, U32)
            else:
                wo_ref[pl.ds(_al(p * (PW // 2), 64), PW // 2), :] = pltpu.bitcast(w, U32)
            return w

        _, arrange, scores, pv = attn_one_layer()
        h = _cat0(mem_ref[...].astype(BF16), hx_ref[0:SEG, :])
        xrows = x_rows(p)
        xl = hxa_ref[xrows, :]
        for c in range(NC):
            st_ref[0, c * 128:(c + 1) * 128, :] = bwqkv_ref[u, :, c * 128:(c + 1) * 128].astype(F32).T
        pwqkv_ref[u] = pltpu.bitcast(permuted_rows(0).T.astype(BF16), U32)
        done = [0]

        def pre(n):
            c0, c1 = done[0], min(done[0] + n, NPRE)
            done[0] = c1
            for c in range(c0, c1):
                pre_ref[c, xrows, :] = _nn(xl, pltpu.bitcast(wn_ref[c], BF16)).astype(BF16)

        pre(S0[0])
        q = _nn(h, wfirst(0)).astype(BF16)
        pre(S0[1])
        kt = arrange(_nn(h, wfirst(1)))
        pre(S0[2])
        s = scores(q, kt)
        pre(S0[3])
        vt = arrange(_nn(h, wfirst(2)))
        pre(S0[4])
        o = pv(s, vt)
        pre(NPRE)
        acc_ref[...] += _nn(o, wfirst(3))
        nrows = x_rows(u + 1)
        hxa_ref[nrows, :] = _ln(x_ref[nrows, :].astype(F32)).astype(BF16)
        issue_rest(p + WIN, 0)
        return carry

    lax.fori_loop(0, NPAIR, step0, 0)
    bwo_copy.wait()
    for c in range(NC):
        st_ref[c, 0:D, :] = bwo_ref[:, c * 128:(c + 1) * 128].astype(F32)
        pwo_ref[c] = pltpu.bitcast(permuted_rows(c).astype(BF16), U32)
    zeros = jnp.zeros((SEG, D), F32)
    mem_ref[0:M, :] = acc_ref[0:M, :]
    xb_ref[...] = _cat0(x_seg(0) + acc_ref[2 * M:, :], zeros)
    hx_ref[...] = _cat0(hxa_ref[SEG:2 * SEG, :], zeros.astype(BF16))
    res_ref[...] = _cat0(x_seg(1), zeros)

    def single(t, carry):
        l = (t >= NSEG).astype(jnp.int32)
        mrows = pl.ds(_al(l * M, M), M)
        xrows = pl.ds(_al(l * SEG, SEG), SEG)
        hooks, box = with_b(t, B_AT1)
        mem = mem_ref[mrows, :]
        h = _cat0(_cat0(mem, mem).astype(BF16), hx_ref[xrows, :])
        acc = a_phase(h, attn_one_layer(), hooks)
        mem_ref[mrows, :] = acc[:M]
        xb_ref[xrows, :] = res_ref[xrows, :] + acc[2 * M:]
        prepare_next(t, box['x2'])
        return carry

    def step(i, carry):
        for j in range(UNROLL):
            t = i * UNROLL + j
            hooks, box = with_b(t, B_AT)
            h = _cat0(mem_ref[...].astype(BF16), hx_ref[...])
            acc = a_phase(h, attn_two_layers(), hooks, t)
            mem_ref[...] = acc[:2 * M]
            xb_ref[...] = res_ref[...] + acc[2 * M:]
            prepare_next(t, box['x2'])
        return carry

    def outer(i, carry):
        lax.fori_loop(1 + (NSEG - 1) * i, 2 + NSEG * i, single, 0)
        lax.fori_loop(2 // UNROLL, (NSEG - (NSEG - 2) * i) // UNROLL, step, 0)
        pl.when(i == 0)(out_a.start)
        return carry

    lax.fori_loop(0, 2, outer, 0)
    b_phase1(NSEG + 2, (1,))
    b_phase2(NSEG + 2, (1,))
    out_b.start()
    out_a.wait()
    out_b.wait()


@jax.jit
def pallas_interleave_layers__memory_aug_recurrent_mem_tr__sliding_local_dilated__prompt_kernel(
    A_x, A_mem0, A_Wq, A_Wk, A_Wv, A_Wo, A_seg_len, B_x, B_wqkv, B_wo,
):
    del A_seg_len, B_x
    wt = lambda w: jnp.transpose(w, (1, 2, 0)).reshape(HD, D)
    hbm = pl.BlockSpec(memory_space=pl.ANY)
    out = pl.pallas_call(
        _kernel,
        out_shape=jax.ShapeDtypeStruct((S, D), A_x.dtype),
        in_specs=[hbm] * 8,
        out_specs=hbm,
        scratch_shapes=[
            pltpu.VMEM((S, D), BF16),
            pltpu.VMEM((S, D), BF16),
            pltpu.VMEM((4, HD, D), BF16),
            pltpu.VMEM((HD // 2, D), U32),
            pltpu.VMEM((3 * NPAIR, D // 2, PW), U32),
            pltpu.VMEM((NU, 128, D), BF16),
            pltpu.VMEM((D, D), BF16),
            pltpu.VMEM((NU, 64, D), U32),
            pltpu.VMEM((NC, D // 2, 128), U32),
            pltpu.VMEM((NC, D + 32, 128), F32),
            pltpu.VMEM((R1, D), F32),
            pltpu.VMEM((2 * M, D), F32),
            pltpu.VMEM((2 * SEG, D), BF16),
            pltpu.VMEM((2 * SEG, D), F32),
            pltpu.VMEM((2 * SEG, D), F32),
            pltpu.VMEM((NC, 2 * SEG, 128), F32),
            pltpu.VMEM((2, 2, NC, 16 + SEG, 128), F32),
            pltpu.VMEM((NPRE, D // 2, PW), U32),
            pltpu.VMEM((S, D), BF16),
            pltpu.VMEM((NPRE, S, PW), BF16),
            pltpu.VMEM((M, D), BF16),
            pltpu.SMEM((1,), jnp.int32),
            pltpu.SemaphoreType.DMA((NPRE + 1,)),
            pltpu.SemaphoreType.DMA((NPAIR,)),
            pltpu.SemaphoreType.DMA((4,)),
        ],
        compiler_params=pltpu.CompilerParams(vmem_limit_bytes=120 * 2 ** 20, disable_bounds_checks=True),
    )(A_x.reshape(S, D), A_mem0.reshape(M, D), wt(A_Wq), wt(A_Wk), wt(A_Wv),
      A_Wo.reshape(HD, D), B_wqkv, B_wo)
    return out.reshape(1, S, D)
```

```python
import jax
import jax.numpy as jnp
from jax import lax
import jax.experimental.pallas as pl
import jax.experimental.pallas.tpu as pltpu

S, D = 2048, 640
H, DH = 32, 192
HD = H * DH
M, SEG = 8, 32
L = M + SEG
NSEG = S // SEG
R = 2 * L
R1 = 2 * M + SEG
NK = R + 4 * M
PW = 2 * DH
NPAIR = H // 2
BDH, BW, BDIL = 20, 8, 2
NC = D // 128
NU = 3 * NC
NPRE = 8
XB = 96
X0 = S - NPAIR * XB
WIN = 4
UNROLL = 2
HELD = 2
S0 = (2, 1, 1, 2, 1)
B_AT = (0, 15, 16)
B_AT1 = (0, 15, 15)
PINS = (2, 3, 4, 5, 8, 9, 10, 11)
F32, BF16, U32 = jnp.float32, jnp.bfloat16, jnp.uint32
LOG2E = 1.4426950408889634


def _ln(x):
    m = jnp.mean(x, axis=-1, keepdims=True)
    xc = x - m
    v = jnp.mean(xc * xc, axis=-1, keepdims=True)
    return xc * lax.rsqrt(v + 1e-5)


def _nt(a, b):
    return lax.dot_general(a, b, (((1,), (1,)), ((), ())), preferred_element_type=F32)


def _nn(a, b):
    return jnp.dot(a, b, preferred_element_type=F32)


def _cat0(*a):
    return jnp.concatenate(a, axis=0)


def _al(v, n):
    return v if isinstance(v, int) else pl.multiple_of(v, n)


def _iota(shape, dim):
    return lax.broadcasted_iota(jnp.int32, shape, dim)


def _transposed(w):
    return _cat0(*[w[:, c * 128:(c + 1) * 128].T for c in range(NC)])


def _kernel(x_hbm, mem0_hbm, wq_hbm, wk_hbm, wv_hbm, wo_hbm, bwqkv_hbm, bwo_hbm,
            out_hbm,
            x_ref, out_ref, wl_ref, wo_ref, wt_ref, bwqkv_ref, bwo_ref, pwqkv_ref, pwo_ref,
            st_ref, acc_ref, mem_ref, hx_ref, res_ref, xb_ref, bq_ref, bkv_ref, wn_ref,
            hxa_ref, pre_ref, mem0_ref, zero_ref, qsem, wsem, sem):
    w_hbm = (wq_hbm, wk_hbm, wv_hbm, wo_hbm)

    def w_copy(m, p, s):
        rows = pl.ds(_al(p * PW, 128), PW)
        return pltpu.make_async_copy(w_hbm[m].at[rows, :], wl_ref.at[m, rows, :], s)

    def x_rows(p):
        return pl.ds(_al(X0 + p * XB, 16), XB)

    def x_copy(p):
        return pltpu.make_async_copy(x_hbm.at[x_rows(p + 1), :], x_ref.at[x_rows(p + 1), :], wsem.at[p])

    def unit_copy(u):
        src = bwqkv_hbm.at[pl.ds(_al((u % NC) * 128, 128), 128), pl.ds(_al((u // NC) * D, 128), D)]
        return pltpu.make_async_copy(src, bwqkv_ref.at[u], wsem.at[u])

    def out_copy(r0, r1, s):
        return pltpu.make_async_copy(out_ref.at[pl.ds(r0, r1 - r0), :], out_hbm.at[pl.ds(r0, r1 - r0), :], s)

    x_head = pl.ds(0, X0 + XB)
    first = [pltpu.make_async_copy(x_hbm.at[x_head, :], x_ref.at[x_head, :], qsem.at[NPRE])] + [
        w_copy(c % 3, c // 3, qsem.at[c]) for c in range(NPRE)]
    mem0_copy = pltpu.make_async_copy(mem0_hbm, mem0_ref, sem.at[0])
    bwo_copy = pltpu.make_async_copy(bwo_hbm, bwo_ref, sem.at[1])
    out_a = out_copy(0, (NSEG - 3) * SEG, sem.at[2])
    out_b = out_copy((NSEG - 3) * SEG, (NSEG - 1) * SEG, sem.at[3])
    out_c = out_copy((NSEG - 1) * SEG, S, sem.at[4])

    def issue_first(i, carry):
        for j, cp in enumerate(first):
            pl.when(i == j)(cp.start)
        return carry

    def group(p, act):
        for m in range(3):
            pl.when((p * 3 + m >= NPRE) & (p < NPAIR))(lambda m=m: act(w_copy(m, p, wsem.at[p])))

        @pl.when(p < NPAIR - 1)
        def _():
            act(unit_copy(p))
            act(x_copy(p))

        pl.when(p < NPAIR)(lambda: act(w_copy(3, p, wsem.at[p])))

    def issue_rest(p, carry):
        group(p, lambda cp: cp.start())
        pl.when(p == NPAIR)(bwo_copy.start)
        return carry

    lax.fori_loop(0, len(first), issue_first, 0)
    mem0_copy.start()
    lax.fori_loop(0, WIN, issue_rest, 0)

    scale = DH ** -0.5
    ninf = -jnp.inf

    def softmax2(s, sel, allowed):
        s = jnp.where(allowed, s, -1e9 / scale)
        m0 = jnp.max(jnp.where(sel, s, ninf), axis=-1, keepdims=True)
        m1 = jnp.max(jnp.where(sel, ninf, s), axis=-1, keepdims=True)
        e = jnp.exp2((s - jnp.where(sel, m0, m1)) * (scale * LOG2E))
        e0, e1 = jnp.where(sel, e, 0.0), jnp.where(sel, 0.0, e)
        d0 = jnp.sum(e0, axis=-1, keepdims=True)
        d1 = jnp.sum(e1, axis=-1, keepdims=True)
        return e, e0, e1, 1.0 / d0, 1.0 / d1

    def attn_two_layers():
        qi, ki = _iota((R, NK), 0), _iota((R, NK), 1)
        special = (qi >= R1) & (qi < R1 + M)
        kk = jnp.where(ki < L, ki, jnp.where(ki < R, ki - L, (ki - R) & (2 * M - 1)))
        qq = M + ((qi - 2 * M) & (SEG - 1))
        allowed = (special == (ki >= R)) & ((qi < 2 * M) | (kk <= qq))
        row_l1 = (qi < M) | ((qi >= 2 * M) & (qi < R1))
        is_a = jnp.where(special, ki - (R + 2 * M), jnp.where(row_l1, L - 1 - ki, ki - L)) >= 0
        lo = _iota((L, 128), 1) < 64
        lo_r = _iota((R, 128), 1) < 64
        g1 = lambda a: _cat0(a[0:M], a[2 * M:R1 + M])
        g2 = lambda a: _cat0(a[M:2 * M], a[R1 + M:])
        merge = lambda u1, u2: _cat0(u1[0:M], u2[0:M], u1[M:], u2[M:])

        def arrange_q(q):
            qm = q[:, 128:256]
            return [u.astype(BF16) for u in (q[:, :128], q[:, 256:], g1(qm), g2(qm))]

        def arrange(a):
            a1 = _cat0(a[0:M], a[2 * M:R1])
            a2 = _cat0(a[M:2 * M], a[R1:])
            cat = lambda *u: _cat0(*u).astype(BF16)
            m1, m2 = a1[:, 128:256], a2[:, 128:256]
            m2b, m2a = jnp.where(lo, 0.0, m2), jnp.where(lo, m2, 0.0)
            e = 2 * M
            return (cat(a1[:, :128], a2[:, :128], a2[:e, :128], a2[:e, :128]),
                    cat(a2[:, 256:], a1[:, 256:], a2[:e, 256:], a2[:e, 256:]),
                    cat(jnp.where(lo, m1, 0.0), jnp.where(lo, 0.0, m1), m2b[:e], m2a[:e]),
                    cat(m2b, m2a, m2b[:e], m2b[:e]))

        def scores(q, kt):
            return [_nt(u, w) for u, w in zip(q, kt)]

        def pv(s4, vt, pin):
            sa, sb, s1, s2 = s4
            if pin is not None:
                s1 = _cat0(s1[0:M] + pin[:, :NK], s1[M:])
            p, pa, pb, ra, rb = softmax2(jnp.where(is_a, sa, sb) + merge(s1, s2), is_a, allowed)
            oa, ob, o1, o2 = [_nn(u.astype(BF16), w) for u, w in zip((pa, pb, g1(p), g2(p)), vt)]
            return jnp.concatenate(
                [oa * ra, merge(o1, o2) * jnp.where(lo_r, ra, rb), ob * rb], axis=1).astype(BF16)

        return arrange_q, arrange, scores, pv

    def attn_one_layer():
        qi, ki = _iota((R1, R), 0), _iota((R1, R), 1)
        is_a = ki < L
        allowed = (qi < 2 * M) | (jnp.where(is_a, ki, ki - L) <= qi - M)
        head_a = _iota((L, PW), 1) < DH
        head_a1 = _iota((R1, PW), 1) < DH

        def arrange(a):
            a1 = _cat0(a[0:M], a[2 * M:])
            return _cat0(jnp.where(head_a, a1, 0.0), jnp.where(head_a, 0.0, a1)).astype(BF16)

        def pv(s, vt, pin=None):
            if pin is not None:
                s = _cat0(s[0:M] + pin[:, :R], s[M:])
            p, _, _, r0, r1 = softmax2(s, is_a, allowed)
            return (_nn(p.astype(BF16), vt) * jnp.where(head_a1, r0, r1)).astype(BF16)

        return lambda q: q.astype(BF16), arrange, _nt, pv

    def a_phase(h, attn, hooks, t=None):
        arrange_q, arrange, scores, pv = attn

        def proj(m, p):
            c = p * 3 + m
            w = pltpu.bitcast(wt_ref[c], BF16)
            if c >= NPRE or t is None:
                return _nn(h, w)
            y = _nn(_cat0(h[0:2 * M], h[R1:]), w)
            pre = pre_ref[c, pl.ds(_al(t * SEG, SEG), SEG), :].astype(F32)
            return _cat0(y[0:2 * M], pre, y[2 * M:])

        st = {'acc': None, 'o': {}, 'done': 0}

        def wo_upto(n):
            while st['done'] < n:
                pp = st['done']
                w = pltpu.bitcast(wo_ref[pp * PW // 2:(pp + 1) * PW // 2, :], BF16)
                y = _nn(st['o'].pop(pp), w)
                st['acc'] = y if st['acc'] is None else st['acc'] + y
                st['done'] += 1

        q, kt = arrange_q(proj(0, 0)), arrange(proj(1, 0))
        vt = arrange(proj(2, 0))
        for p in range(NPAIR):
            last = p == NPAIR - 1
            s = scores(q, kt)
            hooks(p - 0.5)
            if last:
                wo_upto(p - 1)
            else:
                q, kt = arrange_q(proj(0, p + 1)), arrange(proj(1, p + 1))
            st['o'][p] = pv(s, vt, hooks(p))
            if last:
                wo_upto(NPAIR)
            else:
                vt = arrange(proj(2, p + 1))
                wo_upto(min(p + 1, NPAIR - 1 - HELD))
        hooks(NPAIR)
        return st['acc']

    def b_phase1(t, layers=(0, 1), pins=None):
        w = jnp.concatenate([_cat0(*[pltpu.bitcast(pwqkv_ref[j * NC + c], BF16) for c in range(NC)])
                             for j in range(3)], axis=1)
        l0 = layers[0]
        qkv = _nn(_ln(xb_ref[l0 * SEG:(layers[-1] + 1) * SEG, :]).astype(BF16), w)
        for l in layers:
            rows = slice((l - l0) * SEG, (l - l0 + 1) * SEG)
            for c in range(NC):
                bq_ref[c, l * SEG:(l + 1) * SEG, :] = qkv[rows, c * 128:(c + 1) * 128]
                for j in range(2):
                    bkv_ref[l, j, c, 0:16, :] = bkv_ref[l, j, c, SEG:SEG + 16, :]
                    bkv_ref[l, j, c, 16:16 + SEG, :] = qkv[
                        rows, (j + 1) * D + c * 128:(j + 1) * D + (c + 1) * 128]
        bscale = BDH ** -0.5
        for l in layers:
            seg = t - 1 - 2 * l
            for r in range(SEG // 8):
                pos = seg * SEG + r * 8 + _iota((8, 128), 0)
                qrows = slice(l * SEG + r * 8, l * SEG + r * 8 + 8)
                kv = lambda j, c, w: bkv_ref[l, j, c, 16 + r * 8 - BDIL * w:24 + r * 8 - BDIL * w, :]
                q = [bq_ref[c, qrows, :] for c in range(NC)]
                lg = []
                for w in range(BW):
                    s = q[0] * kv(0, 0, w)
                    for c in range(1, NC):
                        s = s + q[c] * kv(0, c, w)
                    s = s + pltpu.roll(s, 64, 1)
                    s = s + pltpu.roll(s, 32, 1)
                    if r * 8 - BDIL * w < 0:
                        s = jnp.where(pos - BDIL * w >= 0, s, -1e9 / bscale)
                    lg.append(s)
                m = lg[0]
                for w in range(1, BW):
                    m = jnp.maximum(m, lg[w])
                e = [jnp.exp2((s - m) * (bscale * LOG2E)) for s in lg]
                den = e[0]
                for w in range(1, BW):
                    den = den + e[w]
                inv = 1.0 / den
                bits = None
                for c in range(NC):
                    o = e[0] * kv(1, c, 0)
                    for w in range(1, BW):
                        o = o + e[w] * kv(1, c, w)
                    o = o * inv
                    bq_ref[c, qrows, :] = o
                    ob = pltpu.bitcast(o, jnp.int32)
                    bits = ob if bits is None else bits | ob
                if pins is not None:
                    pins[PINS[l * 4 + r]] = pltpu.bitcast(bits & zero_ref[0], F32)

    def b_phase2(t, layers=(0, 1)):
        rows = slice(layers[0] * SEG, (layers[-1] + 1) * SEG)
        w = jnp.concatenate([pltpu.bitcast(pwo_ref[c], BF16) for c in range(NC)], axis=1)
        o = jnp.concatenate([bq_ref[c, rows, :] for c in range(NC)], axis=1).astype(BF16)
        yb = xb_ref[rows, :] + _nn(o, w)
        if 1 in layers:
            row = max(t - 3, 0) * SEG if isinstance(t, int) else jnp.maximum(t - 3, 0) * SEG
            out_ref[pl.ds(_al(row, SEG), SEG), :] = yb[-SEG:].astype(out_ref.dtype)
        return yb[:SEG]

    def with_b(t, at):
        at_qkv, at_wo1, at_wo2 = at
        box, pins = {}, {}

        def hooks(p):
            if p == at_qkv - 0.5:
                b_phase1(t, pins=pins)
            elif p == at_wo1 and at_wo2 == at_wo1:
                box['x2'] = b_phase2(t)
            elif p == at_wo1:
                box['x2'] = b_phase2(t, (0,))
            elif p == at_wo2:
                b_phase2(t, (1,))
            return pins.get(p)
        return hooks, box

    def x_seg(s):
        return x_ref[pl.ds(_al(s * SEG, SEG), SEG), :].astype(F32)

    def prepare_next(t, x2):
        sn = jnp.minimum(t + 1, NSEG - 1)
        hx_ref[0:SEG, :] = hxa_ref[pl.ds(_al(sn * SEG, SEG), SEG), :]
        hx_ref[SEG:, :] = _ln(x2).astype(BF16)
        res_ref[...] = _cat0(x_seg(sn), x2)

    def permuted_rows(c):
        return _cat0(*[st_ref[c, pl.ds(d, H, stride=BDH), :] for d in range(BDH)])

    bkv_ref[...] = jnp.zeros(bkv_ref.shape, F32)
    acc_ref[...] = jnp.zeros(acc_ref.shape, F32)
    st_ref[:, D:, :] = jnp.zeros((NC, st_ref.shape[1] - D, 128), F32)
    zero_ref[0] = 0
    first[0].wait()
    xl0 = _ln(x_ref[0:X0 + XB, :].astype(F32)).astype(BF16)
    hxa_ref[0:X0 + XB, :] = xl0
    hx_ref[0:SEG, :] = xl0[0:SEG]

    def early(u, carry):
        rows = pl.ds(_al((u // 3) * PW, 128), PW)
        dst = wl_ref.at[u % 3, rows, :]
        pltpu.make_async_copy(dst, dst, qsem.at[u]).wait()
        w = wl_ref[u % 3, rows, :]
        wn_ref[u] = pltpu.bitcast(_transposed(w), U32)
        pre_ref[u, 2 * SEG:X0, :] = _nt(hxa_ref[2 * SEG:X0, :], w).astype(BF16)
        return carry

    lax.fori_loop(0, NPRE, early, 0)
    mem0_copy.wait()
    mem0 = mem0_ref[...].astype(F32)
    mem_ref[...] = _cat0(mem0, mem0)

    def step0(p, carry):
        group(p, lambda cp: cp.wait())
        u = jnp.minimum(p, NU - 1)

        def wfirst(m):
            w = wl_ref[m, pl.ds(_al(p * PW, 128), PW), :]
            if m < 3:
                w = _transposed(w)
                wt_ref[p * 3 + m] = pltpu.bitcast(w, U32)
            else:
                wo_ref[pl.ds(_al(p * (PW // 2), 64), PW // 2), :] = pltpu.bitcast(w, U32)
            return w

        _, arrange, scores, pv = attn_one_layer()
        h = _cat0(mem_ref[...].astype(BF16), hx_ref[0:SEG, :])
        xrows = x_rows(p)
        xl = hxa_ref[xrows, :]
        for c in range(NC):
            st_ref[0, c * 128:(c + 1) * 128, :] = bwqkv_ref[u, :, c * 128:(c + 1) * 128].astype(F32).T
        pwqkv_ref[u] = pltpu.bitcast(permuted_rows(0).T.astype(BF16), U32)
        done = [0]

        def pre(n):
            c0, c1 = done[0], min(done[0] + n, NPRE)
            done[0] = c1
            for c in range(c0, c1):
                pre_ref[c, xrows, :] = _nn(xl, pltpu.bitcast(wn_ref[c], BF16)).astype(BF16)

        pre(S0[0])
        q = _nn(h, wfirst(0)).astype(BF16)
        pre(S0[1])
        kt = arrange(_nn(h, wfirst(1)))
        pre(S0[2])
        s = scores(q, kt)
        pre(S0[3])
        vt = arrange(_nn(h, wfirst(2)))
        pre(S0[4])
        o = pv(s, vt)
        pre(NPRE)
        acc_ref[...] += _nn(o, wfirst(3))
        nrows = x_rows(u + 1)
        hxa_ref[nrows, :] = _ln(x_ref[nrows, :].astype(F32)).astype(BF16)
        issue_rest(p + WIN, 0)
        return carry

    lax.fori_loop(0, NPAIR, step0, 0)
    bwo_copy.wait()
    for c in range(NC):
        st_ref[c, 0:D, :] = bwo_ref[:, c * 128:(c + 1) * 128].astype(F32)
        pwo_ref[c] = pltpu.bitcast(permuted_rows(c).astype(BF16), U32)
    zeros = jnp.zeros((SEG, D), F32)
    mem_ref[0:M, :] = acc_ref[0:M, :]
    xb_ref[...] = _cat0(x_seg(0) + acc_ref[2 * M:, :], zeros)
    hx_ref[...] = _cat0(hxa_ref[SEG:2 * SEG, :], zeros.astype(BF16))
    res_ref[...] = _cat0(x_seg(1), zeros)

    def single(t, carry):
        l = (t >= NSEG).astype(jnp.int32)
        mrows = pl.ds(_al(l * M, M), M)
        xrows = pl.ds(_al(l * SEG, SEG), SEG)
        hooks, box = with_b(t, B_AT1)
        mem = mem_ref[mrows, :]
        h = _cat0(_cat0(mem, mem).astype(BF16), hx_ref[xrows, :])
        acc = a_phase(h, attn_one_layer(), hooks)
        mem_ref[mrows, :] = acc[:M]
        xb_ref[xrows, :] = res_ref[xrows, :] + acc[2 * M:]
        prepare_next(t, box['x2'])
        return carry

    def step(i, carry):
        for j in range(UNROLL):
            t = i * UNROLL + j
            hooks, box = with_b(t, B_AT)
            h = _cat0(mem_ref[...].astype(BF16), hx_ref[...])
            acc = a_phase(h, attn_two_layers(), hooks, t)
            mem_ref[...] = acc[:2 * M]
            xb_ref[...] = res_ref[...] + acc[2 * M:]
            prepare_next(t, box['x2'])
        return carry

    def outer(i, carry):
        lax.fori_loop(1 + (NSEG - 1) * i, 2 + NSEG * i, single, 0)
        lax.fori_loop(2 // UNROLL, (NSEG - (NSEG - 2) * i) // UNROLL, step, 0)
        pl.when(i == 0)(out_a.start)
        pl.when(i == 1)(out_b.start)
        return carry

    lax.fori_loop(0, 2, outer, 0)
    b_phase1(NSEG + 2, (1,))
    b_phase2(NSEG + 2, (1,))
    out_c.start()
    out_a.wait()
    out_b.wait()
    out_c.wait()


@jax.jit
def pallas_interleave_layers__memory_aug_recurrent_mem_tr__sliding_local_dilated__prompt_kernel(
    A_x, A_mem0, A_Wq, A_Wk, A_Wv, A_Wo, A_seg_len, B_x, B_wqkv, B_wo,
):
    del A_seg_len, B_x
    wt = lambda w: jnp.transpose(w, (1, 2, 0)).reshape(HD, D)
    hbm = pl.BlockSpec(memory_space=pl.ANY)
    out = pl.pallas_call(
        _kernel,
        out_shape=jax.ShapeDtypeStruct((S, D), A_x.dtype),
        in_specs=[hbm] * 8,
        out_specs=hbm,
        scratch_shapes=[
            pltpu.VMEM((S, D), BF16),
            pltpu.VMEM((S, D), BF16),
            pltpu.VMEM((4, HD, D), BF16),
            pltpu.VMEM((HD // 2, D), U32),
            pltpu.VMEM((3 * NPAIR, D // 2, PW), U32),
            pltpu.VMEM((NU, 128, D), BF16),
            pltpu.VMEM((D, D), BF16),
            pltpu.VMEM((NU, 64, D), U32),
            pltpu.VMEM((NC, D // 2, 128), U32),
            pltpu.VMEM((NC, D + 32, 128), F32),
            pltpu.VMEM((R1, D), F32),
            pltpu.VMEM((2 * M, D), F32),
            pltpu.VMEM((2 * SEG, D), BF16),
            pltpu.VMEM((2 * SEG, D), F32),
            pltpu.VMEM((2 * SEG, D), F32),
            pltpu.VMEM((NC, 2 * SEG, 128), F32),
            pltpu.VMEM((2, 2, NC, 16 + SEG, 128), F32),
            pltpu.VMEM((NPRE, D // 2, PW), U32),
            pltpu.VMEM((S, D), BF16),
            pltpu.VMEM((NPRE, S, PW), BF16),
            pltpu.VMEM((M, D), BF16),
            pltpu.SMEM((1,), jnp.int32),
            pltpu.SemaphoreType.DMA((NPRE + 1,)),
            pltpu.SemaphoreType.DMA((NPAIR,)),
            pltpu.SemaphoreType.DMA((5,)),
        ],
        compiler_params=pltpu.CompilerParams(vmem_limit_bytes=120 * 2 ** 20, disable_bounds_checks=True),
    )(A_x.reshape(S, D), A_mem0.reshape(M, D), wt(A_Wq), wt(A_Wk), wt(A_Wv),
      A_Wo.reshape(HD, D), B_wqkv, B_wo)
    return out.reshape(1, S, D)
```
